```python
import jax
import jax.numpy as jnp

def _softmax(x, axis=-1):
    return jax.nn.softmax(x, axis=axis)

def _gelu(x):
    return jax.nn.gelu(x, approximate=True)

def _silu(x):
    return jax.nn.silu(x)

def _sigmoid(x):
    return jax.nn.sigmoid(x)

def _layernorm(x, axis=-1, eps=1e-05):
    m = jnp.mean(x, axis=axis, keepdims=True)
    v = jnp.var(x, axis=axis, keepdims=True)
    return (x - m) / jnp.sqrt(v + eps)

def _scatter_add(tgt, idx, src, axis=0):
    return tgt.at[idx].add(src)

def _segment_sum(src, seg, n):
    return jax.ops.segment_sum(src, seg, n)

class _Rng:

    def __init__(self, key):
        self._k = key

    def _next(self):
        self._k, sub = jax.random.split(self._k)
        return sub

    def normal(self, shape):
        return jax.random.normal(self._next(), shape, dtype=jnp.bfloat16)

    def randint(self, lo, hi, shape):
        return jax.random.randint(self._next(), shape, lo, hi, dtype=jnp.int32)

    def uniform(self, shape, lo=0.0, hi=1.0):
        return jax.random.uniform(self._next(), shape, jnp.bfloat16, lo, hi)

    def permutation(self, n):
        return jax.random.permutation(self._next(), n)
kernel_name = 'interleave_layers__memory_aug_infini_attn__moe_arch_mod__prompt'

def setup_inputs():
    _rng = _Rng(jax.random.key(int.from_bytes(__import__("os").urandom(4), "little")))
    _w = lambda a: (lambda t: t.astype(jnp.bfloat16) if jnp.issubdtype(t.dtype, jnp.floating) else t)(jnp.asarray(a))

    def _A_setup():
        B, S, D, H = (1, 2048, 1024, 32)
        N = 4
        L = max(1, S // N)
        sc = D ** (-0.5)
        return {'x': _w((lambda *s: _rng.normal(s) * 0.05)(B, N * L, D)), 'wq': _w((lambda *s: _rng.normal(s) * 0.05)(D, D) * sc), 'wk': _w((lambda *s: _rng.normal(s) * 0.05)(D, D) * sc), 'wv': _w((lambda *s: _rng.normal(s) * 0.05)(D, D) * sc), 'wo': _w((lambda *s: _rng.normal(s) * 0.05)(D, D) * sc), 'beta': _w((lambda *s: _rng.normal(s) * 0.05)(H))}
    _A_in = _A_setup()

    def _B_setup():
        B, S, D, F, C = (1, 2048, 1024, 3584, 2)
        return {'x': _w((lambda *s: _rng.normal(s) * 0.05)(B, S, D)), 'w_r': _w((lambda *s: _rng.normal(s) * 0.05)(D)), 'w_gate': _w((lambda *s: _rng.normal(s) * 0.05)(D, F)), 'w_up': _w((lambda *s: _rng.normal(s) * 0.05)(D, F)), 'w_down': _w((lambda *s: _rng.normal(s) * 0.05)(F, D))}
    _B_in = _B_setup()
    return {'A_x': _A_in['x'], 'A_wq': _A_in['wq'], 'A_wk': _A_in['wk'], 'A_wv': _A_in['wv'], 'A_wo': _A_in['wo'], 'A_beta': _A_in['beta'], 'B_x': _B_in['x'], 'B_w_r': _B_in['w_r'], 'B_w_gate': _B_in['w_gate'], 'B_w_up': _B_in['w_up'], 'B_w_down': _B_in['w_down']}

def reference(A_x, A_wq, A_wk, A_wv, A_wo, A_beta, B_x, B_w_r, B_w_gate, B_w_up, B_w_down):

    def _A_ref(x, wq, wk, wv, wo, beta):
        B, S, D = x.shape
        H = 32
        Dh = D // H
        N = 4
        L = S // N
        q = (lambda x, *d: x.transpose(*d))((x @ wq).reshape(B, S, H, Dh), 0, 2, 1, 3).reshape(B, H, N, L, Dh)
        k = (lambda x, *d: x.transpose(*d))((x @ wk).reshape(B, S, H, Dh), 0, 2, 1, 3).reshape(B, H, N, L, Dh)
        v = (lambda x, *d: x.transpose(*d))((x @ wv).reshape(B, S, H, Dh), 0, 2, 1, 3).reshape(B, H, N, L, Dh)
        phi = lambda t: jnp.where(t > 0, t + 1.0, jnp.exp(t))
        scale = Dh ** (-0.5)
        ar = jnp.arange(L)
        mask = (lambda x, dt: x.astype(dt))(ar[:, None] < ar[None, :], x.dtype) * -1000000000.0
        g = _sigmoid(beta).reshape(1, H, 1, 1)
        M = jnp.einsum('bhd,bhe->bhde', q[:, :, 0, 0, :] * 0.0, q[:, :, 0, 0, :] * 0.0)
        z = q[:, :, 0, 0, :] * 0.0
        outs = []
        for s in range(N):
            qs, ks, vs = (q[:, :, s].copy(), k[:, :, s].copy(), v[:, :, s].copy())
            logits = jnp.einsum('bhqd,bhkd->bhqk', qs, ks) * scale + mask
            p = _softmax(logits, axis=-1)
            a_dot = jnp.einsum('bhqk,bhkd->bhqd', p, vs)
            pq = phi(qs)
            num = jnp.einsum('bhld,bhde->bhle', pq, M)
            den = jnp.einsum('bhld,bhd->bhl', pq, z)[..., None] + 1e-06
            a_mem = num / den
            o = g * a_mem + (1.0 - g) * a_dot
            outs.append(o)
            pk = phi(ks)
            M = M + jnp.einsum('bhld,bhle->bhde', pk, vs)
            z = z + jnp.einsum('bhld->bhd', pk)
        o = (lambda x, *d: x.transpose(*d))(jnp.stack(outs, 2).reshape(B, H, S, Dh), 0, 2, 1, 3).reshape(B, S, D)
        return o @ wo

    def _B_ref(x, w_r, w_gate, w_up, w_down):
        B, S, D = x.shape
        C = 2
        r = x @ w_r
        idx = jnp.argsort(-r, axis=-1)[:, :C]
        idx_e = jnp.repeat(idx.reshape(B, C, 1), D, axis=2)
        x_sel = jnp.take_along_axis(x, idx_e, axis=1)
        g = _silu(x_sel @ w_gate)
        u = x_sel @ w_up
        y = g * u @ w_down
        r_sel = _sigmoid(jnp.take_along_axis(r, idx, axis=1))
        y = y * r_sel.reshape(B, C, 1)
        b_off = (jnp.arange(B) * S).reshape(B, 1)
        flat_idx = (idx + b_off).reshape(B * C)
        zero = (x * 0.0).reshape(B * S, D)
        upd = _scatter_add(zero, flat_idx, y.reshape(B * C, D), axis=0)
        return x + upd.reshape(B, S, D)
    x = A_x
    x = x + _A_ref(_layernorm(x, axis=-1), A_wq, A_wk, A_wv, A_wo, A_beta)
    x = x + _B_ref(_layernorm(x, axis=-1), B_w_r, B_w_gate, B_w_up, B_w_down)
    x = x + _A_ref(_layernorm(x, axis=-1), A_wq, A_wk, A_wv, A_wo, A_beta)
    x = x + _B_ref(_layernorm(x, axis=-1), B_w_r, B_w_gate, B_w_up, B_w_down)
    return x
```

```python
import functools

import jax
import jax.numpy as jnp
from jax import lax
import jax.experimental.pallas as pl
import jax.experimental.pallas.tpu as pltpu

S, D, H, DH, NSEG, L, F = 2048, 1024, 32, 32, 4, 512, 3584
G = 8
RB = 256
NRB = S // RB
T = 128
EPS = 1e-05
LOG2E = 1.4426950408889634
QSCALE = (DH ** -0.5) * LOG2E
NEG = -1e30
NT = (((1,), (1,)), ((), ()))

f32 = jnp.float32
bf16 = jnp.bfloat16


def _ln(x):
    m = jnp.mean(x, axis=-1, keepdims=True)
    c = x - m
    v = jnp.mean(c * c, axis=-1, keepdims=True)
    return c * lax.rsqrt(v + EPS)


def _phi(t):
    return jnp.where(t > 0, t + 1.0, jnp.exp(t))


def _sigmoid(t):
    return 1.0 / (1.0 + jnp.exp(-t))


def _kernel(zero_smem, beta_smem, x_hbm, wq_hbm, wk_hbm, wv_hbm, wo_hbm, wr_hbm,
            wg_hbm, wu_hbm, wd_hbm, out_hbm,
            x_sc, xb_sc, xn_sc, wq_sc, wk_sc, wv_sc, wo_sc, wqT_sc, wvT_sc, wr_sc,
            wg_sc, wu_sc, wd_sc, k_sc, pk_sc, qT_sc, pqT_sc, vT_sc, o_sc, z_sc,
            gt_sc, r_sc, s0_sc, s1_sc, am_sc, xm_sc, sems):
    cp = {
        "wq": pltpu.make_async_copy(wq_hbm, wq_sc, sems.at[0]),
        "wv": pltpu.make_async_copy(wv_hbm, wv_sc, sems.at[1]),
        "x": pltpu.make_async_copy(x_hbm, xb_sc, sems.at[2]),
        "wk": pltpu.make_async_copy(wk_hbm, wk_sc, sems.at[3]),
        "wo": pltpu.make_async_copy(wo_hbm, wo_sc, sems.at[4]),
        "wr": pltpu.make_async_copy(wr_hbm, wr_sc, sems.at[5]),
        "wg": pltpu.make_async_copy(wg_hbm, wg_sc, sems.at[6]),
        "wu": pltpu.make_async_copy(wu_hbm, wu_sc, sems.at[7]),
        "wd": pltpu.make_async_copy(wd_hbm, wd_sc, sems.at[8]),
    }
    for c in cp.values():
        c.start()
    zero = zero_smem[0]

    def gate_body(h, carry):
        gt_sc[h] = _sigmoid(jnp.full((8, 128), beta_smem[h], f32))
        return carry
    lax.fori_loop(0, H, gate_body, 0)

    cp["wq"].wait()
    for j in range(4):
        for i in range(4):
            wqT_sc[256 * j:256 * (j + 1), 256 * i:256 * (i + 1)] = wq_sc[256 * i:256 * (i + 1), 256 * j:256 * (j + 1)].T
    cp["wv"].wait()
    for j in range(4):
        for i in range(4):
            wvT_sc[256 * j:256 * (j + 1), 256 * i:256 * (i + 1)] = wv_sc[256 * i:256 * (i + 1), 256 * j:256 * (j + 1)].T

    cp["x"].wait()
    def ln0_body(rb, carry):
        rows = pl.ds(pl.multiple_of(rb * RB, RB), RB)
        x = xb_sc[rows, :].astype(f32)
        x_sc[rows, :] = x
        xn_sc[rows, :] = _ln(x).astype(bf16)
        return carry
    lax.fori_loop(0, NRB, ln0_body, 0)
    cp["wk"].wait()

    row = lax.broadcasted_iota(jnp.int32, (T, T), 0)
    col = lax.broadcasted_iota(jnp.int32, (T, T), 1)
    cmask = row <= col
    hmask = (row // 32) == (col // 32)
    zrow = lax.broadcasted_iota(jnp.int32, (32, T), 0)
    zcol = lax.broadcasted_iota(jnp.int32, (32, T), 1)
    zmask = (zrow // 8) == (zcol // 32)
    sb = [s0_sc, s1_sc]

    def sds(off, n):
        return pl.ds(pl.multiple_of(zero + off, 128), n)

    def proj_body(rb, carry):
        rows = pl.ds(pl.multiple_of(rb * RB, RB), RB)
        xb = xn_sc[rows, :]
        kk = jnp.dot(xb, wk_sc[...], preferred_element_type=f32)
        pk = _phi(kk)
        zp = pk[0:8]
        for r in range(1, RB // 8):
            zp = zp + pk[8 * r:8 * r + 8]
        for g in range(G):
            k_sc[g, rows, :] = kk[:, 128 * g:128 * (g + 1)].astype(bf16)
            pk_sc[g, rows, :] = pk[:, 128 * g:128 * (g + 1)].astype(bf16)
            z_sc[rb, g] = zp[:, 128 * g:128 * (g + 1)]
        qq = lax.dot_general(wqT_sc[...], xb, NT, preferred_element_type=f32)
        pq = _phi(qq)
        for g in range(G):
            qT_sc[rb, g] = (qq[128 * g:128 * (g + 1)] * QSCALE).astype(bf16)
            pqT_sc[rb, g] = pq[128 * g:128 * (g + 1)].astype(bf16)
        vv = lax.dot_general(wvT_sc[...], xb, NT, preferred_element_type=f32)
        for g in range(G):
            vT_sc[rb, g] = vv[128 * g:128 * (g + 1)].astype(bf16)
        return carry

    def attn_body(g, carry):
        gates = [gt_sc[4 * g + h] for h in range(4)]
        gates32 = [jnp.concatenate([t] * 4, axis=0) for t in gates]

        def mkW(s, i):
            QT = qT_sc[2 * s + i // 2, g, :, (i % 2) * T:(i % 2 + 1) * T]
            z = jnp.zeros((32, T), bf16)
            Ws = []
            for h in range(4):
                Ws.append(jnp.concatenate([QT[32 * h:32 * h + 32] if hh == h else z for hh in range(4)], axis=0))
            return jnp.concatenate(Ws, axis=1)

        def qk_chunk(s, i, c, W, buf, m):
            K = k_sc[g, s * L + c * T:s * L + (c + 1) * T, :]
            S4 = jnp.dot(K, W, preferred_element_type=f32)
            for h in range(4):
                Sx = S4[:, T * h:T * (h + 1)]
                if c == i:
                    Sx = jnp.where(cmask, Sx, NEG)
                sb[buf][sds(c * T, T), T * h:T * (h + 1)] = Sx
                mm = Sx[0:8]
                for r in range(1, 16):
                    mm = jnp.maximum(mm, Sx[8 * r:8 * r + 8])
                m[h] = mm if m[h] is None else jnp.maximum(m[h], mm)

        def pv_tile(s, c, buf, m, l, O):
            for h in range(4):
                Sx = sb[buf][sds(c * T, T), T * h:T * (h + 1)]
                P = jnp.exp2(Sx - m[h])
                a = P[0:8] + P[8:16]
                b = P[16:24] + P[24:32]
                for r in range(2, 8, 2):
                    a = a + (P[16 * r:16 * r + 8] + P[16 * r + 8:16 * r + 16])
                    b = b + (P[16 * r + 16:16 * r + 24] + P[16 * r + 24:16 * r + 32])
                ll = a + b
                l[h] = ll if l[h] is None else l[h] + ll
                vt = vT_sc[2 * s + c // 2, g, 32 * h:32 * h + 32, (c % 2) * T:(c % 2 + 1) * T]
                o = jnp.dot(vt, P.astype(bf16), preferred_element_type=f32)
                O[h] = o if O[h] is None else O[h] + o

        def fin(s, i, l, O):
            outs = []
            for h in range(4):
                lt = jnp.sum(l[h], axis=0, keepdims=True)
                od = O[h] * (1.0 / lt)
                o = (1.0 - gates32[h]) * od
                if s > 0:
                    o = o + am_sc[32 * h:32 * h + 32, i * T:(i + 1) * T]
                outs.append(o)
            ot = jnp.concatenate(outs, axis=0).astype(bf16)
            o_sc[g, s * L + i * T:s * L + (i + 1) * T, :] = ot.T

        def mem_read(s, M):
            zs = z_sc[0, g]
            for rb in range(1, 2 * s):
                zs = zs + z_sc[rb, g]
            zs = jnp.sum(zs, axis=0, keepdims=True)
            zrows = jnp.where(zmask, zs, 0.0).astype(bf16)
            mbd = jnp.where(hmask, M, 0.0).astype(bf16)
            lhs = jnp.concatenate([mbd, zrows], axis=0)
            pq = jnp.concatenate([pqT_sc[2 * s, g], pqT_sc[2 * s + 1, g]], axis=1)
            nd = jnp.dot(lhs, pq, preferred_element_type=f32)
            for h in range(4):
                den = nd[128 + 8 * h:128 + 8 * h + 8] + 1e-06
                gd = jnp.concatenate([gates[h]] * 4, axis=1) / den
                am_sc[32 * h:32 * h + 32, :] = nd[32 * h:32 * h + 32] * jnp.concatenate([gd] * 4, axis=0)

        def mem_write(s, M):
            vt = jnp.concatenate([vT_sc[2 * s, g], vT_sc[2 * s + 1, g]], axis=1)
            pk = pk_sc[g, s * L:(s + 1) * L, :]
            inc = jnp.dot(vt, pk, preferred_element_type=f32)
            return inc if M is None else M + inc

        seq = [(s, i) for s in range(NSEG) for i in (3, 2, 1, 0)]
        prev = None
        M = None
        for n in range(len(seq) + 1):
            cur = seq[n] if n < len(seq) else None
            buf = n % 2
            nA = nB = 0
            if cur is not None:
                s, i = cur
                W = mkW(s, i)
                m = [None] * 4
                nA = i + 1
            if prev is not None:
                ps, pi, pm = prev
                l = [None] * 4
                O = [None] * 4
                nB = pi + 1
                if pi == 3:
                    if ps > 0:
                        mem_read(ps, M)
                    if ps < NSEG - 1:
                        M = mem_write(ps, M)
            for c in range(max(nA, nB)):
                if c < nA:
                    qk_chunk(s, i, c, W, buf, m)
                if c < nB:
                    pv_tile(ps, c, 1 - buf, pm, l, O)
            if prev is not None:
                fin(ps, pi, l, O)
            if cur is not None:
                m = [jnp.max(x, axis=0, keepdims=True) for x in m]
                prev = (s, i, m)
        return carry

    def out_body(layer, rb, carry):
        rows = pl.ds(pl.multiple_of(rb * RB, RB), RB)
        ob = jnp.concatenate([o_sc[g, rows, :] for g in range(G)], axis=1)
        x1 = x_sc[rows, :] + jnp.dot(ob, wo_sc[...], preferred_element_type=f32)
        c = x1 - jnp.mean(x1, axis=-1, keepdims=True)
        v = jnp.mean(c * c, axis=-1, keepdims=True)
        rs = lax.rsqrt(v + EPS)
        xm = c * rs
        xmb = xm.astype(bf16)
        xm_sc[rows, :] = xmb
        r = jnp.sum(xmb.astype(f32) * wr_sc[...].astype(f32), axis=-1, keepdims=True)
        r = r.astype(bf16).astype(f32)
        r_sc[rows, :] = jnp.broadcast_to(r, (RB, 128))
        x2 = x1 + xm
        x_sc[rows, :] = x2
        a = 1.0 + rs
        xnn = c * (a * lax.rsqrt(v * (a * a) + EPS))
        xn_sc[rows, :] = jnp.where(layer == 0, xnn, x2).astype(bf16)
        return carry

    def ffn(layer):
        R = r_sc[...]
        idx = lax.broadcasted_iota(jnp.int32, (S, 128), 0)
        m1 = jnp.max(R, axis=0, keepdims=True)
        i1v = jnp.min(jnp.where(R == m1, idx, S), axis=0, keepdims=True)
        R2 = jnp.where(idx == i1v, -jnp.inf, R)
        m2 = jnp.max(R2, axis=0, keepdims=True)
        i2v = jnp.min(jnp.where(R2 == m2, idx, S), axis=0, keepdims=True)
        i1 = jnp.clip(jnp.max(i1v), 0, S - 1)
        i2 = jnp.clip(jnp.max(i2v), 0, S - 1)
        b1 = pl.ds(pl.multiple_of((i1 // 8) * 8, 8), 8)
        b2 = pl.ds(pl.multiple_of((i2 // 8) * 8, 8), 8)
        xs = jnp.concatenate([xm_sc[b1, :], xm_sc[b2, :]], axis=0)
        gg = jnp.dot(xs, wg_sc[...], preferred_element_type=f32)
        uu = jnp.dot(xs, wu_sc[...], preferred_element_type=f32)
        hh = (gg * _sigmoid(gg) * uu).astype(bf16)
        y = jnp.dot(hh, wd_sc[...], preferred_element_type=f32)
        r8 = lax.broadcasted_iota(jnp.int32, (8, D), 0)
        s1 = jnp.concatenate([_sigmoid(m1)] * (D // 128), axis=1)
        s2 = jnp.concatenate([_sigmoid(m2)] * (D // 128), axis=1)
        x_sc[b1, :] = x_sc[b1, :] + jnp.where(r8 == i1 % 8, y[0:8] * s1, 0.0)
        x_sc[b2, :] = x_sc[b2, :] + jnp.where(r8 == i2 % 8, y[8:16] * s2, 0.0)
        for b in (b1, b2):
            xx = x_sc[b, :]
            xn_sc[b, :] = jnp.where(layer == 0, _ln(xx), xx).astype(bf16)

    def layer_body(layer, carry):
        lax.fori_loop(0, NRB, proj_body, 0)
        lax.fori_loop(0, G, attn_body, 0)

        @pl.when(layer == 0)
        def _():
            cp["wo"].wait()
            cp["wr"].wait()
        lax.fori_loop(0, NRB, functools.partial(out_body, layer), 0)

        @pl.when(layer == 0)
        def _():
            cp["wg"].wait()
            cp["wu"].wait()
            cp["wd"].wait()
        ffn(layer)
        return carry

    lax.fori_loop(0, 2, layer_body, 0)

    oc = pltpu.make_async_copy(xn_sc, out_hbm, sems.at[9])
    oc.start()
    oc.wait()


@jax.jit
def pallas_interleave_layers__memory_aug_infini_attn__moe_arch_mod__prompt_kernel(
    A_x: jax.Array,
    A_wq: jax.Array,
    A_wk: jax.Array,
    A_wv: jax.Array,
    A_wo: jax.Array,
    A_beta: jax.Array,
    B_x: jax.Array,
    B_w_r: jax.Array,
    B_w_gate: jax.Array,
    B_w_up: jax.Array,
    B_w_down: jax.Array,
):
    del B_x
    x = A_x.reshape(S, D)
    zero = jnp.zeros((1,), jnp.int32)
    beta = A_beta.astype(f32)
    wr = B_w_r.reshape(1, D)
    any_spec = pl.BlockSpec(memory_space=pl.ANY)
    smem_spec = pl.BlockSpec(memory_space=pltpu.SMEM)
    V = pltpu.VMEM
    scratch = [
        V((S, D), f32),
        V((S, D), bf16),
        V((S, D), bf16),
        V((D, D), bf16), V((D, D), bf16), V((D, D), bf16), V((D, D), bf16),
        V((D, D), bf16), V((D, D), bf16),
        V((1, D), bf16),
        V((D, F), bf16), V((D, F), bf16), V((F, D), bf16),
        V((G, S, 128), bf16), V((G, S, 128), bf16),
        V((NRB, G, 128, RB), bf16), V((NRB, G, 128, RB), bf16), V((NRB, G, 128, RB), bf16),
        V((G, S, 128), bf16),
        V((NRB, G, 8, 128), f32),
        V((H, 8, 128), f32),
        V((S, 128), f32),
        V((L, 512), f32), V((L, 512), f32),
        V((128, 512), f32),
        V((S, D), bf16),
        pltpu.SemaphoreType.DMA((10,)),
    ]
    out = pl.pallas_call(
        _kernel,
        in_specs=[smem_spec, smem_spec] + [any_spec] * 9,
        out_specs=any_spec,
        out_shape=jax.ShapeDtypeStruct((S, D), bf16),
        scratch_shapes=scratch,
        compiler_params=pltpu.CompilerParams(vmem_limit_bytes=110 * 1024 * 1024),
    )(zero, beta, x, A_wq, A_wk, A_wv, A_wo, wr, B_w_gate, B_w_up, B_w_down)
    return out.reshape(1, S, D)
```

```python
import functools

import jax
import jax.numpy as jnp
from jax import lax
import jax.experimental.pallas as pl
import jax.experimental.pallas.tpu as pltpu

S, D, H, DH, NSEG, L, F = 2048, 1024, 32, 32, 4, 512, 3584
G = 8
RB = 256
NRB = S // RB
OB = 512
OS = 128
NOB = S // OB
T = 128
NGB = 2
LAGQ = 4
LAGP = 1
NSLOT = LAGQ + 1
EPS = 1e-05
LOG2E = 1.4426950408889634
QSCALE = (DH ** -0.5) * LOG2E
NEG = -1e30
NT = (((1,), (1,)), ((), ()))

f32 = jnp.float32
bf16 = jnp.bfloat16
u32 = jnp.uint32


def _phi(t):
    return jnp.where(t > 0, t + 1.0, jnp.exp(t))


def _sigmoid(t):
    return 1.0 / (1.0 + jnp.exp(-t))


def _pk(x):
    return pltpu.bitcast(x, u32)


def _upk(x):
    return pltpu.bitcast(x, bf16)


def _ln_stats(x):
    c = x - jnp.mean(x, axis=-1, keepdims=True)
    v = jnp.mean(c * c, axis=-1, keepdims=True)
    return c, v


def _row_fold(x, op):
    parts = [x[8 * r:8 * r + 8] for r in range(x.shape[0] // 8)]
    while len(parts) > 1:
        parts = [op(parts[i], parts[i + 1]) if i + 1 < len(parts) else parts[i] for i in range(0, len(parts), 2)]
    return parts[0]


def _kernel(zero_smem, beta_smem, x_hbm, wq_hbm, wk_hbm, wv_hbm, wo_hbm, wr_hbm,
            wg_hbm, wu_hbm, wd_hbm, out_hbm,
            x_sc, xb_sc, xn_sc, xm_sc, wq_sc, wk_sc, wv_sc, wo_sc, wqT_sc, wvT_sc, wr_sc,
            wg_sc, wu_sc, wd_sc, k_sc, pk_sc, qT_sc, pqT_sc, vT_sc, o_sc, z_sc,
            gt_sc, am_sc, sems, osems, *s_sc):
    cp = {
        "wq": pltpu.make_async_copy(wq_hbm, wq_sc, sems.at[0]),
        "wv": pltpu.make_async_copy(wv_hbm, wv_sc, sems.at[1]),
        "x": pltpu.make_async_copy(x_hbm, xb_sc, sems.at[2]),
        "wk": pltpu.make_async_copy(wk_hbm, wk_sc, sems.at[3]),
        "wo": pltpu.make_async_copy(wo_hbm, wo_sc, sems.at[4]),
        "wr": pltpu.make_async_copy(wr_hbm, wr_sc, sems.at[5]),
        "wg": pltpu.make_async_copy(wg_hbm, wg_sc, sems.at[6]),
        "wu": pltpu.make_async_copy(wu_hbm, wu_sc, sems.at[7]),
        "wd": pltpu.make_async_copy(wd_hbm, wd_sc, sems.at[8]),
    }
    for c in cp.values():
        c.start()
    zero = zero_smem[0]

    def rows_of(rb):
        return pl.ds(pl.multiple_of(rb * RB, RB), RB)

    def out_copy(i):
        rows = pl.ds(pl.multiple_of(i * OB, OB), OB)
        return pltpu.make_async_copy(xn_sc.at[rows, :], out_hbm.at[rows, :], osems.at[i])

    def gate_body(h, carry):
        gt_sc[h] = _sigmoid(jnp.full((8, 128), beta_smem[h], f32))
        return carry
    lax.fori_loop(0, H, gate_body, 0)

    cp["wq"].wait()
    for j in range(4):
        for i in range(4):
            wqT_sc[256 * j:256 * (j + 1), 256 * i:256 * (i + 1)] = wq_sc[256 * i:256 * (i + 1), 256 * j:256 * (j + 1)].T
    cp["wv"].wait()
    for j in range(4):
        for i in range(4):
            wvT_sc[256 * j:256 * (j + 1), 256 * i:256 * (i + 1)] = wv_sc[256 * i:256 * (i + 1), 256 * j:256 * (j + 1)].T

    cp["x"].wait()

    def ln0_body(rb, carry):
        rows = rows_of(rb)
        x = xb_sc[rows, :].astype(f32)
        x_sc[rows, :] = x
        c, v = _ln_stats(x)
        xn_sc[rows, :] = (c * lax.rsqrt(v + EPS)).astype(bf16)
        return carry
    lax.fori_loop(0, NRB, ln0_body, 0)
    cp["wk"].wait()

    row = lax.broadcasted_iota(jnp.int32, (T, T), 0)
    col = lax.broadcasted_iota(jnp.int32, (T, T), 1)
    cmask = row <= col
    hmask = (row // 32) == (col // 32)
    zrow = lax.broadcasted_iota(jnp.int32, (32, T), 0)
    zcol = lax.broadcasted_iota(jnp.int32, (32, T), 1)
    zmask = (zrow // 8) == (zcol // 32)

    def proj_body(rb, carry):
        rows = rows_of(rb)
        xb = xn_sc[rows, :]
        kk = jnp.dot(xb, wk_sc[...], preferred_element_type=f32)
        pk = _phi(kk)
        zp = _row_fold(pk, jnp.add)
        for g in range(G):
            k_sc[g, rows, :] = kk[:, 128 * g:128 * (g + 1)].astype(bf16)
            pk_sc[g, rows, :] = pk[:, 128 * g:128 * (g + 1)].astype(bf16)
            z_sc[rb, g] = zp[:, 128 * g:128 * (g + 1)]
        qq = lax.dot_general(wqT_sc[...], xb, NT, preferred_element_type=f32)
        pq = _phi(qq)
        for g in range(G):
            qT_sc[rb, g] = (qq[128 * g:128 * (g + 1)] * QSCALE).astype(bf16)
            pqT_sc[rb, g] = pq[128 * g:128 * (g + 1)].astype(bf16)
        vv = lax.dot_general(wvT_sc[...], xb, NT, preferred_element_type=f32)
        for g in range(G):
            vT_sc[rb, g] = vv[128 * g:128 * (g + 1)].astype(bf16)
        return carry

    def attn_body(gb, carry):
        tiles = [(gg, s, i) for gg in range(NGB) for s in range(NSEG) for i in (3, 2, 1, 0)]
        stream = [(t, c) for t, (gg, s, i) in enumerate(tiles) for c in range(i + 1)]
        n = len(stream)
        m, l, O, W, P, M = {}, {}, {}, {}, {}, {}

        def grp(gg):
            return gb * NGB + gg

        def sref(k, h):
            return s_sc[k % NSLOT].at[pl.ds(pl.multiple_of(zero, 8), T), T * h:T * (h + 1)]

        def mem_read(gg, s):
            g = grp(gg)
            zs = z_sc[0, g]
            for rb in range(1, 2 * s):
                zs = zs + z_sc[rb, g]
            zs = jnp.sum(zs, axis=0, keepdims=True)
            zrows = jnp.where(zmask, zs, 0.0).astype(bf16)
            mbd = jnp.where(hmask, M[gg], 0.0).astype(bf16)
            lhs = jnp.concatenate([mbd, zrows], axis=0)
            pq = jnp.concatenate([pqT_sc[2 * s, g], pqT_sc[2 * s + 1, g]], axis=1)
            nd = jnp.dot(lhs, pq, preferred_element_type=f32)
            for h in range(4):
                den = nd[128 + 8 * h:128 + 8 * h + 8] + 1e-06
                gd = jnp.concatenate([gt_sc[4 * g + h]] * 4, axis=1) / den
                am_sc[32 * h:32 * h + 32, :] = nd[32 * h:32 * h + 32] * jnp.concatenate([gd] * 4, axis=0)

        def mem_write(gg, s):
            g = grp(gg)
            vt = jnp.concatenate([vT_sc[2 * s, g], vT_sc[2 * s + 1, g]], axis=1)
            pk = pk_sc[g, s * L:(s + 1) * L, :]
            inc = jnp.dot(vt, pk, preferred_element_type=f32)
            M[gg] = inc if s == 0 else M[gg] + inc

        def qk(k):
            t, c = stream[k]
            gg, s, i = tiles[t]
            g = grp(gg)
            if c == 0:
                QT = qT_sc[2 * s + i // 2, g, :, (i % 2) * T:(i % 2 + 1) * T]
                z = jnp.zeros((32, T), bf16)
                W[t] = jnp.concatenate(
                    [jnp.concatenate([QT[32 * h:32 * h + 32] if hh == h else z for hh in range(4)], axis=0)
                     for h in range(4)], axis=1)
                m[t] = [None] * 4
            k0 = s * L + c * T
            K = k_sc[g, k0:k0 + T, :]
            S4 = jnp.dot(K, W[t], preferred_element_type=f32)
            for h in range(4):
                Sx = S4[:, T * h:T * (h + 1)]
                if c == i:
                    Sx = jnp.where(cmask, Sx, NEG)
                sref(k, h)[...] = Sx
                mm = Sx[0:8]
                for r in range(1, 16):
                    mm = jnp.maximum(mm, Sx[8 * r:8 * r + 8])
                m[t][h] = mm if m[t][h] is None else jnp.maximum(m[t][h], mm)
            if c == i:
                m[t] = [jnp.max(x, axis=0, keepdims=True) for x in m[t]]

        def ex(k):
            t, c = stream[k]
            if c == 0:
                l[t] = [None] * 4
            out = []
            for h in range(4):
                Pp = jnp.exp2(sref(k, h)[...] - m[t][h])
                a = Pp[0:8] + Pp[8:16]
                b = Pp[16:24] + Pp[24:32]
                for r in range(2, 8, 2):
                    a = a + (Pp[16 * r:16 * r + 8] + Pp[16 * r + 8:16 * r + 16])
                    b = b + (Pp[16 * r + 16:16 * r + 24] + Pp[16 * r + 24:16 * r + 32])
                ll = a + b
                l[t][h] = ll if l[t][h] is None else l[t][h] + ll
                out.append(Pp.astype(bf16))
            P[k] = out

        def pv(k):
            t, c = stream[k]
            gg, s, i = tiles[t]
            g = grp(gg)
            if c == 0:
                O[t] = [None] * 4
            for h in range(4):
                vt = vT_sc[2 * s + c // 2, g, 32 * h:32 * h + 32, (c % 2) * T:(c % 2 + 1) * T]
                o = jnp.dot(vt, P[k][h], preferred_element_type=f32)
                O[t][h] = o if O[t][h] is None else O[t][h] + o
            del P[k]
            if c == i:
                outs = []
                for h in range(4):
                    lt = jnp.sum(l[t][h], axis=0, keepdims=True)
                    gt = jnp.concatenate([gt_sc[4 * g + h]] * 4, axis=0)
                    o = O[t][h] * ((1.0 - gt) * (1.0 / lt))
                    if s > 0:
                        o = o + am_sc[32 * h:32 * h + 32, i * T:(i + 1) * T]
                    outs.append(o)
                ot = jnp.concatenate(outs, axis=0).astype(bf16)
                r0 = s * L + i * T
                o_sc[g, r0:r0 + T, :] = ot.T
                del l[t], O[t], m[t], W[t]
                if i == 3 and s < NSEG - 1:
                    mem_write(gg, s)
                if i == 0 and s < NSEG - 1:
                    mem_read(gg, s + 1)

        for pos in range(n + LAGQ + LAGP):
            if pos < n:
                qk(pos)
            if 0 <= pos - LAGQ - LAGP < n:
                pv(pos - LAGQ - LAGP)
            if 0 <= pos - LAGQ < n:
                ex(pos - LAGQ)
        return carry

    def out_body(layer, ob_i, top):
        m1, i1, m2, i2 = top
        base = pl.multiple_of(ob_i * OB, OB)
        def oproj(k):
            ob = jnp.concatenate([o_sc[g, pl.ds(base + k * OS, OS), :] for g in range(G)], axis=1)
            return jnp.dot(ob, wo_sc[...], preferred_element_type=f32)

        nxt = oproj(0)
        for k in range(OB // OS):
            rows = pl.ds(base + k * OS, OS)
            acc = nxt
            if k + 1 < OB // OS:
                nxt = oproj(k + 1)
            x1 = x_sc[rows, :] + acc
            c, v = _ln_stats(x1)
            rs = lax.rsqrt(v + EPS)
            xm = c * rs
            xmb = xm.astype(bf16)
            xm_sc[rows, :] = xmb
            r = jnp.sum(xmb.astype(f32) * wr_sc[...].astype(f32), axis=-1, keepdims=True)
            r = r.astype(bf16).astype(f32)
            x2 = x1 + xm
            x_sc[rows, :] = x2
            a = 1.0 + rs
            xnn = c * (a * lax.rsqrt(v * (a * a) + EPS))
            xn_sc[rows, :] = jnp.where(layer == 0, xnn, x2).astype(bf16)
            sub = lax.broadcasted_iota(jnp.int32, (8, 1), 0) + (base + k * OS)
            for j in range(OS // 8):
                rj = r[8 * j:8 * j + 8]
                idx = sub + 8 * j
                g1 = rj > m1
                g2 = rj > m2
                m2 = jnp.where(g1, m1, jnp.where(g2, rj, m2))
                i2 = jnp.where(g1, i1, jnp.where(g2, idx, i2))
                m1 = jnp.where(g1, rj, m1)
                i1 = jnp.where(g1, idx, i1)

        @pl.when(layer == 1)
        def _():
            out_copy(ob_i).start()
        return m1, i1, m2, i2

    def ffn(layer, top):
        m1, i1, m2, i2 = top
        cv = jnp.concatenate([m1, m2], axis=0)
        ci = jnp.concatenate([i1, i2], axis=0)
        v1 = jnp.max(cv, axis=0, keepdims=True)
        j1 = jnp.min(jnp.where(cv == v1, ci, S), axis=0, keepdims=True)
        cv2 = jnp.where(ci == j1, -jnp.inf, cv)
        v2 = jnp.max(cv2, axis=0, keepdims=True)
        j2 = jnp.min(jnp.where(cv2 == v2, ci, S), axis=0, keepdims=True)
        t1 = jnp.clip(j1[0, 0], 0, S - 1)
        t2 = jnp.clip(j2[0, 0], 0, S - 1)
        b1 = pl.ds(pl.multiple_of((t1 // 8) * 8, 8), 8)
        b2 = pl.ds(pl.multiple_of((t2 // 8) * 8, 8), 8)
        xs = jnp.concatenate([xm_sc[b1, :], xm_sc[b2, :]], axis=0)
        gg = jnp.dot(xs, wg_sc[...], preferred_element_type=f32)
        uu = jnp.dot(xs, wu_sc[...], preferred_element_type=f32)
        hh = (gg * _sigmoid(gg) * uu).astype(bf16)
        ys = []
        for n in range(4):
            ys.append(jnp.dot(hh, wd_sc[:, 256 * n:256 * (n + 1)], preferred_element_type=f32))
        y = jnp.concatenate(ys, axis=1)
        r8 = lax.broadcasted_iota(jnp.int32, (8, D), 0)
        x_sc[b1, :] = x_sc[b1, :] + jnp.where(r8 == t1 % 8, y[0:8] * _sigmoid(v1), 0.0)
        x_sc[b2, :] = x_sc[b2, :] + jnp.where(r8 == t2 % 8, y[8:16] * _sigmoid(v2), 0.0)

        @pl.when(layer == 1)
        def _():
            for i in range(NOB):
                out_copy(i).wait()

        for b in (b1, b2):
            xx = x_sc[b, :]
            c, v = _ln_stats(xx)
            xn_sc[b, :] = jnp.where(layer == 0, c * lax.rsqrt(v + EPS), xx).astype(bf16)

        @pl.when(layer == 1)
        def _():
            c1 = pltpu.make_async_copy(xn_sc.at[b1, :], out_hbm.at[b1, :], sems.at[9])
            c1.start()

            @pl.when(t1 // 8 != t2 // 8)
            def _():
                c2 = pltpu.make_async_copy(xn_sc.at[b2, :], out_hbm.at[b2, :], sems.at[10])
                c2.start()
                c2.wait()
            c1.wait()

    def layer_body(layer, carry):
        lax.fori_loop(0, NRB, proj_body, 0)
        lax.fori_loop(0, G // NGB, attn_body, 0)

        @pl.when(layer == 0)
        def _():
            cp["wo"].wait()
            cp["wr"].wait()
        top = (jnp.full((8, 1), -jnp.inf, f32), jnp.zeros((8, 1), jnp.int32),
               jnp.full((8, 1), -jnp.inf, f32), jnp.ones((8, 1), jnp.int32))
        top = lax.fori_loop(0, NOB, functools.partial(out_body, layer), top)

        @pl.when(layer == 0)
        def _():
            cp["wg"].wait()
            cp["wu"].wait()
            cp["wd"].wait()
        ffn(layer, top)
        return carry

    lax.fori_loop(0, 2, layer_body, 0)


@jax.jit
def pallas_interleave_layers__memory_aug_infini_attn__moe_arch_mod__prompt_kernel(
    A_x: jax.Array,
    A_wq: jax.Array,
    A_wk: jax.Array,
    A_wv: jax.Array,
    A_wo: jax.Array,
    A_beta: jax.Array,
    B_x: jax.Array,
    B_w_r: jax.Array,
    B_w_gate: jax.Array,
    B_w_up: jax.Array,
    B_w_down: jax.Array,
):
    del B_x
    x = A_x.reshape(S, D)
    zero = jnp.zeros((1,), jnp.int32)
    beta = A_beta.astype(f32)
    wr = B_w_r.reshape(1, D)
    any_spec = pl.BlockSpec(memory_space=pl.ANY)
    smem_spec = pl.BlockSpec(memory_space=pltpu.SMEM)
    V = pltpu.VMEM
    scratch = [
        V((S, D), f32),
        V((S, D), bf16),
        V((S, D), bf16),
        V((S, D), bf16),
        V((D, D), bf16), V((D, D), bf16), V((D, D), bf16), V((D, D), bf16),
        V((D, D), bf16), V((D, D), bf16),
        V((1, D), bf16),
        V((D, F), bf16), V((D, F), bf16), V((F, D), bf16),
        V((G, S, 128), bf16), V((G, S, 128), bf16),
        V((NRB, G, 128, RB), bf16), V((NRB, G, 128, RB), bf16), V((NRB, G, 128, RB), bf16),
        V((G, S, 128), bf16),
        V((NRB, G, 8, 128), f32),
        V((H, 8, 128), f32),
        V((128, 512), f32),
        pltpu.SemaphoreType.DMA((11,)),
        pltpu.SemaphoreType.DMA((NOB,)),
    ] + [V((T, 512), f32)] * NSLOT
    out = pl.pallas_call(
        _kernel,
        in_specs=[smem_spec, smem_spec] + [any_spec] * 9,
        out_specs=any_spec,
        out_shape=jax.ShapeDtypeStruct((S, D), bf16),
        scratch_shapes=scratch,
        compiler_params=pltpu.CompilerParams(vmem_limit_bytes=120 * 1024 * 1024),
    )(zero, beta, x, A_wq, A_wk, A_wv, A_wo, wr, B_w_gate, B_w_up, B_w_down)
    return out.reshape(1, S, D)
```

```python
import functools

import jax
import jax.numpy as jnp
from jax import lax
import jax.experimental.pallas as pl
import jax.experimental.pallas.tpu as pltpu

S, D, H, DH, NSEG, L, F = 2048, 1024, 32, 32, 4, 512, 3584
G = 8
RB = 256
NRB = S // RB
OB = 1024
OS = 128
NOB = S // OB
FC = 256
PLAG = 1
TIE = True
T = 128
NGB = 1
LAGQ = 4
LAGP = 1
NSLOT = LAGQ + 1
EPS = 1e-05
LOG2E = 1.4426950408889634
QSCALE = (DH ** -0.5) * LOG2E
NEG = -1e30
NT = (((1,), (1,)), ((), ()))

f32 = jnp.float32
bf16 = jnp.bfloat16
u32 = jnp.uint32


def _phi(t):
    return jnp.where(t > 0, t + 1.0, jnp.exp(t))


def _sigmoid(t):
    return 1.0 / (1.0 + jnp.exp(-t))


def _pk(x):
    return pltpu.bitcast(x, u32)


def _upk(x):
    return pltpu.bitcast(x, bf16)


def _ln_stats(x):
    c = x - jnp.mean(x, axis=-1, keepdims=True)
    v = jnp.mean(c * c, axis=-1, keepdims=True)
    return c, v


def _row_fold(x, op):
    parts = [x[8 * r:8 * r + 8] for r in range(x.shape[0] // 8)]
    while len(parts) > 1:
        parts = [op(parts[i], parts[i + 1]) if i + 1 < len(parts) else parts[i] for i in range(0, len(parts), 2)]
    return parts[0]


def _kernel(zero_smem, beta_smem, x_hbm, wq_hbm, wk_hbm, wv_hbm, wo_hbm, wr_hbm,
            wg_hbm, wu_hbm, wd_hbm, out_hbm,
            x_sc, x2_sc, xb_sc, xn_sc, rs_sc, tv_sc, ti_sc, wq_sc, wk_sc, wv_sc, wo_sc, wqT_sc, wvT_sc, wr_sc,
            wg_sc, wu_sc, wd_sc, k_sc, pk_sc, qT_sc, pqT_sc, vT_sc, o_sc, z_sc,
            gt_sc, am_sc, sems, osems, *rest):
    s_sc, x1_sc = rest[:NSLOT], rest[NSLOT:]
    cp = {
        "wq": pltpu.make_async_copy(wq_hbm, wq_sc, sems.at[0]),
        "wv": pltpu.make_async_copy(wv_hbm, wv_sc, sems.at[1]),
        "x": pltpu.make_async_copy(x_hbm, xb_sc, sems.at[2]),
        "wk": pltpu.make_async_copy(wk_hbm, wk_sc, sems.at[3]),
        "wo": pltpu.make_async_copy(wo_hbm, wo_sc, sems.at[4]),
        "wr": pltpu.make_async_copy(wr_hbm, wr_sc, sems.at[5]),
        "wg": pltpu.make_async_copy(wg_hbm, wg_sc, sems.at[6]),
        "wu": pltpu.make_async_copy(wu_hbm, wu_sc, sems.at[7]),
        "wd": pltpu.make_async_copy(wd_hbm, wd_sc, sems.at[8]),
    }
    for c in cp.values():
        c.start()
    zero = zero_smem[0]

    def rows_of(rb):
        return pl.ds(pl.multiple_of(rb * RB, RB), RB)

    def out_copy(i):
        rows = pl.ds(pl.multiple_of(i * OB, OB), OB)
        return pltpu.make_async_copy(xn_sc.at[rows, :], out_hbm.at[rows, :], osems.at[i])

    def gate_body(h, carry):
        gt_sc[h] = _sigmoid(jnp.full((8, 128), beta_smem[h], f32))
        return carry
    lax.fori_loop(0, H, gate_body, 0)

    cp["wq"].wait()
    for j in range(4):
        for i in range(4):
            wqT_sc[256 * j:256 * (j + 1), 256 * i:256 * (i + 1)] = wq_sc[256 * i:256 * (i + 1), 256 * j:256 * (j + 1)].T
    cp["wv"].wait()
    for j in range(4):
        for i in range(4):
            wvT_sc[256 * j:256 * (j + 1), 256 * i:256 * (i + 1)] = wv_sc[256 * i:256 * (i + 1), 256 * j:256 * (j + 1)].T

    cp["x"].wait()

    def ln0_body(rb, carry):
        rows = rows_of(rb)
        x = xb_sc[rows, :].astype(f32)
        c, v = _ln_stats(x)
        xn_sc[rows, :] = (c * lax.rsqrt(v + EPS)).astype(bf16)
        return carry
    lax.fori_loop(0, NRB, ln0_body, 0)
    cp["wk"].wait()

    row = lax.broadcasted_iota(jnp.int32, (T, T), 0)
    col = lax.broadcasted_iota(jnp.int32, (T, T), 1)
    cmask = row <= col
    hmask = (row // 32) == (col // 32)
    zrow = lax.broadcasted_iota(jnp.int32, (32, T), 0)
    zcol = lax.broadcasted_iota(jnp.int32, (32, T), 1)
    zmask = (zrow // 8) == (zcol // 32)

    def proj_body(rb, carry):
        rows = rows_of(rb)
        xb = xn_sc[rows, :]
        kk = jnp.dot(xb, wk_sc[...], preferred_element_type=f32)
        pk = _phi(kk)
        zp = _row_fold(pk, jnp.add)
        for g in range(G):
            k_sc[g, rows, :] = kk[:, 128 * g:128 * (g + 1)].astype(bf16)
            pk_sc[g, rows, :] = pk[:, 128 * g:128 * (g + 1)].astype(bf16)
            z_sc[rb, g] = zp[:, 128 * g:128 * (g + 1)]
        qq = lax.dot_general(wqT_sc[...], xb, NT, preferred_element_type=f32)
        pq = _phi(qq)
        for g in range(G):
            qT_sc[rb, g] = (qq[128 * g:128 * (g + 1)] * QSCALE).astype(bf16)
            pqT_sc[rb, g] = pq[128 * g:128 * (g + 1)].astype(bf16)
        vv = lax.dot_general(wvT_sc[...], xb, NT, preferred_element_type=f32)
        for g in range(G):
            vT_sc[rb, g] = vv[128 * g:128 * (g + 1)].astype(bf16)
        return carry

    def attn_body(gb, carry):
        tiles = [(gg, s, i) for gg in range(NGB) for s in range(NSEG) for i in (3, 2, 1, 0)]
        stream = [(t, c) for t, (gg, s, i) in enumerate(tiles) for c in range(i + 1)]
        n = len(stream)
        m, l, O, W, P, M = {}, {}, {}, {}, {}, {}

        def grp(gg):
            return gb * NGB + gg

        def sref(k, h):
            return s_sc[k % NSLOT].at[pl.ds(pl.multiple_of(zero, 8), T), T * h:T * (h + 1)]

        def mem_read(gg, s):
            g = grp(gg)
            zs = z_sc[0, g]
            for rb in range(1, 2 * s):
                zs = zs + z_sc[rb, g]
            zs = jnp.sum(zs, axis=0, keepdims=True)
            zrows = jnp.where(zmask, zs, 0.0).astype(bf16)
            mbd = jnp.where(hmask, M[gg], 0.0).astype(bf16)
            lhs = jnp.concatenate([mbd, zrows], axis=0)
            pq = jnp.concatenate([pqT_sc[2 * s, g], pqT_sc[2 * s + 1, g]], axis=1)
            nd = jnp.dot(lhs, pq, preferred_element_type=f32)
            for h in range(4):
                den = nd[128 + 8 * h:128 + 8 * h + 8] + 1e-06
                gd = jnp.concatenate([gt_sc[4 * g + h]] * 4, axis=1) / den
                am_sc[32 * h:32 * h + 32, :] = nd[32 * h:32 * h + 32] * jnp.concatenate([gd] * 4, axis=0)

        def mem_write(gg, s):
            g = grp(gg)
            vt = jnp.concatenate([vT_sc[2 * s, g], vT_sc[2 * s + 1, g]], axis=1)
            pk = pk_sc[g, s * L:(s + 1) * L, :]
            inc = jnp.dot(vt, pk, preferred_element_type=f32)
            M[gg] = inc if s == 0 else M[gg] + inc

        def qk(k):
            t, c = stream[k]
            gg, s, i = tiles[t]
            g = grp(gg)
            if c == 0:
                QT = qT_sc[2 * s + i // 2, g, :, (i % 2) * T:(i % 2 + 1) * T]
                z = jnp.zeros((32, T), bf16)
                W[t] = jnp.concatenate(
                    [jnp.concatenate([QT[32 * h:32 * h + 32] if hh == h else z for hh in range(4)], axis=0)
                     for h in range(4)], axis=1)
                m[t] = [None] * 4
            k0 = s * L + c * T
            K = k_sc[g, k0:k0 + T, :]
            S4 = jnp.dot(K, W[t], preferred_element_type=f32)
            for h in range(4):
                Sx = S4[:, T * h:T * (h + 1)]
                if c == i:
                    Sx = jnp.where(cmask, Sx, NEG)
                sref(k, h)[...] = Sx
                mm = Sx[0:8]
                for r in range(1, 16):
                    mm = jnp.maximum(mm, Sx[8 * r:8 * r + 8])
                m[t][h] = mm if m[t][h] is None else jnp.maximum(m[t][h], mm)
            if c == i:
                m[t] = [jnp.max(x, axis=0, keepdims=True) for x in m[t]]

        def ex(k):
            t, c = stream[k]
            if c == 0:
                l[t] = [None] * 4
            out = []
            for h in range(4):
                Pp = jnp.exp2(sref(k, h)[...] - m[t][h])
                a = Pp[0:8] + Pp[8:16]
                b = Pp[16:24] + Pp[24:32]
                for r in range(2, 8, 2):
                    a = a + (Pp[16 * r:16 * r + 8] + Pp[16 * r + 8:16 * r + 16])
                    b = b + (Pp[16 * r + 16:16 * r + 24] + Pp[16 * r + 24:16 * r + 32])
                ll = a + b
                l[t][h] = ll if l[t][h] is None else l[t][h] + ll
                out.append(Pp.astype(bf16))
            P[k] = out

        def pv(k):
            t, c = stream[k]
            gg, s, i = tiles[t]
            g = grp(gg)
            if c == 0:
                O[t] = [None] * 4
            for h in range(4):
                vt = vT_sc[2 * s + c // 2, g, 32 * h:32 * h + 32, (c % 2) * T:(c % 2 + 1) * T]
                o = jnp.dot(vt, P[k][h], preferred_element_type=f32)
                O[t][h] = o if O[t][h] is None else O[t][h] + o
            del P[k]
            if c == i:
                outs = []
                for h in range(4):
                    lt = jnp.sum(l[t][h], axis=0, keepdims=True)
                    gt = jnp.concatenate([gt_sc[4 * g + h]] * 4, axis=0)
                    o = O[t][h] * ((1.0 - gt) * (1.0 / lt))
                    if s > 0:
                        o = o + am_sc[32 * h:32 * h + 32, i * T:(i + 1) * T]
                    outs.append(o)
                ot = jnp.concatenate(outs, axis=0).astype(bf16)
                r0 = s * L + i * T
                o_sc[g, r0:r0 + T, :] = ot.T
                del l[t], O[t], m[t], W[t]
                if i == 3 and s < NSEG - 1:
                    mem_write(gg, s)
                if i == 0 and s < NSEG - 1:
                    mem_read(gg, s + 1)

        for pos in range(n + LAGQ + LAGP):
            if pos < n:
                qk(pos)
            if 0 <= pos - LAGQ - LAGP < n:
                pv(pos - LAGQ - LAGP)
            if 0 <= pos - LAGQ < n:
                ex(pos - LAGQ)
        return carry

    def out_body(last, ob_i, top):
        base = pl.multiple_of(ob_i * OB, OB)
        wr = wr_sc[...].astype(f32)
        wr_sum = jnp.sum(wr, axis=-1, keepdims=True)
        NK = OB // OS
        CH = OS // (D // 128)
        never = jnp.full((CH, 1), zero, jnp.int32) != 0
        src = x_sc if last else xb_sc
        dst = x2_sc if last else x_sc

        def proj_stats(k):
            rows = pl.ds(base + k * OS, OS)
            ob = jnp.concatenate([o_sc[g, rows, :] for g in range(G)], axis=1)
            x1 = src[rows, :].astype(f32) + jnp.dot(ob, wo_sc[...], preferred_element_type=f32)
            x1_sc[k][...] = x1
            s1 = s2 = st = None
            for n in range(D // 128):
                d = x1[:, 128 * n:128 * (n + 1)]
                s1 = d if s1 is None else s1 + d
                s2 = d * d if s2 is None else s2 + d * d
                t = d * wr[:, 128 * n:128 * (n + 1)]
                st = t if st is None else st + t
            mean = jnp.sum(s1, axis=-1, keepdims=True) * (1.0 / D)
            v = jnp.maximum(jnp.sum(s2, axis=-1, keepdims=True) * (1.0 / D) - mean * mean, 0.0)
            rs = lax.rsqrt(v + EPS)
            r = rs * (jnp.sum(st, axis=-1, keepdims=True) - mean * wr_sum)
            r = r.astype(bf16).astype(f32)
            rs_sc[rows, :] = jnp.broadcast_to(rs, (OS, 128))
            return mean, v, rs, r, [x1[0:CH, 128 * n:128 * n + 1] for n in range(D // 128)]

        def apply(k, mean, v, rs, toks):
            for n in range(D // 128):
                rows = pl.ds(base + k * OS + n * CH, CH)
                sl = slice(n * CH, (n + 1) * CH)
                mn, vn, rn = mean[sl], v[sl], rs[sl]
                if toks is not None:
                    mn = jnp.where(never, toks[n], mn)
                xr = x1_sc[k][pl.ds(pl.multiple_of(zero + n * CH, 8), CH), :]
                c = xr - mn
                x2 = xr + c * rn
                dst[rows, :] = x2
                if last:
                    xn_sc[rows, :] = x2.astype(bf16)
                else:
                    a = 1.0 + rn
                    xn_sc[rows, :] = (c * (a * lax.rsqrt(vn * (a * a) + EPS))).astype(bf16)

        def route(k, r, top):
            m1, i1, m2, i2 = top
            sub = lax.broadcasted_iota(jnp.int32, (8, 1), 0) + (base + k * OS)
            for j in range(OS // 8):
                rj = r[8 * j:8 * j + 8]
                idx = sub + 8 * j
                g1 = rj > m1
                g2 = rj > m2
                m2 = jnp.where(g1, m1, jnp.where(g2, rj, m2))
                i2 = jnp.where(g1, i1, jnp.where(g2, idx, i2))
                m1 = jnp.where(g1, rj, m1)
                i1 = jnp.where(g1, idx, i1)
            return m1, i1, m2, i2

        st_ = {}
        for k in range(NK + PLAG):
            if k < NK:
                st_[k] = proj_stats(k)
            if k - PLAG >= 0:
                mean, v, rs, r, _ = st_[k - PLAG]
                apply(k - PLAG, mean, v, rs, st_[k - PLAG + 1][4] if (TIE and k - PLAG + 1 < NK) else None)
                top = route(k - PLAG, r, top)
        m1, i1, m2, i2 = top
        if last:
            out_copy(ob_i).start()
        return m1, i1, m2, i2

    def out_phase(last):
        top = (jnp.full((8, 1), -jnp.inf, f32), jnp.zeros((8, 1), jnp.int32),
               jnp.full((8, 1), -jnp.inf, f32), jnp.ones((8, 1), jnp.int32))
        m1, i1, m2, i2 = lax.fori_loop(0, NOB, functools.partial(out_body, last), top)
        tv_sc[0:8, :] = jnp.broadcast_to(m1, (8, 128))
        tv_sc[8:16, :] = jnp.broadcast_to(m2, (8, 128))
        ti_sc[0:8, :] = jnp.broadcast_to(i1, (8, 128))
        ti_sc[8:16, :] = jnp.broadcast_to(i2, (8, 128))

    def ffn(layer):
        cv = tv_sc[...]
        ci = ti_sc[...]
        v1 = jnp.max(cv, axis=0, keepdims=True)
        j1 = jnp.min(jnp.where(cv == v1, ci, S), axis=0, keepdims=True)
        cv2 = jnp.where(ci == j1, -jnp.inf, cv)
        v2 = jnp.max(cv2, axis=0, keepdims=True)
        j2 = jnp.min(jnp.where(cv2 == v2, ci, S), axis=0, keepdims=True)
        t1 = jnp.clip(j1[0, 0], 0, S - 1)
        t2 = jnp.clip(j2[0, 0], 0, S - 1)
        b1 = pl.ds(pl.multiple_of((t1 // 8) * 8, 8), 8)
        b2 = pl.ds(pl.multiple_of((t2 // 8) * 8, 8), 8)
        xr = jnp.where(layer == 0, jnp.concatenate([x_sc[b1, :], x_sc[b2, :]], axis=0),
                       jnp.concatenate([x2_sc[b1, :], x2_sc[b2, :]], axis=0))
        rs = jnp.concatenate([rs_sc[b1, :], rs_sc[b2, :]], axis=0)[:, 0:1]
        c = xr - jnp.mean(xr, axis=-1, keepdims=True)
        xm = c * (rs / (1.0 + rs))
        xs = xm.astype(bf16)
        base = xr
        y = None
        for j in range(F // FC):
            gg = jnp.dot(xs, wg_sc[:, FC * j:FC * (j + 1)], preferred_element_type=f32)
            uu = jnp.dot(xs, wu_sc[:, FC * j:FC * (j + 1)], preferred_element_type=f32)
            hh = (gg * _sigmoid(gg) * uu).astype(bf16)
            t = jnp.dot(hh, wd_sc[FC * j:FC * (j + 1), :], preferred_element_type=f32)
            y = t if y is None else y + t
        r8 = lax.broadcasted_iota(jnp.int32, (8, D), 0)
        y1 = jnp.where(r8 == t1 % 8, y[0:8] * jnp.concatenate([_sigmoid(v1)] * (D // 128), axis=1), 0.0)
        y2 = jnp.where(r8 == t2 % 8, y[8:16] * jnp.concatenate([_sigmoid(v2)] * (D // 128), axis=1), 0.0)
        same = t1 // 8 == t2 // 8
        n1 = base[0:8] + (y1 + jnp.where(same, y2, 0.0))
        n2 = base[8:16] + (y2 + jnp.where(same, y1, 0.0))
        x_sc[b1, :] = n1
        x_sc[b2, :] = n2

        @pl.when(layer == 1)
        def _():
            for i in range(NOB):
                out_copy(i).wait()

        for b, xx in ((b1, n1), (b2, n2)):
            cc, v = _ln_stats(xx)
            xn_sc[b, :] = jnp.where(layer == 0, cc * lax.rsqrt(v + EPS), xx).astype(bf16)

        @pl.when(layer == 1)
        def _():
            c1 = pltpu.make_async_copy(xn_sc.at[b1, :], out_hbm.at[b1, :], sems.at[9])
            c1.start()

            @pl.when(jnp.logical_not(same))
            def _():
                c2 = pltpu.make_async_copy(xn_sc.at[b2, :], out_hbm.at[b2, :], sems.at[10])
                c2.start()
                c2.wait()
            c1.wait()

    def layer_body(layer, carry):
        lax.fori_loop(0, NRB, proj_body, 0)
        lax.fori_loop(0, G // NGB, attn_body, 0)

        @pl.when(layer == 0)
        def _():
            cp["wo"].wait()
            cp["wr"].wait()
            out_phase(False)
            cp["wg"].wait()
            cp["wu"].wait()
            cp["wd"].wait()

        @pl.when(layer == 1)
        def _():
            out_phase(True)

        ffn(layer)
        return carry

    lax.fori_loop(0, 2, layer_body, 0)


@jax.jit
def pallas_interleave_layers__memory_aug_infini_attn__moe_arch_mod__prompt_kernel(
    A_x: jax.Array,
    A_wq: jax.Array,
    A_wk: jax.Array,
    A_wv: jax.Array,
    A_wo: jax.Array,
    A_beta: jax.Array,
    B_x: jax.Array,
    B_w_r: jax.Array,
    B_w_gate: jax.Array,
    B_w_up: jax.Array,
    B_w_down: jax.Array,
):
    del B_x
    x = A_x.reshape(S, D)
    zero = jnp.zeros((1,), jnp.int32)
    beta = A_beta.astype(f32)
    wr = B_w_r.reshape(1, D)
    any_spec = pl.BlockSpec(memory_space=pl.ANY)
    smem_spec = pl.BlockSpec(memory_space=pltpu.SMEM)
    V = pltpu.VMEM
    scratch = [
        V((S, D), f32),
        V((S, D), f32),
        V((S, D), bf16),
        V((S, D), bf16),
        V((S, 128), f32),
        V((16, 128), f32), V((16, 128), jnp.int32),
        V((D, D), bf16), V((D, D), bf16), V((D, D), bf16), V((D, D), bf16),
        V((D, D), bf16), V((D, D), bf16),
        V((1, D), bf16),
        V((D, F), bf16), V((D, F), bf16), V((F, D), bf16),
        V((G, S, 128), bf16), V((G, S, 128), bf16),
        V((NRB, G, 128, RB), bf16), V((NRB, G, 128, RB), bf16), V((NRB, G, 128, RB), bf16),
        V((G, S, 128), bf16),
        V((NRB, G, 8, 128), f32),
        V((H, 8, 128), f32),
        V((128, 512), f32),
        pltpu.SemaphoreType.DMA((11,)),
        pltpu.SemaphoreType.DMA((NOB,)),
    ] + [V((T, 512), f32)] * NSLOT + [V((OS, D), f32)] * (OB // OS)
    out = pl.pallas_call(
        _kernel,
        in_specs=[smem_spec, smem_spec] + [any_spec] * 9,
        out_specs=any_spec,
        out_shape=jax.ShapeDtypeStruct((S, D), bf16),
        scratch_shapes=scratch,
        compiler_params=pltpu.CompilerParams(vmem_limit_bytes=120 * 1024 * 1024),
    )(zero, beta, x, A_wq, A_wk, A_wv, A_wo, wr, B_w_gate, B_w_up, B_w_down)
    return out.reshape(1, S, D)
```

```python
import functools

import jax
import jax.numpy as jnp
from jax import lax
import jax.experimental.pallas as pl
import jax.experimental.pallas.tpu as pltpu

S, D, H, DH, NSEG, L, F = 2048, 1024, 32, 32, 4, 512, 3584
HD = D // 2
G = 8
RB = 256
NRB = S // RB
OB = 1024
OS = 256
NOB = S // OB
FC = 256
PLAG = 1
TIE = True
T = 128
NGB = 1
LAGQ = 4
LAGP = 1
NSLOT = LAGQ + 1
EPS = 1e-05
LOG2E = 1.4426950408889634
QSCALE = (DH ** -0.5) * LOG2E
NEG = -1e30
NT = (((1,), (1,)), ((), ()))

f32 = jnp.float32
bf16 = jnp.bfloat16
u32 = jnp.uint32


def _phi(t):
    return jnp.where(t > 0, t + 1.0, jnp.exp(t))


def _sigmoid(t):
    return 1.0 / (1.0 + jnp.exp(-t))


def _pk(x):
    return pltpu.bitcast(x, u32)


def _upk(x):
    return pltpu.bitcast(x, bf16)


def _ln_stats(x):
    c = x - jnp.mean(x, axis=-1, keepdims=True)
    v = jnp.mean(c * c, axis=-1, keepdims=True)
    return c, v


def _row_fold(x, op):
    parts = [x[8 * r:8 * r + 8] for r in range(x.shape[0] // 8)]
    while len(parts) > 1:
        parts = [op(parts[i], parts[i + 1]) if i + 1 < len(parts) else parts[i] for i in range(0, len(parts), 2)]
    return parts[0]


def _lhs_operands(x):
    h = x.shape[0] // 2
    x00, x01, x10, x11 = x[:h, :HD], x[:h, HD:], x[h:, :HD], x[h:, HD:]
    a00, a01, a10, a11 = (t.astype(f32) for t in (x00, x01, x10, x11))
    return [(a00 + a11).astype(bf16), (a10 + a11).astype(bf16), x00, x11,
            (a00 + a01).astype(bf16), (a10 - a00).astype(bf16), (a01 - a11).astype(bf16)]


def _rhs_sums(t_ref, b11, b12, b21, b22):
    t_ref[0] = (b11() + b22()).astype(bf16)
    t_ref[1] = (b12() - b22()).astype(bf16)
    t_ref[2] = (b21() - b11()).astype(bf16)
    t_ref[3] = (b11() + b12()).astype(bf16)
    t_ref[4] = (b21() + b22()).astype(bf16)


def _strassen(mm):
    M = {}
    for i in (2, 3, 4, 0, 1, 6, 5):
        M[i] = mm(i)
    m1, m2, m3, m4, m5, m6, m7 = (M[i] for i in range(7))
    return (m1 + m4 - m5 + m7, m3 + m5, m2 + m4, m1 - m2 + m3 + m6), M


def _kernel(zero_smem, beta_smem, x_hbm, wq_hbm, wk_hbm, wv_hbm, wo_hbm, wr_hbm,
            wg_hbm, wu_hbm, wd_hbm, out_hbm,
            x_sc, x2_sc, xb_sc, xn_sc, rs_sc, cv_sc, ci_sc, tk_sc, tq_sc, tv_sc, to_sc, wq_sc, wk_sc, wv_sc, wo_sc, wqT_sc, wvT_sc, wr_sc,
            wg_sc, wu_sc, wd_sc, k_sc, pk_sc, qT_sc, pqT_sc, vT_sc, o_sc, z_sc,
            gt_sc, am_sc, sems, osems, *rest):
    s_sc, x1_sc = rest[:NSLOT], rest[NSLOT:]
    cp = {
        "wq": pltpu.make_async_copy(wq_hbm, wq_sc, sems.at[0]),
        "wv": pltpu.make_async_copy(wv_hbm, wv_sc, sems.at[1]),
        "x": pltpu.make_async_copy(x_hbm, xb_sc, sems.at[2]),
        "wk": pltpu.make_async_copy(wk_hbm, wk_sc, sems.at[3]),
        "wo": pltpu.make_async_copy(wo_hbm, wo_sc, sems.at[4]),
        "wr": pltpu.make_async_copy(wr_hbm, wr_sc, sems.at[5]),
        "wg": pltpu.make_async_copy(wg_hbm, wg_sc, sems.at[6]),
        "wu": pltpu.make_async_copy(wu_hbm, wu_sc, sems.at[7]),
        "wd": pltpu.make_async_copy(wd_hbm, wd_sc, sems.at[8]),
    }
    for c in cp.values():
        c.start()
    zero = zero_smem[0]

    def rows_of(rb):
        return pl.ds(pl.multiple_of(rb * RB, RB), RB)

    def out_copy(i):
        rows = pl.ds(pl.multiple_of(i * OB, OB), OB)
        return pltpu.make_async_copy(xn_sc.at[rows, :], out_hbm.at[rows, :], osems.at[i])

    def gate_body(h, carry):
        gt_sc[h] = _sigmoid(jnp.full((8, 128), beta_smem[h], f32))
        return carry
    lax.fori_loop(0, H, gate_body, 0)

    cp["wq"].wait()
    for j in range(4):
        for i in range(4):
            wqT_sc[256 * j:256 * (j + 1), 256 * i:256 * (i + 1)] = wq_sc[256 * i:256 * (i + 1), 256 * j:256 * (j + 1)].T
    cp["wv"].wait()
    for j in range(4):
        for i in range(4):
            wvT_sc[256 * j:256 * (j + 1), 256 * i:256 * (i + 1)] = wv_sc[256 * i:256 * (i + 1), 256 * j:256 * (j + 1)].T

    lo, hi = slice(0, HD), slice(HD, D)

    def quad(ref, r, c):
        return lambda: ref[r, c].astype(f32)

    def nat_ops(w_ref, t_ref):
        return [t_ref[0], w_ref[lo, lo], t_ref[1], t_ref[2], w_ref[hi, hi], t_ref[3], t_ref[4]]

    def tr_ops(w_ref, t_ref):
        return [t_ref[0], w_ref[lo, lo], t_ref[1], t_ref[2], w_ref[hi, hi], t_ref[3], t_ref[4]]

    _rhs_sums(tq_sc, quad(wqT_sc, lo, lo), quad(wqT_sc, hi, lo), quad(wqT_sc, lo, hi), quad(wqT_sc, hi, hi))
    _rhs_sums(tv_sc, quad(wvT_sc, lo, lo), quad(wvT_sc, hi, lo), quad(wvT_sc, lo, hi), quad(wvT_sc, hi, hi))

    cp["x"].wait()

    def ln0_body(rb, carry):
        rows = rows_of(rb)
        x = xb_sc[rows, :].astype(f32)
        c, v = _ln_stats(x)
        xn_sc[rows, :] = (c * lax.rsqrt(v + EPS)).astype(bf16)
        return carry
    lax.fori_loop(0, NRB, ln0_body, 0)
    cp["wk"].wait()
    _rhs_sums(tk_sc, quad(wk_sc, lo, lo), quad(wk_sc, lo, hi), quad(wk_sc, hi, lo), quad(wk_sc, hi, hi))

    row = lax.broadcasted_iota(jnp.int32, (T, T), 0)
    col = lax.broadcasted_iota(jnp.int32, (T, T), 1)
    cmask = row <= col
    hmask = (row // 32) == (col // 32)
    zrow = lax.broadcasted_iota(jnp.int32, (32, T), 0)
    zcol = lax.broadcasted_iota(jnp.int32, (32, T), 1)
    zmask = (zrow // 8) == (zcol // 32)

    def proj_body(rb, carry):
        h = RB // 2
        r0 = pl.multiple_of(rb * RB, RB)
        A = _lhs_operands(xn_sc[pl.ds(r0, RB), :])
        Wk = nat_ops(wk_sc, tk_sc)
        (c11, c12, c21, c22), _ = _strassen(lambda i: jnp.dot(A[i], Wk[i], preferred_element_type=f32))
        zp = [None, None]
        for c, th, nh in ((c12, 0, 1), (c21, 1, 0), (c11, 0, 0), (c22, 1, 1)):
            pk = _phi(c)
            zz = _row_fold(pk, jnp.add)
            zp[nh] = zz if zp[nh] is None else zp[nh] + zz
            rows = pl.ds(r0 + th * h, h)
            for g in range(G // 2):
                k_sc[4 * nh + g, rows, :] = c[:, 128 * g:128 * (g + 1)].astype(bf16)
                pk_sc[4 * nh + g, rows, :] = pk[:, 128 * g:128 * (g + 1)].astype(bf16)
        for nh in range(2):
            for g in range(G // 2):
                z_sc[rb, 4 * nh + g] = zp[nh][:, 128 * g:128 * (g + 1)]
        Wq = tr_ops(wqT_sc, tq_sc)
        (c11, c12, c21, c22), _ = _strassen(lambda i: lax.dot_general(Wq[i], A[i], NT, preferred_element_type=f32))
        for c, th, nh in ((c12, 0, 1), (c21, 1, 0), (c11, 0, 0), (c22, 1, 1)):
            pq = _phi(c)
            for g in range(G // 2):
                qT_sc[rb, 4 * nh + g, :, th * h:(th + 1) * h] = (c[128 * g:128 * (g + 1)] * QSCALE).astype(bf16)
                pqT_sc[rb, 4 * nh + g, :, th * h:(th + 1) * h] = pq[128 * g:128 * (g + 1)].astype(bf16)
        Wv = tr_ops(wvT_sc, tv_sc)
        (c11, c12, c21, c22), _ = _strassen(lambda i: lax.dot_general(Wv[i], A[i], NT, preferred_element_type=f32))
        for c, th, nh in ((c12, 0, 1), (c21, 1, 0), (c11, 0, 0), (c22, 1, 1)):
            for g in range(G // 2):
                vT_sc[rb, 4 * nh + g, :, th * h:(th + 1) * h] = c[128 * g:128 * (g + 1)].astype(bf16)
        return carry

    def attn_body(gb, carry):
        tiles = [(gg, s, i) for gg in range(NGB) for s in range(NSEG) for i in (3, 2, 1, 0)]
        stream = [(t, c) for t, (gg, s, i) in enumerate(tiles) for c in range(i + 1)]
        n = len(stream)
        m, l, O, W, P, M = {}, {}, {}, {}, {}, {}

        def grp(gg):
            return gb * NGB + gg

        def sref(k, h):
            return s_sc[k % NSLOT].at[pl.ds(pl.multiple_of(zero, 8), T), T * h:T * (h + 1)]

        def mem_read(gg, s):
            g = grp(gg)
            zs = z_sc[0, g]
            for rb in range(1, 2 * s):
                zs = zs + z_sc[rb, g]
            zs = jnp.sum(zs, axis=0, keepdims=True)
            zrows = jnp.where(zmask, zs, 0.0).astype(bf16)
            mbd = jnp.where(hmask, M[gg], 0.0).astype(bf16)
            lhs = jnp.concatenate([mbd, zrows], axis=0)
            pq = jnp.concatenate([pqT_sc[2 * s, g], pqT_sc[2 * s + 1, g]], axis=1)
            nd = jnp.dot(lhs, pq, preferred_element_type=f32)
            for h in range(4):
                den = nd[128 + 8 * h:128 + 8 * h + 8] + 1e-06
                gd = jnp.concatenate([gt_sc[4 * g + h]] * 4, axis=1) / den
                am_sc[32 * h:32 * h + 32, :] = nd[32 * h:32 * h + 32] * jnp.concatenate([gd] * 4, axis=0)

        def mem_write(gg, s):
            g = grp(gg)
            vt = jnp.concatenate([vT_sc[2 * s, g], vT_sc[2 * s + 1, g]], axis=1)
            pk = pk_sc[g, s * L:(s + 1) * L, :]
            inc = jnp.dot(vt, pk, preferred_element_type=f32)
            M[gg] = inc if s == 0 else M[gg] + inc

        def qk(k):
            t, c = stream[k]
            gg, s, i = tiles[t]
            g = grp(gg)
            if c == 0:
                QT = qT_sc[2 * s + i // 2, g, :, (i % 2) * T:(i % 2 + 1) * T]
                z = jnp.zeros((32, T), bf16)
                W[t] = jnp.concatenate(
                    [jnp.concatenate([QT[32 * h:32 * h + 32] if hh == h else z for hh in range(4)], axis=0)
                     for h in range(4)], axis=1)
                m[t] = [None] * 4
            k0 = s * L + c * T
            K = k_sc[g, k0:k0 + T, :]
            S4 = jnp.dot(K, W[t], preferred_element_type=f32)
            for h in range(4):
                Sx = S4[:, T * h:T * (h + 1)]
                if c == i:
                    Sx = jnp.where(cmask, Sx, NEG)
                sref(k, h)[...] = Sx
                mm = Sx[0:8]
                for r in range(1, 16):
                    mm = jnp.maximum(mm, Sx[8 * r:8 * r + 8])
                m[t][h] = mm if m[t][h] is None else jnp.maximum(m[t][h], mm)
            if c == i:
                m[t] = [jnp.max(x, axis=0, keepdims=True) for x in m[t]]

        def ex(k):
            t, c = stream[k]
            if c == 0:
                l[t] = [None] * 4
            out = []
            for h in range(4):
                Pp = jnp.exp2(sref(k, h)[...] - m[t][h])
                a = Pp[0:8] + Pp[8:16]
                b = Pp[16:24] + Pp[24:32]
                for r in range(2, 8, 2):
                    a = a + (Pp[16 * r:16 * r + 8] + Pp[16 * r + 8:16 * r + 16])
                    b = b + (Pp[16 * r + 16:16 * r + 24] + Pp[16 * r + 24:16 * r + 32])
                ll = a + b
                l[t][h] = ll if l[t][h] is None else l[t][h] + ll
                out.append(Pp.astype(bf16))
            P[k] = out

        def pv(k):
            t, c = stream[k]
            gg, s, i = tiles[t]
            g = grp(gg)
            if c == 0:
                O[t] = [None] * 4
            for h in range(4):
                vt = vT_sc[2 * s + c // 2, g, 32 * h:32 * h + 32, (c % 2) * T:(c % 2 + 1) * T]
                o = jnp.dot(vt, P[k][h], preferred_element_type=f32)
                O[t][h] = o if O[t][h] is None else O[t][h] + o
            del P[k]
            if c == i:
                outs = []
                for h in range(4):
                    lt = jnp.sum(l[t][h], axis=0, keepdims=True)
                    gt = jnp.concatenate([gt_sc[4 * g + h]] * 4, axis=0)
                    o = O[t][h] * ((1.0 - gt) * (1.0 / lt))
                    if s > 0:
                        o = o + am_sc[32 * h:32 * h + 32, i * T:(i + 1) * T]
                    outs.append(o)
                ot = jnp.concatenate(outs, axis=0).astype(bf16)
                r0 = s * L + i * T
                o_sc[g, r0:r0 + T, :] = ot.T
                del l[t], O[t], m[t], W[t]
                if i == 3 and s < NSEG - 1:
                    mem_write(gg, s)
                if i == 0 and s < NSEG - 1:
                    mem_read(gg, s + 1)

        for pos in range(n + LAGQ + LAGP):
            if pos < n:
                qk(pos)
            if 0 <= pos - LAGQ - LAGP < n:
                pv(pos - LAGQ - LAGP)
            if 0 <= pos - LAGQ < n:
                ex(pos - LAGQ)
        return carry

    def out_body(last, ob_i, top):
        base = pl.multiple_of(ob_i * OB, OB)
        wr = wr_sc[...].astype(f32)
        wr_sum = jnp.sum(wr, axis=-1, keepdims=True)
        NK = OB // OS
        CH = OS // (D // 128)
        never = jnp.full((CH, 1), zero, jnp.int32) != 0
        src = x_sc if last else xb_sc
        dst = x2_sc if last else x_sc

        def proj_stats(k):
            r0 = base + k * OS
            h = OS // 2
            ob = jnp.concatenate([o_sc[g, pl.ds(r0, OS), :] for g in range(G)], axis=1)
            A = _lhs_operands(ob)
            Wo = nat_ops(wo_sc, to_sc)
            (c11, c12, c21, c22), M = _strassen(lambda i: jnp.dot(A[i], Wo[i], preferred_element_type=f32))
            acc = [[None] * 3, [None] * 3]
            for c, th, nh in ((c12, 0, 1), (c21, 1, 0), (c11, 0, 0), (c22, 1, 1)):
                cols = slice(nh * HD, (nh + 1) * HD)
                x1 = src[pl.ds(r0 + th * h, h), cols].astype(f32) + c
                x1_sc[k][th * h:(th + 1) * h, cols] = x1
                s1, s2, st = acc[th]
                for n in range(HD // 128):
                    d = x1[:, 128 * n:128 * (n + 1)]
                    s1 = d if s1 is None else s1 + d
                    s2 = d * d if s2 is None else s2 + d * d
                    t = d * wr[:, nh * HD + 128 * n:nh * HD + 128 * (n + 1)]
                    st = t if st is None else st + t
                acc[th] = [s1, s2, st]
            s1, s2, st = (jnp.concatenate([acc[0][i], acc[1][i]], axis=0) for i in range(3))
            mean = jnp.sum(s1, axis=-1, keepdims=True) * (1.0 / D)
            v = jnp.maximum(jnp.sum(s2, axis=-1, keepdims=True) * (1.0 / D) - mean * mean, 0.0)
            rs = lax.rsqrt(v + EPS)
            r = rs * (jnp.sum(st, axis=-1, keepdims=True) - mean * wr_sum)
            r = r.astype(bf16).astype(f32)
            rs_sc[pl.ds(r0, OS), :] = jnp.broadcast_to(rs, (OS, 128))
            toks = [None] + [M[i][0:CH, 0:1] for i in (2, 3, 4, 0, 1, 6, 5)]
            return mean, v, rs, r, toks

        def apply(k, mean, v, rs, toks):
            for n in range(D // 128):
                rows = pl.ds(base + k * OS + n * CH, CH)
                sl = slice(n * CH, (n + 1) * CH)
                mn, vn, rn = mean[sl], v[sl], rs[sl]
                if toks is not None and toks[n] is not None:
                    mn = jnp.where(never, toks[n], mn)
                xr = x1_sc[k][pl.ds(pl.multiple_of(zero + n * CH, 8), CH), :]
                c = xr - mn
                x2 = xr + c * rn
                dst[rows, :] = x2
                if last:
                    xn_sc[rows, :] = x2.astype(bf16)
                else:
                    a = 1.0 + rn
                    xn_sc[rows, :] = (c * (a * lax.rsqrt(vn * (a * a) + EPS))).astype(bf16)

        def route(k, r, top):
            m1, i1, m2, i2 = top
            sub = lax.broadcasted_iota(jnp.int32, (8, 1), 0) + (base + k * OS)
            for j in range(OS // 8):
                rj = r[8 * j:8 * j + 8]
                idx = sub + 8 * j
                g1 = rj > m1
                g2 = rj > m2
                m2 = jnp.where(g1, m1, jnp.where(g2, rj, m2))
                i2 = jnp.where(g1, i1, jnp.where(g2, idx, i2))
                m1 = jnp.where(g1, rj, m1)
                i1 = jnp.where(g1, idx, i1)
            return m1, i1, m2, i2

        st_ = {}
        for k in range(NK + PLAG):
            if k < NK:
                st_[k] = proj_stats(k)
            if k - PLAG >= 0:
                mean, v, rs, r, _ = st_[k - PLAG]
                apply(k - PLAG, mean, v, rs, st_[k - PLAG + 1][4] if (TIE and k - PLAG + 1 < NK) else None)
                top = route(k - PLAG, r, top)
        m1, i1, m2, i2 = top
        if last:
            out_copy(ob_i).start()
        return m1, i1, m2, i2

    def out_phase(last):
        top = (jnp.full((8, 1), -jnp.inf, f32), jnp.zeros((8, 1), jnp.int32),
               jnp.full((8, 1), -jnp.inf, f32), jnp.ones((8, 1), jnp.int32))
        m1, i1, m2, i2 = lax.fori_loop(0, NOB, functools.partial(out_body, last), top)
        cv_sc[0:8, :] = jnp.broadcast_to(m1, (8, 128))
        cv_sc[8:16, :] = jnp.broadcast_to(m2, (8, 128))
        ci_sc[0:8, :] = jnp.broadcast_to(i1, (8, 128))
        ci_sc[8:16, :] = jnp.broadcast_to(i2, (8, 128))

    def ffn(layer):
        cv = cv_sc[...]
        ci = ci_sc[...]
        v1 = jnp.max(cv, axis=0, keepdims=True)
        j1 = jnp.min(jnp.where(cv == v1, ci, S), axis=0, keepdims=True)
        cv2 = jnp.where(ci == j1, -jnp.inf, cv)
        v2 = jnp.max(cv2, axis=0, keepdims=True)
        j2 = jnp.min(jnp.where(cv2 == v2, ci, S), axis=0, keepdims=True)
        t1 = jnp.clip(j1[0, 0], 0, S - 1)
        t2 = jnp.clip(j2[0, 0], 0, S - 1)
        b1 = pl.ds(pl.multiple_of((t1 // 8) * 8, 8), 8)
        b2 = pl.ds(pl.multiple_of((t2 // 8) * 8, 8), 8)
        xr = jnp.where(layer == 0, jnp.concatenate([x_sc[b1, :], x_sc[b2, :]], axis=0),
                       jnp.concatenate([x2_sc[b1, :], x2_sc[b2, :]], axis=0))
        rs = jnp.concatenate([rs_sc[b1, :], rs_sc[b2, :]], axis=0)[:, 0:1]
        c = xr - jnp.mean(xr, axis=-1, keepdims=True)
        xm = c * (rs / (1.0 + rs))
        xs = xm.astype(bf16)
        base = xr
        y = None
        for j in range(F // FC):
            gg = jnp.dot(xs, wg_sc[:, FC * j:FC * (j + 1)], preferred_element_type=f32)
            uu = jnp.dot(xs, wu_sc[:, FC * j:FC * (j + 1)], preferred_element_type=f32)
            hh = (gg * _sigmoid(gg) * uu).astype(bf16)
            t = jnp.dot(hh, wd_sc[FC * j:FC * (j + 1), :], preferred_element_type=f32)
            y = t if y is None else y + t
        r8 = lax.broadcasted_iota(jnp.int32, (8, D), 0)
        y1 = jnp.where(r8 == t1 % 8, y[0:8] * jnp.concatenate([_sigmoid(v1)] * (D // 128), axis=1), 0.0)
        y2 = jnp.where(r8 == t2 % 8, y[8:16] * jnp.concatenate([_sigmoid(v2)] * (D // 128), axis=1), 0.0)
        same = t1 // 8 == t2 // 8
        n1 = base[0:8] + (y1 + jnp.where(same, y2, 0.0))
        n2 = base[8:16] + (y2 + jnp.where(same, y1, 0.0))
        x_sc[b1, :] = n1
        x_sc[b2, :] = n2

        @pl.when(layer == 1)
        def _():
            for i in range(NOB):
                out_copy(i).wait()

        for b, xx in ((b1, n1), (b2, n2)):
            cc, v = _ln_stats(xx)
            xn_sc[b, :] = jnp.where(layer == 0, cc * lax.rsqrt(v + EPS), xx).astype(bf16)

        @pl.when(layer == 1)
        def _():
            c1 = pltpu.make_async_copy(xn_sc.at[b1, :], out_hbm.at[b1, :], sems.at[9])
            c1.start()

            @pl.when(jnp.logical_not(same))
            def _():
                c2 = pltpu.make_async_copy(xn_sc.at[b2, :], out_hbm.at[b2, :], sems.at[10])
                c2.start()
                c2.wait()
            c1.wait()

    def layer_body(layer, carry):
        lax.fori_loop(0, NRB, proj_body, 0)
        lax.fori_loop(0, G // NGB, attn_body, 0)

        @pl.when(layer == 0)
        def _():
            cp["wo"].wait()
            _rhs_sums(to_sc, quad(wo_sc, lo, lo), quad(wo_sc, lo, hi), quad(wo_sc, hi, lo), quad(wo_sc, hi, hi))
            cp["wr"].wait()
            out_phase(False)
            cp["wg"].wait()
            cp["wu"].wait()
            cp["wd"].wait()

        @pl.when(layer == 1)
        def _():
            out_phase(True)

        ffn(layer)
        return carry

    lax.fori_loop(0, 2, layer_body, 0)


@jax.jit
def pallas_interleave_layers__memory_aug_infini_attn__moe_arch_mod__prompt_kernel(
    A_x: jax.Array,
    A_wq: jax.Array,
    A_wk: jax.Array,
    A_wv: jax.Array,
    A_wo: jax.Array,
    A_beta: jax.Array,
    B_x: jax.Array,
    B_w_r: jax.Array,
    B_w_gate: jax.Array,
    B_w_up: jax.Array,
    B_w_down: jax.Array,
):
    del B_x
    x = A_x.reshape(S, D)
    zero = jnp.zeros((1,), jnp.int32)
    beta = A_beta.astype(f32)
    wr = B_w_r.reshape(1, D)
    any_spec = pl.BlockSpec(memory_space=pl.ANY)
    smem_spec = pl.BlockSpec(memory_space=pltpu.SMEM)
    V = pltpu.VMEM
    scratch = [
        V((S, D), f32),
        V((S, D), f32),
        V((S, D), bf16),
        V((S, D), bf16),
        V((S, 128), f32),
        V((16, 128), f32), V((16, 128), jnp.int32),
        V((5, HD, HD), bf16), V((5, HD, HD), bf16), V((5, HD, HD), bf16), V((5, HD, HD), bf16),
        V((D, D), bf16), V((D, D), bf16), V((D, D), bf16), V((D, D), bf16),
        V((D, D), bf16), V((D, D), bf16),
        V((1, D), bf16),
        V((D, F), bf16), V((D, F), bf16), V((F, D), bf16),
        V((G, S, 128), bf16), V((G, S, 128), bf16),
        V((NRB, G, 128, RB), bf16), V((NRB, G, 128, RB), bf16), V((NRB, G, 128, RB), bf16),
        V((G, S, 128), bf16),
        V((NRB, G, 8, 128), f32),
        V((H, 8, 128), f32),
        V((128, 512), f32),
        pltpu.SemaphoreType.DMA((11,)),
        pltpu.SemaphoreType.DMA((NOB,)),
    ] + [V((T, 512), f32)] * NSLOT + [V((OS, D), f32)] * (OB // OS)
    out = pl.pallas_call(
        _kernel,
        in_specs=[smem_spec, smem_spec] + [any_spec] * 9,
        out_specs=any_spec,
        out_shape=jax.ShapeDtypeStruct((S, D), bf16),
        scratch_shapes=scratch,
        compiler_params=pltpu.CompilerParams(vmem_limit_bytes=120 * 1024 * 1024),
    )(zero, beta, x, A_wq, A_wk, A_wv, A_wo, wr, B_w_gate, B_w_up, B_w_down)
    return out.reshape(1, S, D)
```

```python
import functools

import jax
import jax.numpy as jnp
from jax import lax
import jax.experimental.pallas as pl
import jax.experimental.pallas.tpu as pltpu

S, D, H, DH, NSEG, L, F = 2048, 1024, 32, 32, 4, 512, 3584
HD = D // 2
G = 8
RB = 256
NRB = S // RB
OB = 1024
OS = 128
NOB = S // OB
FC = 256
PLAG = 1
TIE = True
ORDER4 = (2, 3, 4, 0, 1, 6, 5)
NWK = 4
T = 128
NGB = 1
LAGQ = 4
LAGP = 1
NSLOT = LAGQ + 1
EPS = 1e-05
LOG2E = 1.4426950408889634
QSCALE = (DH ** -0.5) * LOG2E
NEG = -1e30
NT = (((1,), (1,)), ((), ()))

f32 = jnp.float32
bf16 = jnp.bfloat16
u32 = jnp.uint32


def _phi(t):
    return jnp.where(t > 0, t + 1.0, jnp.exp(t))


def _sigmoid(t):
    return 1.0 / (1.0 + jnp.exp(-t))


def _pk(x):
    return pltpu.bitcast(x, u32)


def _upk(x):
    return pltpu.bitcast(x, bf16)


def _ln_stats(x):
    c = x - jnp.mean(x, axis=-1, keepdims=True)
    v = jnp.mean(c * c, axis=-1, keepdims=True)
    return c, v


def _row_fold(x, op):
    parts = [x[8 * r:8 * r + 8] for r in range(x.shape[0] // 8)]
    while len(parts) > 1:
        parts = [op(parts[i], parts[i + 1]) if i + 1 < len(parts) else parts[i] for i in range(0, len(parts), 2)]
    return parts[0]


def _lhs_operands(x, tie=None):
    h = x.shape[0] // 2
    x00, x01, x10, x11 = x[:h, :HD], x[:h, HD:], x[h:, :HD], x[h:, HD:]

    def comb(j, a, b, sign):
        if tie is not None:
            a = tie(j, a)
        a, b = a.astype(f32), b.astype(f32)
        return (a + b if sign > 0 else a - b).astype(bf16)
    return [comb(1, x00, x11, 1), comb(3, x10, x11, 1), x00, x11,
            comb(0, x00, x01, 1), comb(4, x10, x00, -1), comb(2, x01, x11, -1)]


def _sums_into(t_ref, rows, b11, b12, b21, b22):
    b11f, b12f, b21f, b22f = (t.astype(f32) for t in (b11, b12, b21, b22))
    ops = ((b11f + b22f).astype(bf16), b11, (b12f - b22f).astype(bf16), (b21f - b11f).astype(bf16),
           b22, (b11f + b12f).astype(bf16), (b21f + b22f).astype(bf16))
    for i, t in enumerate(ops):
        t_ref[i, rows, :] = _pk(t)


def _prep_nat(t_ref, w_ref, n, nch):
    ch = HD // nch
    lo_r = pl.ds(pl.multiple_of(n * ch, ch), ch)
    hi_r = pl.ds(pl.multiple_of(HD + n * ch, ch), ch)
    p_r = pl.ds(pl.multiple_of(n * (ch // 2), ch // 2), ch // 2)
    _sums_into(t_ref, p_r, w_ref[lo_r, :HD], w_ref[lo_r, HD:], w_ref[hi_r, :HD], w_ref[hi_r, HD:])


def _prep_tr(t_ref, w_ref, j, tie=None):
    c_lo = pl.ds(pl.multiple_of(j * 128, 128), 128)
    c_hi = pl.ds(pl.multiple_of(HD + j * 128, 128), 128)

    def blk(r, c):
        t = w_ref[r * HD:(r + 1) * HD, c].T
        return t if tie is None else tie(t)
    p_r = pl.ds(pl.multiple_of(j * 64, 64), 64)
    _sums_into(t_ref, p_r, blk(0, c_lo), blk(0, c_hi), blk(1, c_lo), blk(1, c_hi))


def _strassen(mm, order=(2, 3, 4, 0, 1, 6, 5)):
    M = {}
    for i in order:
        M[i] = mm(i)
    m1, m2, m3, m4, m5, m6, m7 = (M[i] for i in range(7))
    return (m1 + m4 - m5 + m7, m3 + m5, m2 + m4, m1 - m2 + m3 + m6), M


def _kernel(zero_smem, beta_smem, x_hbm, wq_hbm, wk_hbm, wv_hbm, wo_hbm, wr_hbm,
            wg_hbm, wu_hbm, wd_hbm, out_hbm,
            xb_sc, xn_sc, rs_sc, cv_sc, ci_sc, tk_sc, tq_sc, tv_sc, to_sc, wq_sc, wk_sc, wv_sc, wo_sc, wr_sc,
            wg_sc, wu_sc, wd_sc, k_sc, pk_sc, qT_sc, pqT_sc, vT_sc, o_sc, z_sc,
            gt_sc, am_sc, sems, osems, xsems, ksems, *rest):
    s_sc, x1_sc = rest[:NSLOT], rest[NSLOT:]
    cp = {
        "wq": pltpu.make_async_copy(wq_hbm, wq_sc, sems.at[0]),
        "wv": pltpu.make_async_copy(wv_hbm, wv_sc, sems.at[1]),
        "wo": pltpu.make_async_copy(wo_hbm, wo_sc, sems.at[4]),
        "wr": pltpu.make_async_copy(wr_hbm, wr_sc, sems.at[5]),
        "wg": pltpu.make_async_copy(wg_hbm, wg_sc, sems.at[6]),
        "wu": pltpu.make_async_copy(wu_hbm, wu_sc, sems.at[7]),
        "wd": pltpu.make_async_copy(wd_hbm, wd_sc, sems.at[8]),
    }

    def x_copy(rb):
        rows = pl.ds(pl.multiple_of(rb * RB, RB), RB)
        return pltpu.make_async_copy(x_hbm.at[rows, :], xb_sc.at[rows, :], xsems.at[rb])

    def wk_copy(n, half):
        rows = pl.ds(half * HD + n * (HD // NWK), HD // NWK)
        return pltpu.make_async_copy(wk_hbm.at[rows, :], wk_sc.at[rows, :], ksems.at[n, half])

    x_copy(0).start()
    for n in range(NWK):
        wk_copy(n, 0).start()
        wk_copy(n, 1).start()
    x_copy(1).start()
    zero = zero_smem[0]

    def rows_of(rb):
        return pl.ds(pl.multiple_of(rb * RB, RB), RB)

    def out_copy(i):
        rows = pl.ds(pl.multiple_of(i * OB, OB), OB)
        return pltpu.make_async_copy(xb_sc.at[rows, :], out_hbm.at[rows, :], osems.at[i])

    def gate_body(h, carry):
        gt_sc[h] = _sigmoid(jnp.full((8, 128), beta_smem[h], f32))
        return carry
    lax.fori_loop(0, H, gate_body, 0)

    row = lax.broadcasted_iota(jnp.int32, (T, T), 0)
    col = lax.broadcasted_iota(jnp.int32, (T, T), 1)
    cmask = row <= col
    hmask = (row // 32) == (col // 32)
    zrow = lax.broadcasted_iota(jnp.int32, (32, T), 0)
    zcol = lax.broadcasted_iota(jnp.int32, (32, T), 1)
    zmask = (zrow // 8) == (zcol // 32)

    def project_k(rb, A):
        h = RB // 2
        r0 = rb * RB if isinstance(rb, int) else pl.multiple_of(rb * RB, RB)
        (c11, c12, c21, c22), MK = _strassen(lambda i: jnp.dot(A[i], _upk(tk_sc[i]), preferred_element_type=f32))
        zp = [None, None]
        for c, th, nh in ((c12, 0, 1), (c21, 1, 0), (c11, 0, 0), (c22, 1, 1)):
            pk = _phi(c)
            zz = _row_fold(pk, jnp.add)
            zp[nh] = zz if zp[nh] is None else zp[nh] + zz
            rows = pl.ds(r0 + th * h, h)
            for g in range(G // 2):
                k_sc[4 * nh + g, rows, :] = c[:, 128 * g:128 * (g + 1)].astype(bf16)
                pk_sc[4 * nh + g, rows, :] = pk[:, 128 * g:128 * (g + 1)].astype(bf16)
        for nh in range(2):
            for g in range(G // 2):
                z_sc[rb, 4 * nh + g] = zp[nh][:, 128 * g:128 * (g + 1)]
        return MK

    def project_qv(rb, A):
        h = RB // 2
        (c11, c12, c21, c22), _ = _strassen(lambda i: lax.dot_general(_upk(tq_sc[i]), A[i], NT, preferred_element_type=f32))
        for c, th, nh in ((c12, 0, 1), (c21, 1, 0), (c11, 0, 0), (c22, 1, 1)):
            pq = _phi(c)
            for g in range(G // 2):
                qT_sc[rb, 4 * nh + g, :, th * h:(th + 1) * h] = (c[128 * g:128 * (g + 1)] * QSCALE).astype(bf16)
                pqT_sc[rb, 4 * nh + g, :, th * h:(th + 1) * h] = pq[128 * g:128 * (g + 1)].astype(bf16)
        (c11, c12, c21, c22), _ = _strassen(lambda i: lax.dot_general(_upk(tv_sc[i]), A[i], NT, preferred_element_type=f32))
        for c, th, nh in ((c12, 0, 1), (c21, 1, 0), (c11, 0, 0), (c22, 1, 1)):
            for g in range(G // 2):
                vT_sc[rb, 4 * nh + g, :, th * h:(th + 1) * h] = c[128 * g:128 * (g + 1)].astype(bf16)

    def ln_in(rb, toks):
        ch = RB // 8
        never = jnp.full((ch, 1), zero, jnp.int32) != 0
        outs = []
        for n in range(8):
            rows = pl.ds(pl.multiple_of(rb * RB + n * ch, ch), ch)
            x = xb_sc[rows, :].astype(f32)
            m = jnp.mean(x, axis=-1, keepdims=True)
            if toks is not None and toks[n] is not None:
                x = jnp.where(never, toks[n], x)
            c = x - m
            v = jnp.mean(c * c, axis=-1, keepdims=True)
            outs.append((c * lax.rsqrt(v + EPS)).astype(bf16))
        xn = jnp.concatenate(outs, axis=0)
        xn_sc[pl.ds(pl.multiple_of(rb * RB, RB), RB), :] = xn
        return xn

    def first_k_body(prep, rb, xn):
        nxt = jnp.minimum(rb + 1, NRB - 1)

        @pl.when(rb + 1 < NRB)
        def _():
            x_copy(rb + 1).wait()

        if not prep:
            for j, (xs, name) in enumerate((((2, 3, 4), "wq"), ((5, 6, 7), "wv"), ((), "wo"), ((), "wr"))):
                @pl.when(rb == j)
                def _():
                    for i in xs:
                        x_copy(i).start()
                    cp[name].start()
        MK = project_k(rb, _lhs_operands(xn))
        order = (2, 3, 4, 0, 1, 6, 5)
        xn = ln_in(nxt, [None] + [MK[i][0:RB // 8, 0:1] for i in order])
        if prep:
            never = jnp.full((128, 1), zero, jnp.int32) != 0
            j = rb - NRB // 2
            _prep_tr(tq_sc, wq_sc, j, lambda t: jnp.where(never, MK[3][0:128, 0:1].astype(bf16), t))
            _prep_tr(tv_sc, wv_sc, j, lambda t: jnp.where(never, MK[1][0:128, 0:1].astype(bf16), t))
        return xn

    def first_k_phase():
        x_copy(0).wait()
        xn = ln_in(0, None)
        for n in range(NWK):
            wk_copy(n, 0).wait()
            wk_copy(n, 1).wait()
            for m in range(8 // NWK):
                _prep_nat(tk_sc, wk_sc, n * (8 // NWK) + m, 8)
        xn = lax.fori_loop(0, NRB // 2, functools.partial(first_k_body, False), xn)
        cp["wq"].wait()
        cp["wv"].wait()
        lax.fori_loop(NRB // 2, NRB, functools.partial(first_k_body, True), xn)
        cp["wo"].wait()
        lax.fori_loop(0, 8, lambda n, c: (_prep_nat(to_sc, wo_sc, n, 8), c)[1], 0)

    def proj_qv_body(layer, rb, carry):
        @pl.when(jnp.logical_and(layer == 0, rb == 0))
        def _():
            for name in ("wg", "wu", "wd"):
                cp[name].start()
        project_qv(rb, _lhs_operands(xn_sc[pl.ds(pl.multiple_of(rb * RB, RB), RB), :]))
        return carry

    def proj_k_body(rb, carry):
        project_k(rb, _lhs_operands(xn_sc[pl.ds(pl.multiple_of(rb * RB, RB), RB), :]))
        return carry

    def attn_body(gb, carry):
        tiles = [(gg, s, i) for gg in range(NGB) for s in range(NSEG) for i in (3, 2, 1, 0)]
        stream = [(t, c) for t, (gg, s, i) in enumerate(tiles) for c in range(i + 1)]
        n = len(stream)
        m, l, O, W, P, M = {}, {}, {}, {}, {}, {}

        def grp(gg):
            return gb * NGB + gg

        def sref(k, h):
            return s_sc[k % NSLOT].at[pl.ds(pl.multiple_of(zero, 8), T), T * h:T * (h + 1)]

        def mem_read(gg, s):
            g = grp(gg)
            zs = z_sc[0, g]
            for rb in range(1, 2 * s):
                zs = zs + z_sc[rb, g]
            zs = jnp.sum(zs, axis=0, keepdims=True)
            zrows = jnp.where(zmask, zs, 0.0).astype(bf16)
            mbd = jnp.where(hmask, M[gg], 0.0).astype(bf16)
            lhs = jnp.concatenate([mbd, zrows], axis=0)
            pq = jnp.concatenate([pqT_sc[2 * s, g], pqT_sc[2 * s + 1, g]], axis=1)
            nd = jnp.dot(lhs, pq, preferred_element_type=f32)
            for h in range(4):
                den = nd[128 + 8 * h:128 + 8 * h + 8] + 1e-06
                gd = jnp.concatenate([gt_sc[4 * g + h]] * 4, axis=1) / den
                am_sc[32 * h:32 * h + 32, :] = nd[32 * h:32 * h + 32] * jnp.concatenate([gd] * 4, axis=0)

        def mem_write(gg, s):
            g = grp(gg)
            vt = jnp.concatenate([vT_sc[2 * s, g], vT_sc[2 * s + 1, g]], axis=1)
            pk = pk_sc[g, s * L:(s + 1) * L, :]
            inc = jnp.dot(vt, pk, preferred_element_type=f32)
            M[gg] = inc if s == 0 else M[gg] + inc

        def qk(k):
            t, c = stream[k]
            gg, s, i = tiles[t]
            g = grp(gg)
            if c == 0:
                QT = qT_sc[2 * s + i // 2, g, :, (i % 2) * T:(i % 2 + 1) * T]
                z = jnp.zeros((32, T), bf16)
                W[t] = jnp.concatenate(
                    [jnp.concatenate([QT[32 * h:32 * h + 32] if hh == h else z for hh in range(4)], axis=0)
                     for h in range(4)], axis=1)
                m[t] = [None] * 4
            k0 = s * L + c * T
            K = k_sc[g, k0:k0 + T, :]
            S4 = jnp.dot(K, W[t], preferred_element_type=f32)
            for h in range(4):
                Sx = S4[:, T * h:T * (h + 1)]
                if c == i:
                    Sx = jnp.where(cmask, Sx, NEG)
                sref(k, h)[...] = Sx
                mm = Sx[0:8]
                for r in range(1, 16):
                    mm = jnp.maximum(mm, Sx[8 * r:8 * r + 8])
                m[t][h] = mm if m[t][h] is None else jnp.maximum(m[t][h], mm)
            if c == i:
                m[t] = [jnp.max(x, axis=0, keepdims=True) for x in m[t]]

        def ex(k):
            t, c = stream[k]
            if c == 0:
                l[t] = [None] * 4
            out = []
            for h in range(4):
                Pp = jnp.exp2(sref(k, h)[...] - m[t][h])
                a = Pp[0:8] + Pp[8:16]
                b = Pp[16:24] + Pp[24:32]
                for r in range(2, 8, 2):
                    a = a + (Pp[16 * r:16 * r + 8] + Pp[16 * r + 8:16 * r + 16])
                    b = b + (Pp[16 * r + 16:16 * r + 24] + Pp[16 * r + 24:16 * r + 32])
                ll = a + b
                l[t][h] = ll if l[t][h] is None else l[t][h] + ll
                out.append(Pp.astype(bf16))
            P[k] = out

        def pv(k):
            t, c = stream[k]
            gg, s, i = tiles[t]
            g = grp(gg)
            if c == 0:
                O[t] = [None] * 4
            for h in range(4):
                vt = vT_sc[2 * s + c // 2, g, 32 * h:32 * h + 32, (c % 2) * T:(c % 2 + 1) * T]
                o = jnp.dot(vt, P[k][h], preferred_element_type=f32)
                O[t][h] = o if O[t][h] is None else O[t][h] + o
            del P[k]
            if c == i:
                outs = []
                for h in range(4):
                    lt = jnp.sum(l[t][h], axis=0, keepdims=True)
                    gt = jnp.concatenate([gt_sc[4 * g + h]] * 4, axis=0)
                    o = O[t][h] * ((1.0 - gt) * (1.0 / lt))
                    if s > 0:
                        o = o + am_sc[32 * h:32 * h + 32, i * T:(i + 1) * T]
                    outs.append(o)
                ot = jnp.concatenate(outs, axis=0).astype(bf16)
                r0 = s * L + i * T
                o_sc[g, r0:r0 + T, :] = ot.T
                del l[t], O[t], m[t], W[t]
                if i == 3 and s < NSEG - 1:
                    mem_write(gg, s)
                if i == 0 and s < NSEG - 1:
                    mem_read(gg, s + 1)

        for pos in range(n + LAGQ + LAGP):
            if pos < n:
                qk(pos)
            if 0 <= pos - LAGQ - LAGP < n:
                pv(pos - LAGQ - LAGP)
            if 0 <= pos - LAGQ < n:
                ex(pos - LAGQ)
        return carry

    def out_body(layer, ob_i, top):
        base = pl.multiple_of(ob_i * OB, OB)
        wr = wr_sc[...].astype(f32)
        wr_sum = jnp.sum(wr, axis=-1, keepdims=True)
        NK = OB // OS
        HR = OS // 2
        CH = OS // 8
        never = jnp.full((CH, 1), zero, jnp.int32) != 0
        order = ORDER4

        def proj_stats(k):
            r0 = base + k * OS
            ob = jnp.concatenate([o_sc[g, pl.ds(r0, OS), :] for g in range(G)], axis=1)
            A = _lhs_operands(ob)
            (c11, c12, c21, c22), M = _strassen(
                lambda i: jnp.dot(A[i], _upk(to_sc[i]), preferred_element_type=f32), order)
            acc = [[None] * 3, [None] * 3]
            for c, th, nh in ((c12, 0, 1), (c21, 1, 0), (c11, 0, 0), (c22, 1, 1)):
                cols = slice(nh * HD, (nh + 1) * HD)
                x1 = xb_sc[pl.ds(r0 + th * HR, HR), cols].astype(f32) + c
                x1_sc[k][th * HR:(th + 1) * HR, cols] = x1
                s1, s2, st = acc[th]
                for n in range(HD // 128):
                    d = x1[:, 128 * n:128 * (n + 1)]
                    s1 = d if s1 is None else s1 + d
                    s2 = d * d if s2 is None else s2 + d * d
                    t = d * wr[:, nh * HD + 128 * n:nh * HD + 128 * (n + 1)]
                    st = t if st is None else st + t
                acc[th] = [s1, s2, st]
            s1, s2, st = (jnp.concatenate([acc[0][i], acc[1][i]], axis=0) for i in range(3))
            mean = jnp.sum(s1, axis=-1, keepdims=True) * (1.0 / D)
            v = jnp.maximum(jnp.sum(s2, axis=-1, keepdims=True) * (1.0 / D) - mean * mean, 0.0)
            rs = lax.rsqrt(v + EPS)
            r = rs * (jnp.sum(st, axis=-1, keepdims=True) - mean * wr_sum)
            r = r.astype(bf16).astype(f32)
            rs_sc[pl.ds(r0, OS), :] = jnp.broadcast_to(rs, (OS, 128))
            return (mean, v, rs, r), [None] + [M[i][0:CH, 0:1] for i in order]

        def apply(k, mean, v, rs, toks):
            for n in range(OS // CH):
                rows = pl.ds(base + k * OS + n * CH, CH)
                sl = slice(n * CH, (n + 1) * CH)
                mn, vn, rn = mean[sl], v[sl], rs[sl]
                if toks is not None and toks[n] is not None:
                    mn = jnp.where(never, toks[n], mn)
                xr = x1_sc[k][pl.ds(pl.multiple_of(zero + n * CH, 8), CH), :]
                c = xr - mn
                x2 = xr + c * rn
                xb_sc[rows, :] = x2.astype(bf16)
                a = 1.0 + rn
                xn_sc[rows, :] = (c * (a * lax.rsqrt(vn * (a * a) + EPS))).astype(bf16)

        def route(k, r, top):
            m1, i1, m2, i2 = top
            sub = lax.broadcasted_iota(jnp.int32, (8, 1), 0) + (base + k * OS)
            for j in range(OS // 8):
                rj = r[8 * j:8 * j + 8]
                idx = sub + 8 * j
                g1 = rj > m1
                g2 = rj > m2
                m2 = jnp.where(g1, m1, jnp.where(g2, rj, m2))
                i2 = jnp.where(g1, i1, jnp.where(g2, idx, i2))
                m1 = jnp.where(g1, rj, m1)
                i1 = jnp.where(g1, idx, i1)
            return m1, i1, m2, i2

        st_, tk_ = {}, {}
        for k in range(NK + 1):
            if k < NK:
                st_[k], tk_[k] = proj_stats(k)
            if k >= 1:
                apply(k - 1, *st_[k - 1][:3], tk_[k] if k < NK else None)
                top = route(k - 1, st_[k - 1][3], top)
        m1, i1, m2, i2 = top

        @pl.when(layer == 1)
        def _():
            out_copy(ob_i).start()
        return m1, i1, m2, i2

    def out_phase(layer):
        top = (jnp.full((8, 1), -jnp.inf, f32), jnp.zeros((8, 1), jnp.int32),
               jnp.full((8, 1), -jnp.inf, f32), jnp.ones((8, 1), jnp.int32))
        m1, i1, m2, i2 = lax.fori_loop(0, NOB, functools.partial(out_body, layer), top)
        cv_sc[0:8, :] = jnp.broadcast_to(m1, (8, 128))
        cv_sc[8:16, :] = jnp.broadcast_to(m2, (8, 128))
        ci_sc[0:8, :] = jnp.broadcast_to(i1, (8, 128))
        ci_sc[8:16, :] = jnp.broadcast_to(i2, (8, 128))

    def ffn(layer):
        cv = cv_sc[...]
        ci = ci_sc[...]
        v1 = jnp.max(cv, axis=0, keepdims=True)
        j1 = jnp.min(jnp.where(cv == v1, ci, S), axis=0, keepdims=True)
        cv2 = jnp.where(ci == j1, -jnp.inf, cv)
        v2 = jnp.max(cv2, axis=0, keepdims=True)
        j2 = jnp.min(jnp.where(cv2 == v2, ci, S), axis=0, keepdims=True)
        t1 = jnp.clip(j1[0, 0], 0, S - 1)
        t2 = jnp.clip(j2[0, 0], 0, S - 1)
        b1 = pl.ds(pl.multiple_of((t1 // 8) * 8, 8), 8)
        b2 = pl.ds(pl.multiple_of((t2 // 8) * 8, 8), 8)
        xr = jnp.concatenate([xb_sc[b1, :], xb_sc[b2, :]], axis=0).astype(f32)
        rs = jnp.concatenate([rs_sc[b1, :], rs_sc[b2, :]], axis=0)[:, 0:1]
        c = xr - jnp.mean(xr, axis=-1, keepdims=True)
        xm = c * (rs / (1.0 + rs))
        xs = xm.astype(bf16)
        base = xr
        y = None
        for j in range(F // FC):
            gg = jnp.dot(xs, wg_sc[:, FC * j:FC * (j + 1)], preferred_element_type=f32)
            uu = jnp.dot(xs, wu_sc[:, FC * j:FC * (j + 1)], preferred_element_type=f32)
            hh = (gg * _sigmoid(gg) * uu).astype(bf16)
            t = jnp.dot(hh, wd_sc[FC * j:FC * (j + 1), :], preferred_element_type=f32)
            y = t if y is None else y + t
        r8 = lax.broadcasted_iota(jnp.int32, (8, D), 0)
        y1 = jnp.where(r8 == t1 % 8, y[0:8] * jnp.concatenate([_sigmoid(v1)] * (D // 128), axis=1), 0.0)
        y2 = jnp.where(r8 == t2 % 8, y[8:16] * jnp.concatenate([_sigmoid(v2)] * (D // 128), axis=1), 0.0)
        same = t1 // 8 == t2 // 8
        n1 = base[0:8] + (y1 + jnp.where(same, y2, 0.0))
        n2 = base[8:16] + (y2 + jnp.where(same, y1, 0.0))
        @pl.when(layer == 1)
        def _():
            for i in range(NOB):
                out_copy(i).wait()

        for b, xx in ((b1, n1), (b2, n2)):
            cc, v = _ln_stats(xx)
            xb_sc[b, :] = xx.astype(bf16)
            xn_sc[b, :] = (cc * lax.rsqrt(v + EPS)).astype(bf16)

        @pl.when(layer == 1)
        def _():
            c1 = pltpu.make_async_copy(xb_sc.at[b1, :], out_hbm.at[b1, :], sems.at[9])
            c1.start()

            @pl.when(jnp.logical_not(same))
            def _():
                c2 = pltpu.make_async_copy(xb_sc.at[b2, :], out_hbm.at[b2, :], sems.at[10])
                c2.start()
                c2.wait()
            c1.wait()

    def layer_body(layer, carry):
        @pl.when(layer == 1)
        def _():
            lax.fori_loop(0, NRB, proj_k_body, 0)
        lax.fori_loop(0, NRB, functools.partial(proj_qv_body, layer), 0)
        lax.fori_loop(0, G // NGB, attn_body, 0)

        @pl.when(layer == 0)
        def _():
            cp["wr"].wait()

        out_phase(layer)

        @pl.when(layer == 0)
        def _():
            cp["wg"].wait()
            cp["wu"].wait()
            cp["wd"].wait()
        ffn(layer)
        return carry

    first_k_phase()
    lax.fori_loop(0, 2, layer_body, 0)


@jax.jit
def pallas_interleave_layers__memory_aug_infini_attn__moe_arch_mod__prompt_kernel(
    A_x: jax.Array,
    A_wq: jax.Array,
    A_wk: jax.Array,
    A_wv: jax.Array,
    A_wo: jax.Array,
    A_beta: jax.Array,
    B_x: jax.Array,
    B_w_r: jax.Array,
    B_w_gate: jax.Array,
    B_w_up: jax.Array,
    B_w_down: jax.Array,
):
    del B_x
    x = A_x.reshape(S, D)
    zero = jnp.zeros((1,), jnp.int32)
    beta = A_beta.astype(f32)
    wr = B_w_r.reshape(1, D)
    any_spec = pl.BlockSpec(memory_space=pl.ANY)
    smem_spec = pl.BlockSpec(memory_space=pltpu.SMEM)
    V = pltpu.VMEM
    scratch = [
        V((S, D), bf16),
        V((S, D), bf16),
        V((S, 128), f32),
        V((16, 128), f32), V((16, 128), jnp.int32),
        V((7, HD // 2, HD), u32), V((7, HD // 2, HD), u32), V((7, HD // 2, HD), u32), V((7, HD // 2, HD), u32),
        V((D, D), bf16), V((D, D), bf16), V((D, D), bf16), V((D, D), bf16),
        V((1, D), bf16),
        V((D, F), bf16), V((D, F), bf16), V((F, D), bf16),
        V((G, S, 128), bf16), V((G, S, 128), bf16),
        V((NRB, G, 128, RB), bf16), V((NRB, G, 128, RB), bf16), V((NRB, G, 128, RB), bf16),
        V((G, S, 128), bf16),
        V((NRB, G, 8, 128), f32),
        V((H, 8, 128), f32),
        V((128, 512), f32),
        pltpu.SemaphoreType.DMA((11,)),
        pltpu.SemaphoreType.DMA((NOB,)),
        pltpu.SemaphoreType.DMA((NRB,)),
        pltpu.SemaphoreType.DMA((NWK, 2)),
    ] + [V((T, 512), f32)] * NSLOT + [V((OS, D), f32)] * (OB // OS)
    out = pl.pallas_call(
        _kernel,
        in_specs=[smem_spec, smem_spec] + [any_spec] * 9,
        out_specs=any_spec,
        out_shape=jax.ShapeDtypeStruct((S, D), bf16),
        scratch_shapes=scratch,
        compiler_params=pltpu.CompilerParams(vmem_limit_bytes=120 * 1024 * 1024),
    )(zero, beta, x, A_wq, A_wk, A_wv, A_wo, wr, B_w_gate, B_w_up, B_w_down)
    return out.reshape(1, S, D)
```

```python
import functools

import jax
import jax.numpy as jnp
from jax import lax
import jax.experimental.pallas as pl
import jax.experimental.pallas.tpu as pltpu

S, D, H, DH, NSEG, L, F = 2048, 1024, 32, 32, 4, 512, 3584
HD = D // 2
G = 8
RB = 256
NRB = S // RB
OB = 1024
OS = 128
NOB = S // OB
FC = 256
PLAG = 1
TIE = True
ORDER4 = (2, 3, 4, 0, 1, 6, 5)
NWK = 4
T = 128
LAG = 5
NSLOT = 5
EPS = 1e-05
LOG2E = 1.4426950408889634
QSCALE = (DH ** -0.5) * LOG2E
NEG = -1e30
NT = (((1,), (1,)), ((), ()))

f32 = jnp.float32
bf16 = jnp.bfloat16
u32 = jnp.uint32


def _phi(t):
    return jnp.where(t > 0, t + 1.0, jnp.exp(t))


def _sigmoid(t):
    return 1.0 / (1.0 + jnp.exp(-t))


def _pk(x):
    return pltpu.bitcast(x, u32)


def _upk(x):
    return pltpu.bitcast(x, bf16)


def _ln_stats(x):
    c = x - jnp.mean(x, axis=-1, keepdims=True)
    v = jnp.mean(c * c, axis=-1, keepdims=True)
    return c, v


def _row_fold(x, op):
    parts = [x[8 * r:8 * r + 8] for r in range(x.shape[0] // 8)]
    while len(parts) > 1:
        parts = [op(parts[i], parts[i + 1]) if i + 1 < len(parts) else parts[i] for i in range(0, len(parts), 2)]
    return parts[0]


def _lhs_operands(x, tie=None):
    h = x.shape[0] // 2
    x00, x01, x10, x11 = x[:h, :HD], x[:h, HD:], x[h:, :HD], x[h:, HD:]

    def comb(j, a, b, sign):
        if tie is not None:
            a = tie(j, a)
        a, b = a.astype(f32), b.astype(f32)
        return (a + b if sign > 0 else a - b).astype(bf16)
    return [comb(1, x00, x11, 1), comb(3, x10, x11, 1), x00, x11,
            comb(0, x00, x01, 1), comb(4, x10, x00, -1), comb(2, x01, x11, -1)]


def _sums_into(t_ref, rows, b11, b12, b21, b22):
    b11f, b12f, b21f, b22f = (t.astype(f32) for t in (b11, b12, b21, b22))
    ops = ((b11f + b22f).astype(bf16), b11, (b12f - b22f).astype(bf16), (b21f - b11f).astype(bf16),
           b22, (b11f + b12f).astype(bf16), (b21f + b22f).astype(bf16))
    for i, t in enumerate(ops):
        t_ref[i, rows, :] = _pk(t)


def _prep_nat(t_ref, w_ref, n, nch):
    ch = HD // nch
    lo_r = pl.ds(pl.multiple_of(n * ch, ch), ch)
    hi_r = pl.ds(pl.multiple_of(HD + n * ch, ch), ch)
    p_r = pl.ds(pl.multiple_of(n * (ch // 2), ch // 2), ch // 2)
    _sums_into(t_ref, p_r, w_ref[lo_r, :HD], w_ref[lo_r, HD:], w_ref[hi_r, :HD], w_ref[hi_r, HD:])


def _prep_tr(t_ref, w_ref, j, tie=None):
    c_lo = pl.ds(pl.multiple_of(j * 128, 128), 128)
    c_hi = pl.ds(pl.multiple_of(HD + j * 128, 128), 128)

    def blk(r, c):
        t = w_ref[r * HD:(r + 1) * HD, c].T
        return t if tie is None else tie(t)
    p_r = pl.ds(pl.multiple_of(j * 64, 64), 64)
    _sums_into(t_ref, p_r, blk(0, c_lo), blk(0, c_hi), blk(1, c_lo), blk(1, c_hi))


def _strassen(mm, order=(2, 3, 4, 0, 1, 6, 5)):
    M = {}
    for i in order:
        M[i] = mm(i)
    m1, m2, m3, m4, m5, m6, m7 = (M[i] for i in range(7))
    return (m1 + m4 - m5 + m7, m3 + m5, m2 + m4, m1 - m2 + m3 + m6), M


def _kernel(zero_smem, beta_smem, x_hbm, wq_hbm, wk_hbm, wv_hbm, wo_hbm, wr_hbm,
            wg_hbm, wu_hbm, wd_hbm, out_hbm,
            xb_sc, xn_sc, rs_sc, cv_sc, ci_sc, tk_sc, tq_sc, tv_sc, to_sc, wq_sc, wk_sc, wv_sc, wo_sc, wr_sc,
            wg_sc, wu_sc, wd_sc, k_sc, pk_sc, qT_sc, pqT_sc, vT_sc, o_sc, z_sc,
            gt_sc, am_sc, sems, osems, xsems, ksems, *rest):
    s_sc, x1_sc = rest[:NSLOT], rest[NSLOT:]
    cp = {
        "wq": pltpu.make_async_copy(wq_hbm, wq_sc, sems.at[0]),
        "wv": pltpu.make_async_copy(wv_hbm, wv_sc, sems.at[1]),
        "wo": pltpu.make_async_copy(wo_hbm, wo_sc, sems.at[4]),
        "wr": pltpu.make_async_copy(wr_hbm, wr_sc, sems.at[5]),
        "wg": pltpu.make_async_copy(wg_hbm, wg_sc, sems.at[6]),
        "wu": pltpu.make_async_copy(wu_hbm, wu_sc, sems.at[7]),
        "wd": pltpu.make_async_copy(wd_hbm, wd_sc, sems.at[8]),
    }

    def x_copy(rb):
        rows = pl.ds(pl.multiple_of(rb * RB, RB), RB)
        return pltpu.make_async_copy(x_hbm.at[rows, :], xb_sc.at[rows, :], xsems.at[rb])

    def wk_copy(n, half):
        rows = pl.ds(half * HD + n * (HD // NWK), HD // NWK)
        return pltpu.make_async_copy(wk_hbm.at[rows, :], wk_sc.at[rows, :], ksems.at[n, half])

    x_copy(0).start()
    for n in range(NWK):
        wk_copy(n, 0).start()
        wk_copy(n, 1).start()
    x_copy(1).start()
    zero = zero_smem[0]

    def rows_of(rb):
        return pl.ds(pl.multiple_of(rb * RB, RB), RB)

    def out_copy(i):
        rows = pl.ds(pl.multiple_of(i * OB, OB), OB)
        return pltpu.make_async_copy(xb_sc.at[rows, :], out_hbm.at[rows, :], osems.at[i])

    am_sc[...] = jnp.zeros((T, 4 * T), f32)

    def gate_body(h, carry):
        gt_sc[h] = _sigmoid(jnp.full((8, 128), beta_smem[h], f32))
        return carry
    lax.fori_loop(0, H, gate_body, 0)

    row = lax.broadcasted_iota(jnp.int32, (T, T), 0)
    col = lax.broadcasted_iota(jnp.int32, (T, T), 1)
    cmask = row <= col
    hmask = (row // 32) == (col // 32)
    zrow = lax.broadcasted_iota(jnp.int32, (32, T), 0)
    zcol = lax.broadcasted_iota(jnp.int32, (32, T), 1)
    zmask = (zrow // 8) == (zcol // 32)

    def project_k(rb, A):
        h = RB // 2
        r0 = rb * RB if isinstance(rb, int) else pl.multiple_of(rb * RB, RB)
        (c11, c12, c21, c22), MK = _strassen(lambda i: jnp.dot(A[i], _upk(tk_sc[i]), preferred_element_type=f32))
        zp = [None, None]
        for c, th, nh in ((c12, 0, 1), (c21, 1, 0), (c11, 0, 0), (c22, 1, 1)):
            pk = _phi(c)
            zz = _row_fold(pk, jnp.add)
            zp[nh] = zz if zp[nh] is None else zp[nh] + zz
            rows = pl.ds(r0 + th * h, h)
            for g in range(G // 2):
                k_sc[4 * nh + g, rows, :] = c[:, 128 * g:128 * (g + 1)].astype(bf16)
                pk_sc[4 * nh + g, rows, :] = pk[:, 128 * g:128 * (g + 1)].astype(bf16)
        for nh in range(2):
            for g in range(G // 2):
                z_sc[rb, 4 * nh + g] = zp[nh][:, 128 * g:128 * (g + 1)]
        return MK

    def project_qv(rb, A):
        h = RB // 2
        (c11, c12, c21, c22), _ = _strassen(lambda i: lax.dot_general(_upk(tq_sc[i]), A[i], NT, preferred_element_type=f32))
        for c, th, nh in ((c12, 0, 1), (c21, 1, 0), (c11, 0, 0), (c22, 1, 1)):
            pq = _phi(c)
            for g in range(G // 2):
                qT_sc[rb, 4 * nh + g, :, th * h:(th + 1) * h] = (c[128 * g:128 * (g + 1)] * QSCALE).astype(bf16)
                pqT_sc[rb, 4 * nh + g, :, th * h:(th + 1) * h] = pq[128 * g:128 * (g + 1)].astype(bf16)
        (c11, c12, c21, c22), _ = _strassen(lambda i: lax.dot_general(_upk(tv_sc[i]), A[i], NT, preferred_element_type=f32))
        for c, th, nh in ((c12, 0, 1), (c21, 1, 0), (c11, 0, 0), (c22, 1, 1)):
            for g in range(G // 2):
                vT_sc[rb, 4 * nh + g, :, th * h:(th + 1) * h] = c[128 * g:128 * (g + 1)].astype(bf16)

    def ln_in(rb, toks):
        ch = RB // 8
        never = jnp.full((ch, 1), zero, jnp.int32) != 0
        outs = []
        for n in range(8):
            rows = pl.ds(pl.multiple_of(rb * RB + n * ch, ch), ch)
            x = xb_sc[rows, :].astype(f32)
            m = jnp.mean(x, axis=-1, keepdims=True)
            if toks is not None and toks[n] is not None:
                x = jnp.where(never, toks[n], x)
            c = x - m
            v = jnp.mean(c * c, axis=-1, keepdims=True)
            outs.append((c * lax.rsqrt(v + EPS)).astype(bf16))
        xn = jnp.concatenate(outs, axis=0)
        xn_sc[pl.ds(pl.multiple_of(rb * RB, RB), RB), :] = xn
        return xn

    def first_k_body(prep, rb, xn):
        nxt = jnp.minimum(rb + 1, NRB - 1)

        @pl.when(rb + 1 < NRB)
        def _():
            x_copy(rb + 1).wait()

        if not prep:
            for j, (xs, name) in enumerate((((2, 3, 4), "wq"), ((5, 6, 7), "wv"), ((), "wo"), ((), "wr"))):
                @pl.when(rb == j)
                def _():
                    for i in xs:
                        x_copy(i).start()
                    cp[name].start()
        MK = project_k(rb, _lhs_operands(xn))
        order = (2, 3, 4, 0, 1, 6, 5)
        xn = ln_in(nxt, [None] + [MK[i][0:RB // 8, 0:1] for i in order])
        if prep:
            never = jnp.full((128, 1), zero, jnp.int32) != 0
            j = rb - NRB // 2
            _prep_tr(tq_sc, wq_sc, j, lambda t: jnp.where(never, MK[3][0:128, 0:1].astype(bf16), t))
            _prep_tr(tv_sc, wv_sc, j, lambda t: jnp.where(never, MK[1][0:128, 0:1].astype(bf16), t))
        return xn

    def first_k_phase():
        x_copy(0).wait()
        xn = ln_in(0, None)
        for n in range(NWK):
            wk_copy(n, 0).wait()
            wk_copy(n, 1).wait()
            for m in range(8 // NWK):
                _prep_nat(tk_sc, wk_sc, n * (8 // NWK) + m, 8)
        xn = lax.fori_loop(0, NRB // 2, functools.partial(first_k_body, False), xn)
        cp["wq"].wait()
        cp["wv"].wait()
        lax.fori_loop(NRB // 2, NRB, functools.partial(first_k_body, True), xn)
        cp["wo"].wait()
        lax.fori_loop(0, 8, lambda n, c: (_prep_nat(to_sc, wo_sc, n, 8), c)[1], 0)

    def proj_qv_body(layer, rb, carry):
        @pl.when(jnp.logical_and(layer == 0, rb == 0))
        def _():
            for name in ("wg", "wu", "wd"):
                cp[name].start()
        project_qv(rb, _lhs_operands(xn_sc[pl.ds(pl.multiple_of(rb * RB, RB), RB), :]))
        return carry

    def proj_k_body(rb, carry):
        project_k(rb, _lhs_operands(xn_sc[pl.ds(pl.multiple_of(rb * RB, RB), RB), :]))
        return carry

    TILES = [(s, i) for s in range(NSEG) for i in (3, 2, 1, 0)]
    STREAM = [(t, c) for t, (s, i) in enumerate(TILES) for c in range(i + 1)]
    NPOS = len(STREAM)

    def sref(k, h):
        return s_sc[k % NSLOT].at[pl.ds(pl.multiple_of(zero, 8), T), T * h:T * (h + 1)]

    def q_weights(g, s, i):
        QT = qT_sc[2 * s + i // 2, g, :, (i % 2) * T:(i % 2 + 1) * T]
        z = jnp.zeros((32, T), bf16)
        return jnp.concatenate(
            [jnp.concatenate([QT[32 * h:32 * h + 32] if hh == h else z for hh in range(4)], axis=0)
             for h in range(4)], axis=1)

    def qk(g, k, m):
        t, c = STREAM[k]
        s, i = TILES[t]
        k0 = s * L + c * T
        K = k_sc[g, k0:k0 + T, :]
        S4 = jnp.dot(K, q_weights(g, s, i), preferred_element_type=f32)
        out = []
        for h in range(4):
            Sx = S4[:, T * h:T * (h + 1)]
            if c == i:
                Sx = jnp.where(cmask, Sx, NEG)
            sref(k, h)[...] = Sx
            mm = Sx[0:8]
            for r in range(1, 16):
                mm = jnp.maximum(mm, Sx[8 * r:8 * r + 8])
            mm = mm if c == 0 else jnp.maximum(m[h], mm)
            if c == i:
                mm = jnp.broadcast_to(jnp.max(mm, axis=0, keepdims=True), (8, T))
            out.append(mm)
        return out

    def attn_prologue():
        m = {}
        for k in range(LAG):
            t = STREAM[k][0]
            m[t] = qk(0, k, m.get(t))
        return tuple(m[STREAM[0][0]]) + tuple(m[STREAM[LAG - 1][0]])

    def finish(g, s, i, O, l):
        outs = []
        for h in range(4):
            lt = jnp.sum(l[h], axis=0, keepdims=True)
            gt = jnp.concatenate([gt_sc[4 * g + h]] * 4, axis=0)
            o = O[h] * ((1.0 - gt) * (1.0 / lt))
            if s > 0:
                o = o + am_sc[32 * h:32 * h + 32, i * T:(i + 1) * T]
            outs.append(o)
        ot = jnp.concatenate(outs, axis=0).astype(bf16)
        r0 = s * L + i * T
        o_sc[g, r0:r0 + T, :] = ot.T

    def attn_body(g, carry):
        gn = jnp.minimum(g + 1, G - 1)
        m = {STREAM[0][0]: list(carry[0:4]), STREAM[LAG - 1][0]: list(carry[4:8])}
        l, O, P, M, mn = {}, {}, {}, {}, {}

        def mem_read(s):
            zs = z_sc[0, g]
            for rb in range(1, 2 * s):
                zs = zs + z_sc[rb, g]
            zs = jnp.sum(zs, axis=0, keepdims=True)
            zrows = jnp.where(zmask, zs, 0.0).astype(bf16)
            mbd = jnp.where(hmask, M[0], 0.0).astype(bf16)
            lhs = jnp.concatenate([mbd, zrows], axis=0)
            pq = jnp.concatenate([pqT_sc[2 * s, g], pqT_sc[2 * s + 1, g]], axis=1)
            nd = jnp.dot(lhs, pq, preferred_element_type=f32)
            for h in range(4):
                den = nd[128 + 8 * h:128 + 8 * h + 8] + 1e-06
                gd = jnp.concatenate([gt_sc[4 * g + h]] * 4, axis=1) / den
                am_sc[32 * h:32 * h + 32, :] = nd[32 * h:32 * h + 32] * jnp.concatenate([gd] * 4, axis=0)

        def mem_write(s):
            vt = jnp.concatenate([vT_sc[2 * s, g], vT_sc[2 * s + 1, g]], axis=1)
            pk = pk_sc[g, s * L:(s + 1) * L, :]
            inc = jnp.dot(vt, pk, preferred_element_type=f32)
            M[0] = inc if s == 0 else M[0] + inc

        def ex(k):
            t, c = STREAM[k]
            out = []
            for h in range(4):
                Pp = jnp.exp2(sref(k, h)[...] - jnp.concatenate([m[t][h]] * (T // 8), axis=0))
                a = Pp[0:8] + Pp[8:16]
                b = Pp[16:24] + Pp[24:32]
                for r in range(2, 8, 2):
                    a = a + (Pp[16 * r:16 * r + 8] + Pp[16 * r + 8:16 * r + 16])
                    b = b + (Pp[16 * r + 16:16 * r + 24] + Pp[16 * r + 24:16 * r + 32])
                ll = a + b
                if c == 0:
                    l.setdefault(t, [None] * 4)[h] = ll
                else:
                    l[t][h] = l[t][h] + ll
                out.append(Pp.astype(bf16))
            P[k] = out

        def pv(k):
            t, c = STREAM[k]
            s, i = TILES[t]
            if c == 0:
                O[t] = [None] * 4
            for h in range(4):
                vt = vT_sc[2 * s + c // 2, g, 32 * h:32 * h + 32, (c % 2) * T:(c % 2 + 1) * T]
                o = jnp.dot(vt, P[k][h], preferred_element_type=f32)
                O[t][h] = o if O[t][h] is None else O[t][h] + o
            del P[k]

        finish(jnp.maximum(g - 1, 0), NSEG - 1, 0, carry[8:12], carry[12:16])
        done = None
        for j in range(NPOS):
            ex(j)
            k = j + LAG
            if k < NPOS:
                t = STREAM[k][0]
                m[t] = qk(g, k, m.get(t))
            else:
                t = STREAM[k - NPOS][0]
                mn[t] = qk(gn, k - NPOS, mn.get(t))
            pv(j)
            if done is not None:
                s, i = TILES[done]
                finish(g, s, i, O[done], l[done])
                if i == 0:
                    mem_read(s + 1)
                done = None
            t, c = STREAM[j]
            if c == TILES[t][1]:
                done = t
                if TILES[t][1] == 3 and TILES[t][0] < NSEG - 1:
                    mem_write(TILES[t][0])
        return (tuple(mn[STREAM[0][0]]) + tuple(mn[STREAM[LAG - 1][0]]) + tuple(O[done]) + tuple(l[done]))

    def attn_phase():
        init = attn_prologue() + (jnp.zeros((32, T), f32),) * 4 + (jnp.ones((8, T), f32),) * 4
        carry = lax.fori_loop(0, G, attn_body, init)
        finish(G - 1, NSEG - 1, 0, carry[8:12], carry[12:16])

    def out_body(layer, ob_i, top):
        base = pl.multiple_of(ob_i * OB, OB)
        wr = wr_sc[...].astype(f32)
        wr_sum = jnp.sum(wr, axis=-1, keepdims=True)
        NK = OB // OS
        HR = OS // 2
        CH = OS // 8
        never = jnp.full((CH, 1), zero, jnp.int32) != 0
        order = ORDER4

        def proj_stats(k):
            r0 = base + k * OS
            ob = jnp.concatenate([o_sc[g, pl.ds(r0, OS), :] for g in range(G)], axis=1)
            A = _lhs_operands(ob)
            (c11, c12, c21, c22), M = _strassen(
                lambda i: jnp.dot(A[i], _upk(to_sc[i]), preferred_element_type=f32), order)
            acc = [[None] * 3, [None] * 3]
            for c, th, nh in ((c12, 0, 1), (c21, 1, 0), (c11, 0, 0), (c22, 1, 1)):
                cols = slice(nh * HD, (nh + 1) * HD)
                x1 = xb_sc[pl.ds(r0 + th * HR, HR), cols].astype(f32) + c
                x1_sc[k][th * HR:(th + 1) * HR, cols] = x1
                s1, s2, st = acc[th]
                for n in range(HD // 128):
                    d = x1[:, 128 * n:128 * (n + 1)]
                    s1 = d if s1 is None else s1 + d
                    s2 = d * d if s2 is None else s2 + d * d
                    t = d * wr[:, nh * HD + 128 * n:nh * HD + 128 * (n + 1)]
                    st = t if st is None else st + t
                acc[th] = [s1, s2, st]
            s1, s2, st = (jnp.concatenate([acc[0][i], acc[1][i]], axis=0) for i in range(3))
            mean = jnp.sum(s1, axis=-1, keepdims=True) * (1.0 / D)
            v = jnp.maximum(jnp.sum(s2, axis=-1, keepdims=True) * (1.0 / D) - mean * mean, 0.0)
            rs = lax.rsqrt(v + EPS)
            r = rs * (jnp.sum(st, axis=-1, keepdims=True) - mean * wr_sum)
            r = r.astype(bf16).astype(f32)
            rs_sc[pl.ds(r0, OS), :] = jnp.broadcast_to(rs, (OS, 128))
            return (mean, v, rs, r), [None] + [M[i][0:CH, 0:1] for i in order]

        def apply(k, mean, v, rs, toks):
            for n in range(OS // CH):
                rows = pl.ds(base + k * OS + n * CH, CH)
                sl = slice(n * CH, (n + 1) * CH)
                mn, vn, rn = mean[sl], v[sl], rs[sl]
                if toks is not None and toks[n] is not None:
                    mn = jnp.where(never, toks[n], mn)
                xr = x1_sc[k][pl.ds(pl.multiple_of(zero + n * CH, 8), CH), :]
                c = xr - mn
                x2 = xr + c * rn
                xb_sc[rows, :] = x2.astype(bf16)
                a = 1.0 + rn
                xn_sc[rows, :] = (c * (a * lax.rsqrt(vn * (a * a) + EPS))).astype(bf16)

        def route(k, r, top):
            m1, i1, m2, i2 = top
            sub = lax.broadcasted_iota(jnp.int32, (8, 1), 0) + (base + k * OS)
            for j in range(OS // 8):
                rj = r[8 * j:8 * j + 8]
                idx = sub + 8 * j
                g1 = rj > m1
                g2 = rj > m2
                m2 = jnp.where(g1, m1, jnp.where(g2, rj, m2))
                i2 = jnp.where(g1, i1, jnp.where(g2, idx, i2))
                m1 = jnp.where(g1, rj, m1)
                i1 = jnp.where(g1, idx, i1)
            return m1, i1, m2, i2

        st_, tk_ = {}, {}
        for k in range(NK + 1):
            if k < NK:
                st_[k], tk_[k] = proj_stats(k)
            if k >= 1:
                apply(k - 1, *st_[k - 1][:3], tk_[k] if k < NK else None)
                top = route(k - 1, st_[k - 1][3], top)
        m1, i1, m2, i2 = top

        @pl.when(layer == 1)
        def _():
            out_copy(ob_i).start()
        return m1, i1, m2, i2

    def out_phase(layer):
        top = (jnp.full((8, 1), -jnp.inf, f32), jnp.zeros((8, 1), jnp.int32),
               jnp.full((8, 1), -jnp.inf, f32), jnp.ones((8, 1), jnp.int32))
        m1, i1, m2, i2 = lax.fori_loop(0, NOB, functools.partial(out_body, layer), top)
        cv_sc[0:8, :] = jnp.broadcast_to(m1, (8, 128))
        cv_sc[8:16, :] = jnp.broadcast_to(m2, (8, 128))
        ci_sc[0:8, :] = jnp.broadcast_to(i1, (8, 128))
        ci_sc[8:16, :] = jnp.broadcast_to(i2, (8, 128))

    def ffn(layer):
        cv = cv_sc[...]
        ci = ci_sc[...]
        v1 = jnp.max(cv, axis=0, keepdims=True)
        j1 = jnp.min(jnp.where(cv == v1, ci, S), axis=0, keepdims=True)
        cv2 = jnp.where(ci == j1, -jnp.inf, cv)
        v2 = jnp.max(cv2, axis=0, keepdims=True)
        j2 = jnp.min(jnp.where(cv2 == v2, ci, S), axis=0, keepdims=True)
        t1 = jnp.clip(j1[0, 0], 0, S - 1)
        t2 = jnp.clip(j2[0, 0], 0, S - 1)
        b1 = pl.ds(pl.multiple_of((t1 // 8) * 8, 8), 8)
        b2 = pl.ds(pl.multiple_of((t2 // 8) * 8, 8), 8)
        xr = jnp.concatenate([xb_sc[b1, :], xb_sc[b2, :]], axis=0).astype(f32)
        rs = jnp.concatenate([rs_sc[b1, :], rs_sc[b2, :]], axis=0)[:, 0:1]
        c = xr - jnp.mean(xr, axis=-1, keepdims=True)
        xm = c * (rs / (1.0 + rs))
        xs = xm.astype(bf16)
        base = xr
        y = None
        for j in range(F // FC):
            gg = jnp.dot(xs, wg_sc[:, FC * j:FC * (j + 1)], preferred_element_type=f32)
            uu = jnp.dot(xs, wu_sc[:, FC * j:FC * (j + 1)], preferred_element_type=f32)
            hh = (gg * _sigmoid(gg) * uu).astype(bf16)
            t = jnp.dot(hh, wd_sc[FC * j:FC * (j + 1), :], preferred_element_type=f32)
            y = t if y is None else y + t
        r8 = lax.broadcasted_iota(jnp.int32, (8, D), 0)
        y1 = jnp.where(r8 == t1 % 8, y[0:8] * jnp.concatenate([_sigmoid(v1)] * (D // 128), axis=1), 0.0)
        y2 = jnp.where(r8 == t2 % 8, y[8:16] * jnp.concatenate([_sigmoid(v2)] * (D // 128), axis=1), 0.0)
        same = t1 // 8 == t2 // 8
        n1 = base[0:8] + (y1 + jnp.where(same, y2, 0.0))
        n2 = base[8:16] + (y2 + jnp.where(same, y1, 0.0))
        @pl.when(layer == 1)
        def _():
            for i in range(NOB):
                out_copy(i).wait()

        for b, xx in ((b1, n1), (b2, n2)):
            cc, v = _ln_stats(xx)
            xb_sc[b, :] = xx.astype(bf16)
            xn_sc[b, :] = (cc * lax.rsqrt(v + EPS)).astype(bf16)

        @pl.when(layer == 1)
        def _():
            c1 = pltpu.make_async_copy(xb_sc.at[b1, :], out_hbm.at[b1, :], sems.at[9])
            c1.start()

            @pl.when(jnp.logical_not(same))
            def _():
                c2 = pltpu.make_async_copy(xb_sc.at[b2, :], out_hbm.at[b2, :], sems.at[10])
                c2.start()
                c2.wait()
            c1.wait()

    def layer_body(layer, carry):
        @pl.when(layer == 1)
        def _():
            lax.fori_loop(0, NRB, proj_k_body, 0)
        lax.fori_loop(0, NRB, functools.partial(proj_qv_body, layer), 0)
        attn_phase()

        @pl.when(layer == 0)
        def _():
            cp["wr"].wait()

        out_phase(layer)

        @pl.when(layer == 0)
        def _():
            cp["wg"].wait()
            cp["wu"].wait()
            cp["wd"].wait()
        ffn(layer)
        return carry

    first_k_phase()
    lax.fori_loop(0, 2, layer_body, 0)


@jax.jit
def pallas_interleave_layers__memory_aug_infini_attn__moe_arch_mod__prompt_kernel(
    A_x: jax.Array,
    A_wq: jax.Array,
    A_wk: jax.Array,
    A_wv: jax.Array,
    A_wo: jax.Array,
    A_beta: jax.Array,
    B_x: jax.Array,
    B_w_r: jax.Array,
    B_w_gate: jax.Array,
    B_w_up: jax.Array,
    B_w_down: jax.Array,
):
    del B_x
    x = A_x.reshape(S, D)
    zero = jnp.zeros((1,), jnp.int32)
    beta = A_beta.astype(f32)
    wr = B_w_r.reshape(1, D)
    any_spec = pl.BlockSpec(memory_space=pl.ANY)
    smem_spec = pl.BlockSpec(memory_space=pltpu.SMEM)
    V = pltpu.VMEM
    scratch = [
        V((S, D), bf16),
        V((S, D), bf16),
        V((S, 128), f32),
        V((16, 128), f32), V((16, 128), jnp.int32),
        V((7, HD // 2, HD), u32), V((7, HD // 2, HD), u32), V((7, HD // 2, HD), u32), V((7, HD // 2, HD), u32),
        V((D, D), bf16), V((D, D), bf16), V((D, D), bf16), V((D, D), bf16),
        V((1, D), bf16),
        V((D, F), bf16), V((D, F), bf16), V((F, D), bf16),
        V((G, S, 128), bf16), V((G, S, 128), bf16),
        V((NRB, G, 128, RB), bf16), V((NRB, G, 128, RB), bf16), V((NRB, G, 128, RB), bf16),
        V((G, S, 128), bf16),
        V((NRB, G, 8, 128), f32),
        V((H, 8, 128), f32),
        V((128, 512), f32),
        pltpu.SemaphoreType.DMA((11,)),
        pltpu.SemaphoreType.DMA((NOB,)),
        pltpu.SemaphoreType.DMA((NRB,)),
        pltpu.SemaphoreType.DMA((NWK, 2)),
    ] + [V((T, 512), f32)] * NSLOT + [V((OS, D), f32)] * (OB // OS)
    out = pl.pallas_call(
        _kernel,
        in_specs=[smem_spec, smem_spec] + [any_spec] * 9,
        out_specs=any_spec,
        out_shape=jax.ShapeDtypeStruct((S, D), bf16),
        scratch_shapes=scratch,
        compiler_params=pltpu.CompilerParams(vmem_limit_bytes=120 * 1024 * 1024),
    )(zero, beta, x, A_wq, A_wk, A_wv, A_wo, wr, B_w_gate, B_w_up, B_w_down)
    return out.reshape(1, S, D)
```

```python
import functools
import itertools

import jax
import jax.numpy as jnp
from jax import lax
import jax.experimental.pallas as pl
import jax.experimental.pallas.tpu as pltpu

S, D, H, DH, NSEG, L, F = 2048, 1024, 32, 32, 4, 512, 3584
G = 8
LEV = 2
NP = 7 ** LEV
BD = D >> LEV
HD = D // 2
RB = 128 << LEV
NRB = S // RB
OB = 1024
NOB = S // OB
NOUT = 4
FC = 256
NWK = 4
T = 128
LAG = 5
NSLOT = 5
EPS = 1e-05
LOG2E = 1.4426950408889634
QSCALE = (DH ** -0.5) * LOG2E
NEG = -1e30
NT = (((1,), (1,)), ((), ()))
ORDER = (2, 3, 4, 0, 1, 6, 5)

f32 = jnp.float32
bf16 = jnp.bfloat16
u32 = jnp.uint32


def _phi(t):
    return jnp.where(t > 0, t + 1.0, jnp.exp(t))


def _sigmoid(t):
    return 1.0 / (1.0 + jnp.exp(-t))


def _pk(x):
    return pltpu.bitcast(x, u32)


def _upk(x):
    return pltpu.bitcast(x, bf16)


def _row_fold(x, op):
    parts = [x[8 * r:8 * r + 8] for r in range(x.shape[0] // 8)]
    while len(parts) > 1:
        parts = [op(parts[i], parts[i + 1]) if i + 1 < len(parts) else parts[i] for i in range(0, len(parts), 2)]
    return parts[0]


def _quads(x):
    h, w = x.shape[0] // 2, x.shape[1] // 2
    return x[:h, :w], x[:h, w:], x[h:, :w], x[h:, w:]


def _lhs_ops(x, lev):
    if lev == 0:
        return [x.astype(bf16)]
    x00, x01, x10, x11 = _quads(x)
    a00, a01, a10, a11 = (t.astype(f32) for t in (x00, x01, x10, x11))
    ops = (a00 + a11, a10 + a11, x00, x11, a00 + a01, a10 - a00, a01 - a11)
    return [o for t in ops for o in _lhs_ops(t, lev - 1)]


def _rhs_ops(w, lev):
    if lev == 0:
        return [w[()].astype(bf16)]

    def sub(r, c):
        return {p[1:]: v for p, v in w.items() if p[0] == (r, c)}

    def add(x, y, sign=1):
        return {p: (x[p].astype(f32) + y[p].astype(f32) if sign > 0 else x[p].astype(f32) - y[p].astype(f32))
                for p in x}
    b11, b12, b21, b22 = sub(0, 0), sub(0, 1), sub(1, 0), sub(1, 1)
    ops = (add(b11, b22), b11, add(b12, b22, -1), add(b21, b11, -1), b22, add(b11, b12), add(b21, b22))
    return [o for t in ops for o in _rhs_ops(t, lev - 1)]


def _offsets(path):
    r = sum(rc[0] * (D >> (i + 1)) for i, rc in enumerate(path))
    c = sum(rc[1] * (D >> (i + 1)) for i, rc in enumerate(path))
    return r, c


def _prep(t_ref, w_ref, n, nch, transposed):
    ch = BD // nch
    w = {}
    for path in itertools.product(((0, 0), (0, 1), (1, 0), (1, 1)), repeat=LEV):
        r, c = _offsets(path)
        if transposed:
            r, c = c, r
        w[path] = w_ref[pl.ds(pl.multiple_of(r + n * ch, ch), ch), c:c + BD]
    rows = pl.ds(pl.multiple_of(n * (ch // 2), ch // 2), ch // 2)
    for i, t in enumerate(_rhs_ops(w, LEV)):
        t_ref[i, rows, :] = _pk(t)


def _combine(M):
    m1, m2, m3, m4, m5, m6, m7 = M
    return m1 + m4 - m5 + m7, m3 + m5, m2 + m4, m1 - m2 + m3 + m6


def _strassen(mm, transposed):
    def assemble(c11, c12, c21, c22):
        if transposed:
            c12, c21 = c21, c12
        return jnp.concatenate([jnp.concatenate([c11, c12], axis=1), jnp.concatenate([c21, c22], axis=1)], axis=0)

    def rec(base, lev):
        M = [None] * 7
        for i in ORDER:
            M[i] = mm(base * 7 + i) if lev == 1 else assemble(*rec(base * 7 + i, lev - 1)[0])
        return _combine(M), M
    return rec(0, LEV)


def _kernel(zero_smem, beta_smem, x_hbm, wq_hbm, wk_hbm, wv_hbm, wo_hbm, wr_hbm,
            wg_hbm, wu_hbm, wd_hbm, out_hbm,
            x1_sc, xb_sc, xn_sc, mean_sc, rs_sc, cv_sc, ci_sc, tk_sc, tq_sc, tv_sc, to_sc,
            wq_sc, wk_sc, wv_sc, wo_sc, wT_sc, wr_sc,
            wg_sc, wu_sc, wd_sc, k_sc, pk_sc, qT_sc, pqT_sc, vT_sc, o_sc, z_sc,
            gt_sc, am_sc, sems, osems, xsems, ksems, *s_sc):
    cp = {
        "wq": pltpu.make_async_copy(wq_hbm, wq_sc, sems.at[0]),
        "wv": pltpu.make_async_copy(wv_hbm, wv_sc, sems.at[1]),
        "wo": pltpu.make_async_copy(wo_hbm, wo_sc, sems.at[2]),
        "wr": pltpu.make_async_copy(wr_hbm, wr_sc, sems.at[3]),
        "wg": pltpu.make_async_copy(wg_hbm, wg_sc, sems.at[4]),
        "wu": pltpu.make_async_copy(wu_hbm, wu_sc, sems.at[5]),
        "wd": pltpu.make_async_copy(wd_hbm, wd_sc, sems.at[6]),
    }

    def x_copy(rb):
        rows = pl.ds(pl.multiple_of(rb * RB, RB), RB)
        return pltpu.make_async_copy(x_hbm.at[rows, :], xb_sc.at[rows, :], xsems.at[rb])

    def wk_copy(n, part):
        rows = pl.ds(part * BD + n * (BD // NWK), BD // NWK)
        return pltpu.make_async_copy(wk_hbm.at[rows, :], wk_sc.at[rows, :], ksems.at[n, part])

    def out_copy(i):
        rows = pl.ds(i * (S // NOUT), S // NOUT)
        return pltpu.make_async_copy(xb_sc.at[rows, :], out_hbm.at[rows, :], osems.at[i])

    x_copy(0).start()
    for n in range(NWK):
        for part in range(1 << LEV):
            wk_copy(n, part).start()
    x_copy(1).start()
    zero = zero_smem[0]

    am_sc[...] = jnp.zeros((T, 4 * T), f32)

    def gate_body(h, carry):
        gt_sc[h] = _sigmoid(jnp.full((8, 128), beta_smem[h], f32))
        return carry
    lax.fori_loop(0, H, gate_body, 0)

    row = lax.broadcasted_iota(jnp.int32, (T, T), 0)
    col = lax.broadcasted_iota(jnp.int32, (T, T), 1)
    cmask = row <= col
    hmask = (row // 32) == (col // 32)
    zrow = lax.broadcasted_iota(jnp.int32, (32, T), 0)
    zcol = lax.broadcasted_iota(jnp.int32, (32, T), 1)
    zmask = (zrow // 8) == (zcol // 32)

    def rows_of(rb):
        return pl.ds(pl.multiple_of(rb * RB, RB), RB)

    def prep_nat(t_ref, w_ref):
        lax.fori_loop(0, 8, lambda n, c: (_prep(t_ref, w_ref, n, 8, False), c)[1], 0)

    def prep_tr(t_ref, w_ref):
        for j in range(4):
            for i in range(4):
                wT_sc[256 * j:256 * (j + 1), 256 * i:256 * (i + 1)] = w_ref[256 * i:256 * (i + 1), 256 * j:256 * (j + 1)].T
        lax.fori_loop(0, 8, lambda n, c: (_prep(t_ref, wT_sc, n, 8, True), c)[1], 0)

    QUADS = lambda c: ((c[1], 0, 1), (c[2], 1, 0), (c[0], 0, 0), (c[3], 1, 1))

    def ln_rows(rb, toks):
        ch = RB // 8
        never = jnp.full((ch, 1), zero, jnp.int32) != 0
        outs = []
        for n in range(8):
            x = xb_sc[pl.ds(pl.multiple_of(rb * RB + n * ch, ch), ch), :].astype(f32)
            m = jnp.mean(x, axis=-1, keepdims=True)
            if toks is not None and toks[n] is not None:
                x = jnp.where(never, toks[n], x)
            c = x - m
            v = jnp.mean(c * c, axis=-1, keepdims=True)
            outs.append((c * lax.rsqrt(v + EPS)).astype(bf16))
        xn = jnp.concatenate(outs, axis=0)
        xn_sc[rows_of(rb), :] = xn
        return xn

    def proj_k_body(layer, rb, xn):
        first = layer == 0

        @pl.when(jnp.logical_and(first, rb + 1 < NRB))
        def _():
            x_copy(rb + 1).wait()

        for j, names in enumerate(((2, "wq"), (3, "wv"), ("wo", "wr"))):
            @pl.when(jnp.logical_and(first, rb == j))
            def _():
                for nm in names:
                    (x_copy(nm) if isinstance(nm, int) else cp[nm]).start()

        h = RB // 2
        r0 = pl.multiple_of(rb * RB, RB)
        A = _lhs_ops(xn, LEV)
        c, MK = _strassen(lambda i: jnp.dot(A[i], _upk(tk_sc[i]), preferred_element_type=f32), False)
        zp = [None, None]
        for kk, th, nh in QUADS(c):
            pk = _phi(kk)
            zz = _row_fold(pk, jnp.add)
            zp[nh] = zz if zp[nh] is None else zp[nh] + zz
            rows = pl.ds(pl.multiple_of(r0 + th * h, h), h)
            for g in range(G // 2):
                k_sc[4 * nh + g, rows, :] = kk[:, 128 * g:128 * (g + 1)].astype(bf16)
                pk_sc[4 * nh + g, rows, :] = pk[:, 128 * g:128 * (g + 1)].astype(bf16)
        for nh in range(2):
            for g in range(G // 2):
                z_sc[rb, 4 * nh + g] = zp[nh][:, 128 * g:128 * (g + 1)]
        return ln_rows(jnp.minimum(rb + 1, NRB - 1), [None] + [MK[i][0:RB // 8, 0:1] for i in ORDER])

    def proj_q_body(layer, rb, carry):
        @pl.when(jnp.logical_and(layer == 0, rb == 0))
        def _():
            for name in ("wg", "wu", "wd"):
                cp[name].start()
        h = RB // 2
        A = _lhs_ops(xn_sc[rows_of(rb), :], LEV)
        c, _ = _strassen(lambda i: lax.dot_general(_upk(tq_sc[i]), A[i], NT, preferred_element_type=f32), True)
        for qq, th, nh in QUADS(c):
            pq = _phi(qq)
            for g in range(G // 2):
                qT_sc[rb, 4 * nh + g, :, th * h:(th + 1) * h] = (qq[128 * g:128 * (g + 1)] * QSCALE).astype(bf16)
                pqT_sc[rb, 4 * nh + g, :, th * h:(th + 1) * h] = pq[128 * g:128 * (g + 1)].astype(bf16)
        return carry

    def proj_v_body(rb, carry):
        h = RB // 2
        A = _lhs_ops(xn_sc[rows_of(rb), :], LEV)
        c, _ = _strassen(lambda i: lax.dot_general(_upk(tv_sc[i]), A[i], NT, preferred_element_type=f32), True)
        for vv, th, nh in QUADS(c):
            for g in range(G // 2):
                vT_sc[rb, 4 * nh + g, :, th * h:(th + 1) * h] = vv[128 * g:128 * (g + 1)].astype(bf16)
        return carry

    TILES = [(s, i) for s in range(NSEG) for i in (3, 2, 1, 0)]
    STREAM = [(t, c) for t, (s, i) in enumerate(TILES) for c in range(i + 1)]
    NPOS = len(STREAM)

    def sref(k, h):
        return s_sc[k % NSLOT].at[pl.ds(pl.multiple_of(zero, 8), T), T * h:T * (h + 1)]

    def tcols(ref, g, t0, n, rows=slice(None)):
        parts = []
        for t in range(t0, t0 + n, min(n, RB)):
            parts.append(ref[t // RB, g, rows, t % RB:t % RB + min(n, RB)])
        return parts[0] if len(parts) == 1 else jnp.concatenate(parts, axis=1)

    def q_weights(g, s, i):
        QT = tcols(qT_sc, g, s * L + i * T, T)
        z = jnp.zeros((32, T), bf16)
        return jnp.concatenate(
            [jnp.concatenate([QT[32 * h:32 * h + 32] if hh == h else z for hh in range(4)], axis=0)
             for h in range(4)], axis=1)

    def qk(g, k, m):
        t, c = STREAM[k]
        s, i = TILES[t]
        k0 = s * L + c * T
        K = k_sc[g, k0:k0 + T, :]
        S4 = jnp.dot(K, q_weights(g, s, i), preferred_element_type=f32)
        out = []
        for h in range(4):
            Sx = S4[:, T * h:T * (h + 1)]
            if c == i:
                Sx = jnp.where(cmask, Sx, NEG)
            sref(k, h)[...] = Sx
            mm = Sx[0:8]
            for r in range(1, 16):
                mm = jnp.maximum(mm, Sx[8 * r:8 * r + 8])
            mm = mm if c == 0 else jnp.maximum(m[h], mm)
            if c == i:
                mm = jnp.broadcast_to(jnp.max(mm, axis=0, keepdims=True), (8, T))
            out.append(mm)
        return out

    def attn_prologue():
        m = {}
        for k in range(LAG):
            t = STREAM[k][0]
            m[t] = qk(0, k, m.get(t))
        return tuple(m[STREAM[0][0]]) + tuple(m[STREAM[LAG - 1][0]])

    def finish(g, s, i, O, l):
        outs = []
        for h in range(4):
            lt = jnp.sum(l[h], axis=0, keepdims=True)
            gt = jnp.concatenate([gt_sc[4 * g + h]] * 4, axis=0)
            o = O[h] * ((1.0 - gt) * (1.0 / lt))
            if s > 0:
                o = o + am_sc[32 * h:32 * h + 32, i * T:(i + 1) * T]
            outs.append(o)
        ot = jnp.concatenate(outs, axis=0).astype(bf16)
        r0 = s * L + i * T
        o_sc[g, r0:r0 + T, :] = ot.T

    def attn_body(g, carry):
        gn = jnp.minimum(g + 1, G - 1)
        m = {STREAM[0][0]: list(carry[0:4]), STREAM[LAG - 1][0]: list(carry[4:8])}
        l, O, P, M, mn = {}, {}, {}, {}, {}

        def mem_read(s):
            zs = z_sc[0, g]
            for rb in range(1, s * L // RB):
                zs = zs + z_sc[rb, g]
            zs = jnp.sum(zs, axis=0, keepdims=True)
            zrows = jnp.where(zmask, zs, 0.0).astype(bf16)
            mbd = jnp.where(hmask, M[0], 0.0).astype(bf16)
            lhs = jnp.concatenate([mbd, zrows], axis=0)
            pq = tcols(pqT_sc, g, s * L, L)
            nd = jnp.dot(lhs, pq, preferred_element_type=f32)
            for h in range(4):
                den = nd[128 + 8 * h:128 + 8 * h + 8] + 1e-06
                gd = jnp.concatenate([gt_sc[4 * g + h]] * 4, axis=1) / den
                am_sc[32 * h:32 * h + 32, :] = nd[32 * h:32 * h + 32] * jnp.concatenate([gd] * 4, axis=0)

        def mem_write(s):
            vt = tcols(vT_sc, g, s * L, L)
            pk = pk_sc[g, s * L:(s + 1) * L, :]
            inc = jnp.dot(vt, pk, preferred_element_type=f32)
            M[0] = inc if s == 0 else M[0] + inc

        def ex(k):
            t, c = STREAM[k]
            out = []
            for h in range(4):
                Pp = jnp.exp2(sref(k, h)[...] - jnp.concatenate([m[t][h]] * (T // 8), axis=0))
                a = Pp[0:8] + Pp[8:16]
                b = Pp[16:24] + Pp[24:32]
                for r in range(2, 8, 2):
                    a = a + (Pp[16 * r:16 * r + 8] + Pp[16 * r + 8:16 * r + 16])
                    b = b + (Pp[16 * r + 16:16 * r + 24] + Pp[16 * r + 24:16 * r + 32])
                ll = a + b
                if c == 0:
                    l.setdefault(t, [None] * 4)[h] = ll
                else:
                    l[t][h] = l[t][h] + ll
                out.append(Pp.astype(bf16))
            P[k] = out

        def pv(k):
            t, c = STREAM[k]
            s, i = TILES[t]
            if c == 0:
                O[t] = [None] * 4
            for h in range(4):
                vt = tcols(vT_sc, g, s * L + c * T, T, slice(32 * h, 32 * h + 32))
                o = jnp.dot(vt, P[k][h], preferred_element_type=f32)
                O[t][h] = o if O[t][h] is None else O[t][h] + o
            del P[k]

        finish(jnp.maximum(g - 1, 0), NSEG - 1, 0, carry[8:12], carry[12:16])
        done = None
        for j in range(NPOS):
            ex(j)
            k = j + LAG
            if k < NPOS:
                t = STREAM[k][0]
                m[t] = qk(g, k, m.get(t))
            else:
                t = STREAM[k - NPOS][0]
                mn[t] = qk(gn, k - NPOS, mn.get(t))
            pv(j)
            if done is not None:
                s, i = TILES[done]
                finish(g, s, i, O[done], l[done])
                if i == 0:
                    mem_read(s + 1)
                done = None
            t, c = STREAM[j]
            if c == TILES[t][1]:
                done = t
                if TILES[t][1] == 3 and TILES[t][0] < NSEG - 1:
                    mem_write(TILES[t][0])
        return (tuple(mn[STREAM[0][0]]) + tuple(mn[STREAM[LAG - 1][0]]) + tuple(O[done]) + tuple(l[done]))

    def attn_phase():
        init = attn_prologue() + (jnp.zeros((32, T), f32),) * 4 + (jnp.ones((8, T), f32),) * 4
        carry = lax.fori_loop(0, G, attn_body, init)
        finish(G - 1, NSEG - 1, 0, carry[8:12], carry[12:16])

    def out_body(ob_i, top):
        wr = wr_sc[...].astype(f32)
        wr_sum = jnp.sum(wr, axis=-1, keepdims=True)
        h = RB // 2
        m1, i1, m2, i2 = top
        for k in range(OB // RB):
            r0 = pl.multiple_of(ob_i * OB + k * RB, RB)
            ob = jnp.concatenate([o_sc[g, pl.ds(r0, RB), :] for g in range(G)], axis=1)
            A = _lhs_ops(ob, LEV)
            c, _ = _strassen(lambda i: jnp.dot(A[i], _upk(to_sc[i]), preferred_element_type=f32), False)
            acc = [[None] * 3, [None] * 3]
            for cc, th, nh in QUADS(c):
                rows = pl.ds(pl.multiple_of(r0 + th * h, h), h)
                cols = slice(nh * HD, (nh + 1) * HD)
                x1 = xb_sc[rows, cols].astype(f32) + cc
                x1_sc[rows, cols] = x1
                s1, s2, st = acc[th]
                for n in range(HD // 128):
                    d = x1[:, 128 * n:128 * (n + 1)]
                    s1 = d if s1 is None else s1 + d
                    s2 = d * d if s2 is None else s2 + d * d
                    t = d * wr[:, nh * HD + 128 * n:nh * HD + 128 * (n + 1)]
                    st = t if st is None else st + t
                acc[th] = [s1, s2, st]
            for th in range(2):
                s1, s2, st = acc[th]
                rows = pl.ds(pl.multiple_of(r0 + th * h, h), h)
                mean = jnp.sum(s1, axis=-1, keepdims=True) * (1.0 / D)
                v = jnp.maximum(jnp.sum(s2, axis=-1, keepdims=True) * (1.0 / D) - mean * mean, 0.0)
                rs = lax.rsqrt(v + EPS)
                r = rs * (jnp.sum(st, axis=-1, keepdims=True) - mean * wr_sum)
                r = r.astype(bf16).astype(f32)
                mean_sc[rows, :] = jnp.broadcast_to(mean, (h, 128))
                rs_sc[rows, :] = jnp.broadcast_to(rs, (h, 128))
                sub = lax.broadcasted_iota(jnp.int32, (8, 1), 0) + (r0 + th * h)
                for j in range(h // 8):
                    rj = r[8 * j:8 * j + 8]
                    idx = sub + 8 * j
                    g1 = rj > m1
                    g2 = rj > m2
                    m2 = jnp.where(g1, m1, jnp.where(g2, rj, m2))
                    i2 = jnp.where(g1, i1, jnp.where(g2, idx, i2))
                    m1 = jnp.where(g1, rj, m1)
                    i1 = jnp.where(g1, idx, i1)
        return m1, i1, m2, i2

    def out_phase():
        top = (jnp.full((8, 1), -jnp.inf, f32), jnp.zeros((8, 1), jnp.int32),
               jnp.full((8, 1), -jnp.inf, f32), jnp.ones((8, 1), jnp.int32))
        return lax.fori_loop(0, NOB, out_body, top)

    def ffn(layer, top):
        m1, i1, m2, i2 = top
        cv = jnp.concatenate([m1, m2], axis=0)
        ci = jnp.concatenate([i1, i2], axis=0)
        v1 = jnp.max(cv, axis=0, keepdims=True)
        j1 = jnp.min(jnp.where(cv == v1, ci, S), axis=0, keepdims=True)
        cv2 = jnp.where(ci == j1, -jnp.inf, cv)
        v2 = jnp.max(cv2, axis=0, keepdims=True)
        j2 = jnp.min(jnp.where(cv2 == v2, ci, S), axis=0, keepdims=True)
        t1 = jnp.clip(j1[0, 0], 0, S - 1)
        t2 = jnp.clip(j2[0, 0], 0, S - 1)
        b1 = pl.ds(pl.multiple_of((t1 // 8) * 8, 8), 8)
        b2 = pl.ds(pl.multiple_of((t2 // 8) * 8, 8), 8)

        def two(ref):
            return jnp.concatenate([ref[b1, :], ref[b2, :]], axis=0)
        xm = (two(x1_sc) - two(mean_sc)[:, 0:1]) * two(rs_sc)[:, 0:1]
        xs = xm.astype(bf16)
        base = two(x1_sc) + xm

        NCH = 16
        CH = S // NCH
        never = jnp.full((CH, 1), zero, jnp.int32) != 0

        def mod_rows(n, tok):
            rows = slice(n * CH, (n + 1) * CH)
            x1 = x1_sc[rows, :]
            mn = mean_sc[rows, 0:1]
            if tok is not None:
                mn = jnp.where(never, tok, mn)
            xb_sc[rows, :] = (x1 + (x1 - mn) * rs_sc[rows, 0:1]).astype(bf16)
            if (n + 1) % (NCH // NOUT) == 0:
                @pl.when(layer == 1)
                def _():
                    out_copy(n // (NCH // NOUT)).start()

        y = None
        mod_rows(0, None)
        mod_rows(1, None)
        for j in range(F // FC):
            gg = jnp.dot(xs, wg_sc[:, FC * j:FC * (j + 1)], preferred_element_type=f32)
            uu = jnp.dot(xs, wu_sc[:, FC * j:FC * (j + 1)], preferred_element_type=f32)
            hh = (gg * _sigmoid(gg) * uu).astype(bf16)
            t = jnp.dot(hh, wd_sc[FC * j:FC * (j + 1), :], preferred_element_type=f32)
            y = t if y is None else y + t
            mod_rows(2 + j, jnp.broadcast_to(gg[0:1, 0:1], (CH, 1)))
        r8 = lax.broadcasted_iota(jnp.int32, (8, D), 0)
        y1 = jnp.where(r8 == t1 % 8, y[0:8] * _sigmoid(v1), 0.0)
        y2 = jnp.where(r8 == t2 % 8, y[8:16] * _sigmoid(v2), 0.0)
        same = t1 // 8 == t2 // 8
        n1 = base[0:8] + (y1 + jnp.where(same, y2, 0.0))
        n2 = base[8:16] + (y2 + jnp.where(same, y1, 0.0))

        @pl.when(layer == 1)
        def _():
            for i in range(NOUT):
                out_copy(i).wait()

        xb_sc[b1, :] = n1.astype(bf16)
        xb_sc[b2, :] = n2.astype(bf16)

        @pl.when(layer == 1)
        def _():
            c1 = pltpu.make_async_copy(xb_sc.at[b1, :], out_hbm.at[b1, :], sems.at[7])
            c1.start()

            @pl.when(jnp.logical_not(same))
            def _():
                c2 = pltpu.make_async_copy(xb_sc.at[b2, :], out_hbm.at[b2, :], sems.at[8])
                c2.start()
                c2.wait()
            c1.wait()

    def layer_body(layer, carry):
        first = layer == 0

        @pl.when(first)
        def _():
            x_copy(0).wait()
        xn = ln_rows(0, None)

        @pl.when(first)
        def _():
            def piece(n, c):
                for part in range(1 << LEV):
                    wk_copy(n, part).wait()
                for m in range(8 // NWK):
                    _prep(tk_sc, wk_sc, n * (8 // NWK) + m, 8, False)
                return c
            lax.fori_loop(0, NWK, piece, 0)
        lax.fori_loop(0, NRB, functools.partial(proj_k_body, layer), xn)

        @pl.when(first)
        def _():
            cp["wq"].wait()
            prep_tr(tq_sc, wq_sc)
        lax.fori_loop(0, NRB, functools.partial(proj_q_body, layer), 0)

        @pl.when(first)
        def _():
            cp["wv"].wait()
            prep_tr(tv_sc, wv_sc)
        lax.fori_loop(0, NRB, proj_v_body, 0)
        attn_phase()

        @pl.when(first)
        def _():
            cp["wo"].wait()
            cp["wr"].wait()
            prep_nat(to_sc, wo_sc)
        top = out_phase()

        @pl.when(first)
        def _():
            cp["wg"].wait()
            cp["wu"].wait()
            cp["wd"].wait()
        ffn(layer, top)
        return carry

    lax.fori_loop(0, 2, layer_body, 0)


@jax.jit
def pallas_interleave_layers__memory_aug_infini_attn__moe_arch_mod__prompt_kernel(
    A_x: jax.Array,
    A_wq: jax.Array,
    A_wk: jax.Array,
    A_wv: jax.Array,
    A_wo: jax.Array,
    A_beta: jax.Array,
    B_x: jax.Array,
    B_w_r: jax.Array,
    B_w_gate: jax.Array,
    B_w_up: jax.Array,
    B_w_down: jax.Array,
):
    del B_x
    x = A_x.reshape(S, D)
    zero = jnp.zeros((1,), jnp.int32)
    beta = A_beta.astype(f32)
    wr = B_w_r.reshape(1, D)
    any_spec = pl.BlockSpec(memory_space=pl.ANY)
    smem_spec = pl.BlockSpec(memory_space=pltpu.SMEM)
    V = pltpu.VMEM
    scratch = [
        V((S, D), f32),
        V((S, D), bf16),
        V((S, D), bf16),
        V((S, 128), f32), V((S, 128), f32),
        V((16, 128), f32), V((16, 128), jnp.int32),
    ] + [V((NP, BD // 2, BD), u32)] * 4 + [
        V((D, D), bf16), V((D, D), bf16), V((D, D), bf16), V((D, D), bf16),
        V((D, D), bf16),
        V((1, D), bf16),
        V((D, F), bf16), V((D, F), bf16), V((F, D), bf16),
        V((G, S, 128), bf16), V((G, S, 128), bf16),
        V((NRB, G, 128, RB), bf16), V((NRB, G, 128, RB), bf16), V((NRB, G, 128, RB), bf16),
        V((G, S, 128), bf16),
        V((NRB, G, 8, 128), f32),
        V((H, 8, 128), f32),
        V((T, 4 * T), f32),
        pltpu.SemaphoreType.DMA((9,)),
        pltpu.SemaphoreType.DMA((NOUT,)),
        pltpu.SemaphoreType.DMA((NRB,)),
        pltpu.SemaphoreType.DMA((NWK, 1 << LEV)),
    ] + [V((T, 4 * T), f32)] * NSLOT
    out = pl.pallas_call(
        _kernel,
        in_specs=[smem_spec, smem_spec] + [any_spec] * 9,
        out_specs=any_spec,
        out_shape=jax.ShapeDtypeStruct((S, D), bf16),
        scratch_shapes=scratch,
        compiler_params=pltpu.CompilerParams(vmem_limit_bytes=120 * 1024 * 1024),
    )(zero, beta, x, A_wq, A_wk, A_wv, A_wo, wr, B_w_gate, B_w_up, B_w_down)
    return out.reshape(1, S, D)
```

```python
import functools
import itertools

import jax
import jax.numpy as jnp
from jax import lax
import jax.experimental.pallas as pl
import jax.experimental.pallas.tpu as pltpu

S, D, H, DH, NSEG, L, F = 2048, 1024, 32, 32, 4, 512, 3584
G = 8
LEV = 2
NP = 7 ** LEV
BD = D >> LEV
HD = D // 2
RB = 128 << LEV
NRB = S // RB
OB = 1024
NOB = S // OB
NOUT = 4
FC = 256
NWK = 4
T = 128
LAG = 5
NSLOT = 5
EPS = 1e-05
LOG2E = 1.4426950408889634
QSCALE = (DH ** -0.5) * LOG2E
NEG = -1e30
NT = (((1,), (1,)), ((), ()))
ORDER = (2, 4, 3, 1, 0, 6, 5)

f32 = jnp.float32
bf16 = jnp.bfloat16
u32 = jnp.uint32


def _phi(t):
    return jnp.where(t > 0, t + 1.0, jnp.exp(t))


def _sigmoid(t):
    return 1.0 / (1.0 + jnp.exp(-t))


def _pk(x):
    return pltpu.bitcast(x, u32)


def _upk(x):
    return pltpu.bitcast(x, bf16)


def _row_fold(x, op):
    parts = [x[8 * r:8 * r + 8] for r in range(x.shape[0] // 8)]
    while len(parts) > 1:
        parts = [op(parts[i], parts[i + 1]) if i + 1 < len(parts) else parts[i] for i in range(0, len(parts), 2)]
    return parts[0]


def _quads(x):
    h, w = x.shape[0] // 2, x.shape[1] // 2
    return x[:h, :w], x[:h, w:], x[h:, :w], x[h:, w:]


def _lhs_ops(x, lev):
    if lev == 0:
        return [x.astype(bf16)]
    x00, x01, x10, x11 = _quads(x)
    a00, a01, a10, a11 = (t.astype(f32) for t in (x00, x01, x10, x11))
    ops = (a00 + a11, a10 + a11, x00, x11, a00 + a01, a10 - a00, a01 - a11)
    return [o for t in ops for o in _lhs_ops(t, lev - 1)]


def _rhs_ops(w, lev):
    if lev == 0:
        return [w[()].astype(bf16)]

    def sub(r, c):
        return {p[1:]: v for p, v in w.items() if p[0] == (r, c)}

    def add(x, y, sign=1):
        return {p: (x[p].astype(f32) + y[p].astype(f32) if sign > 0 else x[p].astype(f32) - y[p].astype(f32))
                for p in x}
    b11, b12, b21, b22 = sub(0, 0), sub(0, 1), sub(1, 0), sub(1, 1)
    ops = (add(b11, b22), b11, add(b12, b22, -1), add(b21, b11, -1), b22, add(b11, b12), add(b21, b22))
    return [o for t in ops for o in _rhs_ops(t, lev - 1)]


def _offsets(path):
    r = sum(rc[0] * (D >> (i + 1)) for i, rc in enumerate(path))
    c = sum(rc[1] * (D >> (i + 1)) for i, rc in enumerate(path))
    return r, c


def _prep(t_ref, w_ref, n, nch, transposed):
    ch = BD // nch
    w = {}
    for path in itertools.product(((0, 0), (0, 1), (1, 0), (1, 1)), repeat=LEV):
        r, c = _offsets(path)
        if transposed:
            r, c = c, r
        w[path] = w_ref[pl.ds(pl.multiple_of(r + n * ch, ch), ch), c:c + BD]
    rows = pl.ds(pl.multiple_of(n * (ch // 2), ch // 2), ch // 2)
    for i, t in enumerate(_rhs_ops(w, LEV)):
        t_ref[i, rows, :] = _pk(t)


def _combine(M):
    m1, m2, m3, m4, m5, m6, m7 = M
    return m1 + m4 - m5 + m7, m3 + m5, m2 + m4, m1 - m2 + m3 + m6


def _strassen(mm, transposed):
    def assemble(c11, c12, c21, c22):
        if transposed:
            c12, c21 = c21, c12
        return jnp.concatenate([jnp.concatenate([c11, c12], axis=1), jnp.concatenate([c21, c22], axis=1)], axis=0)

    def rec(base, lev):
        M = [None] * 7
        for i in ORDER:
            M[i] = mm(base * 7 + i) if lev == 1 else assemble(*rec(base * 7 + i, lev - 1)[0])
        return _combine(M), M
    return rec(0, LEV)


def _kernel(zero_smem, beta_smem, x_hbm, wq_hbm, wk_hbm, wv_hbm, wo_hbm, wr_hbm,
            wg_hbm, wu_hbm, wd_hbm, out_hbm,
            x1_sc, xb_sc, xn_sc, mean_sc, rs_sc, kn_sc, tk_sc, tq_sc, tv_sc, to_sc,
            wq_sc, wk_sc, wv_sc, wo_sc, wT_sc, wr_sc,
            wg_sc, wu_sc, wd_sc, k_sc, pk_sc, qT_sc, pqT_sc, vT_sc, o_sc, z_sc,
            gt_sc, am_sc, sems, osems, xsems, ksems, *s_sc):
    cp = {
        "wq": pltpu.make_async_copy(wq_hbm, wq_sc, sems.at[0]),
        "wv": pltpu.make_async_copy(wv_hbm, wv_sc, sems.at[1]),
        "wo": pltpu.make_async_copy(wo_hbm, wo_sc, sems.at[2]),
        "wr": pltpu.make_async_copy(wr_hbm, wr_sc, sems.at[3]),
        "wg": pltpu.make_async_copy(wg_hbm, wg_sc, sems.at[4]),
        "wu": pltpu.make_async_copy(wu_hbm, wu_sc, sems.at[5]),
        "wd": pltpu.make_async_copy(wd_hbm, wd_sc, sems.at[6]),
    }

    def x_copy(rb):
        rows = pl.ds(pl.multiple_of(rb * RB, RB), RB)
        return pltpu.make_async_copy(x_hbm.at[rows, :], xb_sc.at[rows, :], xsems.at[rb])

    def wk_copy(n, part):
        rows = pl.ds(part * BD + n * (BD // NWK), BD // NWK)
        return pltpu.make_async_copy(wk_hbm.at[rows, :], wk_sc.at[rows, :], ksems.at[n, part])

    def out_copy(i):
        rows = pl.ds(i * (S // NOUT), S // NOUT)
        return pltpu.make_async_copy(xb_sc.at[rows, :], out_hbm.at[rows, :], osems.at[i])

    for rb in range(NRB):
        x_copy(rb).start()
    zero = zero_smem[0]

    am_sc[...] = jnp.zeros((T, 4 * T), f32)

    def gate_body(h, carry):
        gt_sc[h] = _sigmoid(jnp.full((8, 128), beta_smem[h], f32))
        return carry
    lax.fori_loop(0, H, gate_body, 0)

    row = lax.broadcasted_iota(jnp.int32, (T, T), 0)
    col = lax.broadcasted_iota(jnp.int32, (T, T), 1)
    cmask = row <= col
    hmask = (row // 32) == (col // 32)
    zrow = lax.broadcasted_iota(jnp.int32, (32, T), 0)
    zcol = lax.broadcasted_iota(jnp.int32, (32, T), 1)
    zmask = (zrow // 8) == (zcol // 32)

    def rows_of(rb):
        return pl.ds(pl.multiple_of(rb * RB, RB), RB)

    def prep_nat(t_ref, w_ref):
        lax.fori_loop(0, 8, lambda n, c: (_prep(t_ref, w_ref, n, 8, False), c)[1], 0)

    def prep_tr(t_ref, w_ref):
        for j in range(4):
            for i in range(4):
                wT_sc[256 * j:256 * (j + 1), 256 * i:256 * (i + 1)] = w_ref[256 * i:256 * (i + 1), 256 * j:256 * (j + 1)].T
        lax.fori_loop(0, 8, lambda n, c: (_prep(t_ref, wT_sc, n, 8, True), c)[1], 0)

    QUADS = lambda c: ((c[1], 0, 1), (c[2], 1, 0), (c[0], 0, 0), (c[3], 1, 1))

    def ln_input(rb, carry):
        x_copy(rb).wait()

        @pl.when(rb == 0)
        def _():
            for n in range(NWK):
                for part in range(1 << LEV):
                    wk_copy(n, part).start()
        for n in range(RB // 128):
            rows = pl.ds(pl.multiple_of(rb * RB + n * 128, 128), 128)
            x = xb_sc[rows, :].astype(f32)
            c = x - jnp.mean(x, axis=-1, keepdims=True)
            v = jnp.mean(c * c, axis=-1, keepdims=True)
            xn_sc[rows, :] = (c * lax.rsqrt(v + EPS)).astype(bf16)
        return carry

    def proj_k_body(layer, rb, carry):
        for j, name in enumerate(("wq", "wv", "wo", "wr")):
            @pl.when(jnp.logical_and(layer == 0, rb == j))
            def _():
                cp[name].start()
        h = RB // 2
        r0 = pl.multiple_of(rb * RB, RB)
        A = _lhs_ops(xn_sc[rows_of(rb), :], LEV)
        c, _ = _strassen(lambda i: jnp.dot(A[i], _upk(tk_sc[i]), preferred_element_type=f32), False)
        zp = [None, None]
        for kk, th, nh in QUADS(c):
            pk = _phi(kk)
            zz = _row_fold(pk, jnp.add)
            zp[nh] = zz if zp[nh] is None else zp[nh] + zz
            rows = pl.ds(pl.multiple_of(r0 + th * h, h), h)
            for g in range(G // 2):
                k_sc[4 * nh + g, rows, :] = kk[:, 128 * g:128 * (g + 1)].astype(bf16)
                pk_sc[4 * nh + g, rows, :] = pk[:, 128 * g:128 * (g + 1)].astype(bf16)
        for nh in range(2):
            for g in range(G // 2):
                z_sc[rb, 4 * nh + g] = zp[nh][:, 128 * g:128 * (g + 1)]
        return carry

    def proj_q_body(layer, rb, carry):
        @pl.when(jnp.logical_and(layer == 0, rb == 0))
        def _():
            for name in ("wg", "wu", "wd"):
                cp[name].start()
        h = RB // 2
        A = _lhs_ops(xn_sc[rows_of(rb), :], LEV)
        c, _ = _strassen(lambda i: lax.dot_general(_upk(tq_sc[i]), A[i], NT, preferred_element_type=f32), True)
        for qq, th, nh in QUADS(c):
            pq = _phi(qq)
            for g in range(G // 2):
                qT_sc[rb, 4 * nh + g, :, th * h:(th + 1) * h] = (qq[128 * g:128 * (g + 1)] * QSCALE).astype(bf16)
                pqT_sc[rb, 4 * nh + g, :, th * h:(th + 1) * h] = pq[128 * g:128 * (g + 1)].astype(bf16)
        return carry

    def proj_v_body(rb, carry):
        h = RB // 2
        A = _lhs_ops(xn_sc[rows_of(rb), :], LEV)
        c, _ = _strassen(lambda i: lax.dot_general(_upk(tv_sc[i]), A[i], NT, preferred_element_type=f32), True)
        for vv, th, nh in QUADS(c):
            for g in range(G // 2):
                vT_sc[rb, 4 * nh + g, :, th * h:(th + 1) * h] = vv[128 * g:128 * (g + 1)].astype(bf16)
        return carry

    TILES = [(s, i) for s in range(NSEG) for i in (3, 2, 1, 0)]
    STREAM = [(t, c) for t, (s, i) in enumerate(TILES) for c in range(i + 1)]
    NPOS = len(STREAM)

    def sref(k, h):
        return s_sc[k % NSLOT].at[pl.ds(pl.multiple_of(zero, 8), T), T * h:T * (h + 1)]

    def tcols(ref, g, t0, n, rows=slice(None)):
        parts = []
        for t in range(t0, t0 + n, min(n, RB)):
            parts.append(ref[t // RB, g, rows, t % RB:t % RB + min(n, RB)])
        return parts[0] if len(parts) == 1 else jnp.concatenate(parts, axis=1)

    def q_weights(g, s, i):
        QT = tcols(qT_sc, g, s * L + i * T, T)
        z = jnp.zeros((32, T), bf16)
        return jnp.concatenate(
            [jnp.concatenate([QT[32 * h:32 * h + 32] if hh == h else z for hh in range(4)], axis=0)
             for h in range(4)], axis=1)

    def qk(g, k, m):
        t, c = STREAM[k]
        s, i = TILES[t]
        k0 = s * L + c * T
        K = k_sc[g, k0:k0 + T, :]
        S4 = jnp.dot(K, q_weights(g, s, i), preferred_element_type=f32)
        out = []
        for h in range(4):
            Sx = S4[:, T * h:T * (h + 1)]
            if c == i:
                Sx = jnp.where(cmask, Sx, NEG)
            sref(k, h)[...] = Sx
            mm = Sx[0:8]
            for r in range(1, 16):
                mm = jnp.maximum(mm, Sx[8 * r:8 * r + 8])
            mm = mm if c == 0 else jnp.maximum(m[h], mm)
            if c == i:
                mm = jnp.broadcast_to(jnp.max(mm, axis=0, keepdims=True), (8, T))
            out.append(mm)
        return out

    def attn_prologue():
        m = {}
        for k in range(LAG):
            t = STREAM[k][0]
            m[t] = qk(0, k, m.get(t))
        return tuple(m[STREAM[0][0]]) + tuple(m[STREAM[LAG - 1][0]])

    def finish(g, s, i, O, l):
        outs = []
        for h in range(4):
            lt = jnp.sum(l[h], axis=0, keepdims=True)
            gt = jnp.concatenate([gt_sc[4 * g + h]] * 4, axis=0)
            o = O[h] * ((1.0 - gt) * (1.0 / lt))
            if s > 0:
                o = o + am_sc[32 * h:32 * h + 32, i * T:(i + 1) * T]
            outs.append(o)
        ot = jnp.concatenate(outs, axis=0).astype(bf16)
        r0 = s * L + i * T
        o_sc[g, r0:r0 + T, :] = ot.T

    def attn_body(g, carry):
        gn = jnp.minimum(g + 1, G - 1)
        m = {STREAM[0][0]: list(carry[0:4]), STREAM[LAG - 1][0]: list(carry[4:8])}
        l, O, P, M, mn = {}, {}, {}, {}, {}

        def mem_read(s):
            zs = z_sc[0, g]
            for rb in range(1, s * L // RB):
                zs = zs + z_sc[rb, g]
            zs = jnp.sum(zs, axis=0, keepdims=True)
            zrows = jnp.where(zmask, zs, 0.0).astype(bf16)
            mbd = jnp.where(hmask, M[0], 0.0).astype(bf16)
            lhs = jnp.concatenate([mbd, zrows], axis=0)
            pq = tcols(pqT_sc, g, s * L, L)
            nd = jnp.dot(lhs, pq, preferred_element_type=f32)
            for h in range(4):
                den = nd[128 + 8 * h:128 + 8 * h + 8] + 1e-06
                gd = jnp.concatenate([gt_sc[4 * g + h]] * 4, axis=1) / den
                am_sc[32 * h:32 * h + 32, :] = nd[32 * h:32 * h + 32] * jnp.concatenate([gd] * 4, axis=0)

        def mem_write(s):
            vt = tcols(vT_sc, g, s * L, L)
            pk = pk_sc[g, s * L:(s + 1) * L, :]
            inc = jnp.dot(vt, pk, preferred_element_type=f32)
            M[0] = inc if s == 0 else M[0] + inc

        def ex(k):
            t, c = STREAM[k]
            out = []
            for h in range(4):
                Pp = jnp.exp2(sref(k, h)[...] - jnp.concatenate([m[t][h]] * (T // 8), axis=0))
                a = Pp[0:8] + Pp[8:16]
                b = Pp[16:24] + Pp[24:32]
                for r in range(2, 8, 2):
                    a = a + (Pp[16 * r:16 * r + 8] + Pp[16 * r + 8:16 * r + 16])
                    b = b + (Pp[16 * r + 16:16 * r + 24] + Pp[16 * r + 24:16 * r + 32])
                ll = a + b
                if c == 0:
                    l.setdefault(t, [None] * 4)[h] = ll
                else:
                    l[t][h] = l[t][h] + ll
                out.append(Pp.astype(bf16))
            P[k] = out

        def pv(k):
            t, c = STREAM[k]
            s, i = TILES[t]
            if c == 0:
                O[t] = [None] * 4
            for h in range(4):
                vt = tcols(vT_sc, g, s * L + c * T, T, slice(32 * h, 32 * h + 32))
                o = jnp.dot(vt, P[k][h], preferred_element_type=f32)
                O[t][h] = o if O[t][h] is None else O[t][h] + o
            del P[k]

        finish(jnp.maximum(g - 1, 0), NSEG - 1, 0, carry[8:12], carry[12:16])
        done = None
        for j in range(NPOS):
            ex(j)
            k = j + LAG
            if k < NPOS:
                t = STREAM[k][0]
                m[t] = qk(g, k, m.get(t))
            else:
                t = STREAM[k - NPOS][0]
                mn[t] = qk(gn, k - NPOS, mn.get(t))
            pv(j)
            if done is not None:
                s, i = TILES[done]
                finish(g, s, i, O[done], l[done])
                if i == 0:
                    mem_read(s + 1)
                done = None
            t, c = STREAM[j]
            if c == TILES[t][1]:
                done = t
                if TILES[t][1] == 3 and TILES[t][0] < NSEG - 1:
                    mem_write(TILES[t][0])
        return (tuple(mn[STREAM[0][0]]) + tuple(mn[STREAM[LAG - 1][0]]) + tuple(O[done]) + tuple(l[done]))

    def attn_phase():
        init = attn_prologue() + (jnp.zeros((32, T), f32),) * 4 + (jnp.ones((8, T), f32),) * 4
        carry = lax.fori_loop(0, G, attn_body, init)
        finish(G - 1, NSEG - 1, 0, carry[8:12], carry[12:16])

    def out_body(ob_i, top):
        wr = wr_sc[...].astype(f32)
        wr_sum = jnp.sum(wr, axis=-1, keepdims=True)
        h = RB // 2
        m1, i1, m2, i2 = top
        for k in range(OB // RB):
            r0 = pl.multiple_of(ob_i * OB + k * RB, RB)
            ob = jnp.concatenate([o_sc[g, pl.ds(r0, RB), :] for g in range(G)], axis=1)
            A = _lhs_ops(ob, LEV)
            c, _ = _strassen(lambda i: jnp.dot(A[i], _upk(to_sc[i]), preferred_element_type=f32), False)
            acc = [[None] * 3, [None] * 3]
            for cc, th, nh in QUADS(c):
                rows = pl.ds(pl.multiple_of(r0 + th * h, h), h)
                cols = slice(nh * HD, (nh + 1) * HD)
                x1 = xb_sc[rows, cols].astype(f32) + cc
                x1_sc[rows, cols] = x1
                s1, s2, st = acc[th]
                for n in range(HD // 128):
                    d = x1[:, 128 * n:128 * (n + 1)]
                    s1 = d if s1 is None else s1 + d
                    s2 = d * d if s2 is None else s2 + d * d
                    t = d * wr[:, nh * HD + 128 * n:nh * HD + 128 * (n + 1)]
                    st = t if st is None else st + t
                acc[th] = [s1, s2, st]
            for th in range(2):
                s1, s2, st = acc[th]
                rows = pl.ds(pl.multiple_of(r0 + th * h, h), h)
                mean = jnp.sum(s1, axis=-1, keepdims=True) * (1.0 / D)
                v = jnp.maximum(jnp.sum(s2, axis=-1, keepdims=True) * (1.0 / D) - mean * mean, 0.0)
                rs = lax.rsqrt(v + EPS)
                r = rs * (jnp.sum(st, axis=-1, keepdims=True) - mean * wr_sum)
                r = r.astype(bf16).astype(f32)
                mean_sc[rows, :] = jnp.broadcast_to(mean, (h, 128))
                rs_sc[rows, :] = jnp.broadcast_to(rs, (h, 128))
                a = 1.0 + rs
                kn_sc[rows, :] = jnp.broadcast_to(a * lax.rsqrt(v * (a * a) + EPS), (h, 128))
                sub = lax.broadcasted_iota(jnp.int32, (8, 1), 0) + (r0 + th * h)
                for j in range(h // 8):
                    rj = r[8 * j:8 * j + 8]
                    idx = sub + 8 * j
                    g1 = rj > m1
                    g2 = rj > m2
                    m2 = jnp.where(g1, m1, jnp.where(g2, rj, m2))
                    i2 = jnp.where(g1, i1, jnp.where(g2, idx, i2))
                    m1 = jnp.where(g1, rj, m1)
                    i1 = jnp.where(g1, idx, i1)
        return m1, i1, m2, i2

    def out_phase():
        top = (jnp.full((8, 1), -jnp.inf, f32), jnp.zeros((8, 1), jnp.int32),
               jnp.full((8, 1), -jnp.inf, f32), jnp.ones((8, 1), jnp.int32))
        return lax.fori_loop(0, NOB, out_body, top)

    def ffn(layer, top):
        m1, i1, m2, i2 = top
        cv = jnp.concatenate([m1, m2], axis=0)
        ci = jnp.concatenate([i1, i2], axis=0)
        v1 = jnp.max(cv, axis=0, keepdims=True)
        j1 = jnp.min(jnp.where(cv == v1, ci, S), axis=0, keepdims=True)
        cv2 = jnp.where(ci == j1, -jnp.inf, cv)
        v2 = jnp.max(cv2, axis=0, keepdims=True)
        j2 = jnp.min(jnp.where(cv2 == v2, ci, S), axis=0, keepdims=True)
        t1 = jnp.clip(j1[0, 0], 0, S - 1)
        t2 = jnp.clip(j2[0, 0], 0, S - 1)
        b1 = pl.ds(pl.multiple_of((t1 // 8) * 8, 8), 8)
        b2 = pl.ds(pl.multiple_of((t2 // 8) * 8, 8), 8)

        def two(ref):
            return jnp.concatenate([ref[b1, :], ref[b2, :]], axis=0)
        xm = (two(x1_sc) - two(mean_sc)[:, 0:1]) * two(rs_sc)[:, 0:1]
        xs = xm.astype(bf16)
        base = two(x1_sc) + xm

        NCH = 16
        CH = S // NCH
        never = jnp.full((CH, 1), zero, jnp.int32) != 0

        def mod_rows(n, tok):
            rows = slice(n * CH, (n + 1) * CH)
            x1 = x1_sc[rows, :]
            mn = mean_sc[rows, 0:1]
            if tok is not None:
                mn = jnp.where(never, tok, mn)
            c = x1 - mn
            xb_sc[rows, :] = (x1 + c * rs_sc[rows, 0:1]).astype(bf16)
            xn_sc[rows, :] = (c * kn_sc[rows, 0:1]).astype(bf16)
            if (n + 1) % (NCH // NOUT) == 0:
                @pl.when(layer == 1)
                def _():
                    out_copy(n // (NCH // NOUT)).start()

        y = None
        mod_rows(0, None)
        mod_rows(1, None)
        for j in range(F // FC):
            gg = jnp.dot(xs, wg_sc[:, FC * j:FC * (j + 1)], preferred_element_type=f32)
            uu = jnp.dot(xs, wu_sc[:, FC * j:FC * (j + 1)], preferred_element_type=f32)
            hh = (gg * _sigmoid(gg) * uu).astype(bf16)
            t = jnp.dot(hh, wd_sc[FC * j:FC * (j + 1), :], preferred_element_type=f32)
            y = t if y is None else y + t
            mod_rows(2 + j, jnp.broadcast_to(gg[0:1, 0:1], (CH, 1)))
        r8 = lax.broadcasted_iota(jnp.int32, (8, D), 0)
        y1 = jnp.where(r8 == t1 % 8, y[0:8] * _sigmoid(v1), 0.0)
        y2 = jnp.where(r8 == t2 % 8, y[8:16] * _sigmoid(v2), 0.0)
        same = t1 // 8 == t2 // 8
        n1 = base[0:8] + (y1 + jnp.where(same, y2, 0.0))
        n2 = base[8:16] + (y2 + jnp.where(same, y1, 0.0))

        @pl.when(layer == 1)
        def _():
            for i in range(NOUT):
                out_copy(i).wait()

        for b, xx in ((b1, n1), (b2, n2)):
            xb_sc[b, :] = xx.astype(bf16)
            cc = xx - jnp.mean(xx, axis=-1, keepdims=True)
            xn_sc[b, :] = (cc * lax.rsqrt(jnp.mean(cc * cc, axis=-1, keepdims=True) + EPS)).astype(bf16)

        @pl.when(layer == 1)
        def _():
            c1 = pltpu.make_async_copy(xb_sc.at[b1, :], out_hbm.at[b1, :], sems.at[7])
            c1.start()

            @pl.when(jnp.logical_not(same))
            def _():
                c2 = pltpu.make_async_copy(xb_sc.at[b2, :], out_hbm.at[b2, :], sems.at[8])
                c2.start()
                c2.wait()
            c1.wait()

    def prep_k_piece(n, c):
        for part in range(1 << LEV):
            wk_copy(n, part).wait()
        for m in range(8 // NWK):
            _prep(tk_sc, wk_sc, n * (8 // NWK) + m, 8, False)
        return c

    lax.fori_loop(0, NRB, ln_input, 0)
    lax.fori_loop(0, NWK, prep_k_piece, 0)

    def layer_body(layer, carry):
        first = layer == 0
        lax.fori_loop(0, NRB, functools.partial(proj_k_body, layer), 0)

        @pl.when(first)
        def _():
            cp["wq"].wait()
            prep_tr(tq_sc, wq_sc)
        lax.fori_loop(0, NRB, functools.partial(proj_q_body, layer), 0)

        @pl.when(first)
        def _():
            cp["wv"].wait()
            prep_tr(tv_sc, wv_sc)
        lax.fori_loop(0, NRB, proj_v_body, 0)
        attn_phase()

        @pl.when(first)
        def _():
            cp["wo"].wait()
            cp["wr"].wait()
            prep_nat(to_sc, wo_sc)
        top = out_phase()

        @pl.when(first)
        def _():
            cp["wg"].wait()
            cp["wu"].wait()
            cp["wd"].wait()
        ffn(layer, top)
        return carry

    lax.fori_loop(0, 2, layer_body, 0)


@jax.jit
def pallas_interleave_layers__memory_aug_infini_attn__moe_arch_mod__prompt_kernel(
    A_x: jax.Array,
    A_wq: jax.Array,
    A_wk: jax.Array,
    A_wv: jax.Array,
    A_wo: jax.Array,
    A_beta: jax.Array,
    B_x: jax.Array,
    B_w_r: jax.Array,
    B_w_gate: jax.Array,
    B_w_up: jax.Array,
    B_w_down: jax.Array,
):
    del B_x
    x = A_x.reshape(S, D)
    zero = jnp.zeros((1,), jnp.int32)
    beta = A_beta.astype(f32)
    wr = B_w_r.reshape(1, D)
    any_spec = pl.BlockSpec(memory_space=pl.ANY)
    smem_spec = pl.BlockSpec(memory_space=pltpu.SMEM)
    V = pltpu.VMEM
    scratch = [
        V((S, D), f32),
        V((S, D), bf16),
        V((S, D), bf16),
        V((S, 128), f32), V((S, 128), f32), V((S, 128), f32),
    ] + [V((NP, BD // 2, BD), u32)] * 4 + [
        V((D, D), bf16), V((D, D), bf16), V((D, D), bf16), V((D, D), bf16),
        V((D, D), bf16),
        V((1, D), bf16),
        V((D, F), bf16), V((D, F), bf16), V((F, D), bf16),
        V((G, S, 128), bf16), V((G, S, 128), bf16),
        V((NRB, G, 128, RB), bf16), V((NRB, G, 128, RB), bf16), V((NRB, G, 128, RB), bf16),
        V((G, S, 128), bf16),
        V((NRB, G, 8, 128), f32),
        V((H, 8, 128), f32),
        V((T, 4 * T), f32),
        pltpu.SemaphoreType.DMA((9,)),
        pltpu.SemaphoreType.DMA((NOUT,)),
        pltpu.SemaphoreType.DMA((NRB,)),
        pltpu.SemaphoreType.DMA((NWK, 1 << LEV)),
    ] + [V((T, 4 * T), f32)] * NSLOT
    out = pl.pallas_call(
        _kernel,
        in_specs=[smem_spec, smem_spec] + [any_spec] * 9,
        out_specs=any_spec,
        out_shape=jax.ShapeDtypeStruct((S, D), bf16),
        scratch_shapes=scratch,
        compiler_params=pltpu.CompilerParams(vmem_limit_bytes=120 * 1024 * 1024),
    )(zero, beta, x, A_wq, A_wk, A_wv, A_wo, wr, B_w_gate, B_w_up, B_w_down)
    return out.reshape(1, S, D)
```

```python
import functools
import itertools

import jax
import jax.numpy as jnp
from jax import lax
import jax.experimental.pallas as pl
import jax.experimental.pallas.tpu as pltpu

S, D, H, DH, NSEG, L, F = 2048, 1024, 32, 32, 4, 512, 3584
G = 8
LEV = 2
NP = 7 ** LEV
BD = D >> LEV
HD = D // 2
RB = 128 << LEV
NRB = S // RB
OB = 1024
NOB = S // OB
NOUT = 16
FC = 256
NWK = 4
T = 128
LAG = 5
NSLOT = 5
EPS = 1e-05
LOG2E = 1.4426950408889634
QSCALE = (DH ** -0.5) * LOG2E
NEG = -1e30
NT = (((1,), (1,)), ((), ()))
ORDER = (2, 4, 3, 1, 0, 6, 5)

f32 = jnp.float32
bf16 = jnp.bfloat16
u32 = jnp.uint32


def _phi(t):
    return jnp.where(t > 0, t + 1.0, jnp.exp(t))


def _sigmoid(t):
    return 1.0 / (1.0 + jnp.exp(-t))


def _pk(x):
    return pltpu.bitcast(x, u32)


def _upk(x):
    return pltpu.bitcast(x, bf16)


def _row_fold(x, op):
    parts = [x[8 * r:8 * r + 8] for r in range(x.shape[0] // 8)]
    while len(parts) > 1:
        parts = [op(parts[i], parts[i + 1]) if i + 1 < len(parts) else parts[i] for i in range(0, len(parts), 2)]
    return parts[0]


def _quads(x):
    h, w = x.shape[0] // 2, x.shape[1] // 2
    return x[:h, :w], x[:h, w:], x[h:, :w], x[h:, w:]


def _lhs_ops(x, lev):
    if lev == 0:
        return [x.astype(bf16)]
    x00, x01, x10, x11 = _quads(x)
    a00, a01, a10, a11 = (t.astype(f32) for t in (x00, x01, x10, x11))
    ops = (a00 + a11, a10 + a11, x00, x11, a00 + a01, a10 - a00, a01 - a11)
    return [o for t in ops for o in _lhs_ops(t, lev - 1)]


def _rhs_ops(w, lev):
    if lev == 0:
        return [w[()].astype(bf16)]

    def sub(r, c):
        return {p[1:]: v for p, v in w.items() if p[0] == (r, c)}

    def add(x, y, sign=1):
        return {p: (x[p].astype(f32) + y[p].astype(f32) if sign > 0 else x[p].astype(f32) - y[p].astype(f32))
                for p in x}
    b11, b12, b21, b22 = sub(0, 0), sub(0, 1), sub(1, 0), sub(1, 1)
    ops = (add(b11, b22), b11, add(b12, b22, -1), add(b21, b11, -1), b22, add(b11, b12), add(b21, b22))
    return [o for t in ops for o in _rhs_ops(t, lev - 1)]


def _offsets(path):
    r = sum(rc[0] * (D >> (i + 1)) for i, rc in enumerate(path))
    c = sum(rc[1] * (D >> (i + 1)) for i, rc in enumerate(path))
    return r, c


def _prep(t_ref, w_ref, n, nch, transposed):
    ch = BD // nch
    w = {}
    for path in itertools.product(((0, 0), (0, 1), (1, 0), (1, 1)), repeat=LEV):
        r, c = _offsets(path)
        if transposed:
            r, c = c, r
        w[path] = w_ref[pl.ds(pl.multiple_of(r + n * ch, ch), ch), c:c + BD]
    rows = pl.ds(pl.multiple_of(n * (ch // 2), ch // 2), ch // 2)
    for i, t in enumerate(_rhs_ops(w, LEV)):
        t_ref[i, rows, :] = _pk(t)


def _combine(M):
    m1, m2, m3, m4, m5, m6, m7 = M
    return m1 + m4 - m5 + m7, m3 + m5, m2 + m4, m1 - m2 + m3 + m6


def _strassen(mm, transposed):
    def assemble(c11, c12, c21, c22):
        if transposed:
            c12, c21 = c21, c12
        return jnp.concatenate([jnp.concatenate([c11, c12], axis=1), jnp.concatenate([c21, c22], axis=1)], axis=0)

    def rec(base, lev):
        M = [None] * 7
        for i in ORDER:
            M[i] = mm(base * 7 + i) if lev == 1 else assemble(*rec(base * 7 + i, lev - 1)[0])
        return _combine(M), M
    return rec(0, LEV)


def _kernel(zero_smem, beta_ref, x_hbm, wq_hbm, wk_hbm, wv_hbm, wo_hbm, wr_hbm,
            wg_hbm, wu_hbm, wd_hbm, out_hbm,
            x1_sc, xb_sc, xn_sc, mean_sc, rs_sc, kn_sc, tk_sc, tq_sc, tv_sc, to_sc,
            wq_sc, wk_sc, wv_sc, wo_sc, wT_sc, wr_sc,
            wg_sc, wu_sc, wd_sc, k_sc, pk_sc, qT_sc, pqT_sc, vT_sc, o_sc, z_sc,
            gt_sc, am_sc, sems, osems, xsems, ksems, *s_sc):
    cp = {
        "wq": pltpu.make_async_copy(wq_hbm, wq_sc, sems.at[0]),
        "wv": pltpu.make_async_copy(wv_hbm, wv_sc, sems.at[1]),
        "wo": pltpu.make_async_copy(wo_hbm, wo_sc, sems.at[2]),
        "wr": pltpu.make_async_copy(wr_hbm, wr_sc, sems.at[3]),
        "wg": pltpu.make_async_copy(wg_hbm, wg_sc, sems.at[4]),
        "wu": pltpu.make_async_copy(wu_hbm, wu_sc, sems.at[5]),
        "wd": pltpu.make_async_copy(wd_hbm, wd_sc, sems.at[6]),
    }

    def x_copy(rb):
        rows = pl.ds(pl.multiple_of(rb * RB, RB), RB)
        return pltpu.make_async_copy(x_hbm.at[rows, :], xb_sc.at[rows, :], xsems.at[rb])

    def wk_copy(n, part):
        rows = pl.ds(part * BD + n * (BD // NWK), BD // NWK)
        return pltpu.make_async_copy(wk_hbm.at[rows, :], wk_sc.at[rows, :], ksems.at[n, part])

    def out_copy(i):
        rows = pl.ds(i * (S // NOUT), S // NOUT)
        return pltpu.make_async_copy(xb_sc.at[rows, :], out_hbm.at[rows, :], osems.at[i])

    for rb in range(NRB):
        x_copy(rb).start()
    zero = zero_smem[0]

    am_sc[...] = jnp.zeros((T, 4 * T), f32)

    gates = _sigmoid(beta_ref[...].reshape(1, H).astype(f32))
    for h in range(H):
        gt_sc[h] = jnp.broadcast_to(gates[:, h:h + 1], (8, 128))

    row = lax.broadcasted_iota(jnp.int32, (T, T), 0)
    col = lax.broadcasted_iota(jnp.int32, (T, T), 1)
    cmask = row <= col
    hmask = (row // 32) == (col // 32)
    zrow = lax.broadcasted_iota(jnp.int32, (32, T), 0)
    zcol = lax.broadcasted_iota(jnp.int32, (32, T), 1)
    zmask = (zrow // 8) == (zcol // 32)

    def rows_of(rb):
        return pl.ds(pl.multiple_of(rb * RB, RB), RB)

    def prep_nat(t_ref, w_ref):
        lax.fori_loop(0, 8, lambda n, c: (_prep(t_ref, w_ref, n, 8, False), c)[1], 0)

    def prep_tr(t_ref, w_ref):
        for j in range(4):
            for i in range(4):
                wT_sc[256 * j:256 * (j + 1), 256 * i:256 * (i + 1)] = w_ref[256 * i:256 * (i + 1), 256 * j:256 * (j + 1)].T
        lax.fori_loop(0, 8, lambda n, c: (_prep(t_ref, wT_sc, n, 8, True), c)[1], 0)

    QUADS = lambda c: ((c[1], 0, 1), (c[2], 1, 0), (c[0], 0, 0), (c[3], 1, 1))

    def ln_input(rb, carry):
        x_copy(rb).wait()

        @pl.when(rb == 0)
        def _():
            for n in range(NWK):
                for part in range(1 << LEV):
                    wk_copy(n, part).start()
        for n in range(RB // 128):
            rows = pl.ds(pl.multiple_of(rb * RB + n * 128, 128), 128)
            x = xb_sc[rows, :].astype(f32)
            c = x - jnp.mean(x, axis=-1, keepdims=True)
            v = jnp.mean(c * c, axis=-1, keepdims=True)
            xn_sc[rows, :] = (c * lax.rsqrt(v + EPS)).astype(bf16)
        return carry

    def proj_k_body(layer, rb, carry):
        for j, name in enumerate(("wq", "wv", "wo", "wr")):
            @pl.when(jnp.logical_and(layer == 0, rb == j))
            def _():
                cp[name].start()
        h = RB // 2
        r0 = pl.multiple_of(rb * RB, RB)
        A = _lhs_ops(xn_sc[rows_of(rb), :], LEV)
        c, _ = _strassen(lambda i: jnp.dot(A[i], _upk(tk_sc[i]), preferred_element_type=f32), False)
        zp = [None, None]
        for kk, th, nh in QUADS(c):
            pk = _phi(kk)
            zz = _row_fold(pk, jnp.add)
            zp[nh] = zz if zp[nh] is None else zp[nh] + zz
            rows = pl.ds(pl.multiple_of(r0 + th * h, h), h)
            for g in range(G // 2):
                k_sc[4 * nh + g, rows, :] = kk[:, 128 * g:128 * (g + 1)].astype(bf16)
                pk_sc[4 * nh + g, rows, :] = pk[:, 128 * g:128 * (g + 1)].astype(bf16)
        for nh in range(2):
            for g in range(G // 2):
                z_sc[rb, 4 * nh + g] = zp[nh][:, 128 * g:128 * (g + 1)]
        return carry

    def proj_q_body(layer, rb, carry):
        @pl.when(jnp.logical_and(layer == 0, rb == 0))
        def _():
            for name in ("wg", "wu", "wd"):
                cp[name].start()
        h = RB // 2
        A = _lhs_ops(xn_sc[rows_of(rb), :], LEV)
        c, _ = _strassen(lambda i: lax.dot_general(_upk(tq_sc[i]), A[i], NT, preferred_element_type=f32), True)
        for qq, th, nh in QUADS(c):
            pq = _phi(qq)
            for g in range(G // 2):
                qT_sc[rb, 4 * nh + g, :, th * h:(th + 1) * h] = (qq[128 * g:128 * (g + 1)] * QSCALE).astype(bf16)
                pqT_sc[rb, 4 * nh + g, :, th * h:(th + 1) * h] = pq[128 * g:128 * (g + 1)].astype(bf16)
        return carry

    def proj_v_body(rb, carry):
        h = RB // 2
        A = _lhs_ops(xn_sc[rows_of(rb), :], LEV)
        c, _ = _strassen(lambda i: lax.dot_general(_upk(tv_sc[i]), A[i], NT, preferred_element_type=f32), True)
        for vv, th, nh in QUADS(c):
            for g in range(G // 2):
                vT_sc[rb, 4 * nh + g, :, th * h:(th + 1) * h] = vv[128 * g:128 * (g + 1)].astype(bf16)
        return carry

    TILES = [(s, i) for s in range(NSEG) for i in (3, 2, 1, 0)]
    STREAM = [(t, c) for t, (s, i) in enumerate(TILES) for c in range(i + 1)]
    NPOS = len(STREAM)

    def sref(k, h):
        return s_sc[k % NSLOT].at[pl.ds(pl.multiple_of(zero, 8), T), T * h:T * (h + 1)]

    def tcols(ref, g, t0, n, rows=slice(None)):
        parts = []
        for t in range(t0, t0 + n, min(n, RB)):
            parts.append(ref[t // RB, g, rows, t % RB:t % RB + min(n, RB)])
        return parts[0] if len(parts) == 1 else jnp.concatenate(parts, axis=1)

    def q_weights(g, s, i):
        QT = tcols(qT_sc, g, s * L + i * T, T)
        z = jnp.zeros((32, T), bf16)
        return jnp.concatenate(
            [jnp.concatenate([QT[32 * h:32 * h + 32] if hh == h else z for hh in range(4)], axis=0)
             for h in range(4)], axis=1)

    def qk(g, k, m):
        t, c = STREAM[k]
        s, i = TILES[t]
        k0 = s * L + c * T
        K = k_sc[g, k0:k0 + T, :]
        S4 = jnp.dot(K, q_weights(g, s, i), preferred_element_type=f32)
        out = []
        for h in range(4):
            Sx = S4[:, T * h:T * (h + 1)]
            if c == i:
                Sx = jnp.where(cmask, Sx, NEG)
            sref(k, h)[...] = Sx
            mm = Sx[0:8]
            for r in range(1, 16):
                mm = jnp.maximum(mm, Sx[8 * r:8 * r + 8])
            mm = mm if c == 0 else jnp.maximum(m[h], mm)
            if c == i:
                mm = jnp.broadcast_to(jnp.max(mm, axis=0, keepdims=True), (8, T))
            out.append(mm)
        return out

    def attn_prologue():
        m = {}
        for k in range(LAG):
            t = STREAM[k][0]
            m[t] = qk(0, k, m.get(t))
        return tuple(m[STREAM[0][0]]) + tuple(m[STREAM[LAG - 1][0]])

    def finish(g, s, i, O, l):
        outs = []
        for h in range(4):
            lt = jnp.sum(l[h], axis=0, keepdims=True)
            gt = jnp.concatenate([gt_sc[4 * g + h]] * 4, axis=0)
            o = O[h] * ((1.0 - gt) * (1.0 / lt))
            if s > 0:
                o = o + am_sc[32 * h:32 * h + 32, i * T:(i + 1) * T]
            outs.append(o)
        ot = jnp.concatenate(outs, axis=0).astype(bf16)
        r0 = s * L + i * T
        o_sc[g, r0:r0 + T, :] = ot.T

    def attn_body(g, carry):
        gn = jnp.minimum(g + 1, G - 1)
        m = {STREAM[0][0]: list(carry[0:4]), STREAM[LAG - 1][0]: list(carry[4:8])}
        l, O, P, M, mn = {}, {}, {}, {}, {}

        def mem_read(s):
            zs = z_sc[0, g]
            for rb in range(1, s * L // RB):
                zs = zs + z_sc[rb, g]
            zs = jnp.sum(zs, axis=0, keepdims=True)
            zrows = jnp.where(zmask, zs, 0.0).astype(bf16)
            mbd = jnp.where(hmask, M[0], 0.0).astype(bf16)
            lhs = jnp.concatenate([mbd, zrows], axis=0)
            pq = tcols(pqT_sc, g, s * L, L)
            nd = jnp.dot(lhs, pq, preferred_element_type=f32)
            for h in range(4):
                den = nd[128 + 8 * h:128 + 8 * h + 8] + 1e-06
                gd = jnp.concatenate([gt_sc[4 * g + h]] * 4, axis=1) / den
                am_sc[32 * h:32 * h + 32, :] = nd[32 * h:32 * h + 32] * jnp.concatenate([gd] * 4, axis=0)

        def mem_write(s):
            vt = tcols(vT_sc, g, s * L, L)
            pk = pk_sc[g, s * L:(s + 1) * L, :]
            inc = jnp.dot(vt, pk, preferred_element_type=f32)
            M[0] = inc if s == 0 else M[0] + inc

        def ex(k):
            t, c = STREAM[k]
            out = []
            for h in range(4):
                Pp = jnp.exp2(sref(k, h)[...] - jnp.concatenate([m[t][h]] * (T // 8), axis=0))
                a = Pp[0:8] + Pp[8:16]
                b = Pp[16:24] + Pp[24:32]
                for r in range(2, 8, 2):
                    a = a + (Pp[16 * r:16 * r + 8] + Pp[16 * r + 8:16 * r + 16])
                    b = b + (Pp[16 * r + 16:16 * r + 24] + Pp[16 * r + 24:16 * r + 32])
                ll = a + b
                if c == 0:
                    l.setdefault(t, [None] * 4)[h] = ll
                else:
                    l[t][h] = l[t][h] + ll
                out.append(Pp.astype(bf16))
            P[k] = out

        def pv(k):
            t, c = STREAM[k]
            s, i = TILES[t]
            if c == 0:
                O[t] = [None] * 4
            for h in range(4):
                vt = tcols(vT_sc, g, s * L + c * T, T, slice(32 * h, 32 * h + 32))
                o = jnp.dot(vt, P[k][h], preferred_element_type=f32)
                O[t][h] = o if O[t][h] is None else O[t][h] + o
            del P[k]

        finish(jnp.maximum(g - 1, 0), NSEG - 1, 0, carry[8:12], carry[12:16])
        done = None
        for j in range(NPOS):
            ex(j)
            k = j + LAG
            if k < NPOS:
                t = STREAM[k][0]
                m[t] = qk(g, k, m.get(t))
            else:
                t = STREAM[k - NPOS][0]
                mn[t] = qk(gn, k - NPOS, mn.get(t))
            pv(j)
            if done is not None:
                s, i = TILES[done]
                finish(g, s, i, O[done], l[done])
                if i == 0:
                    mem_read(s + 1)
                done = None
            t, c = STREAM[j]
            if c == TILES[t][1]:
                done = t
                if TILES[t][1] == 3 and TILES[t][0] < NSEG - 1:
                    mem_write(TILES[t][0])
        return (tuple(mn[STREAM[0][0]]) + tuple(mn[STREAM[LAG - 1][0]]) + tuple(O[done]) + tuple(l[done]))

    def attn_phase():
        init = attn_prologue() + (jnp.zeros((32, T), f32),) * 4 + (jnp.ones((8, T), f32),) * 4
        carry = lax.fori_loop(0, G, attn_body, init)
        finish(G - 1, NSEG - 1, 0, carry[8:12], carry[12:16])

    def out_body(ob_i, top):
        wr = wr_sc[...].reshape(1, D).astype(f32)
        wr_sum = jnp.sum(wr, axis=-1, keepdims=True)
        h = RB // 2
        m1, i1, m2, i2 = top
        for k in range(OB // RB):
            r0 = pl.multiple_of(ob_i * OB + k * RB, RB)
            ob = jnp.concatenate([o_sc[g, pl.ds(r0, RB), :] for g in range(G)], axis=1)
            A = _lhs_ops(ob, LEV)
            c, _ = _strassen(lambda i: jnp.dot(A[i], _upk(to_sc[i]), preferred_element_type=f32), False)
            acc = [[None] * 3, [None] * 3]
            for cc, th, nh in QUADS(c):
                rows = pl.ds(pl.multiple_of(r0 + th * h, h), h)
                cols = slice(nh * HD, (nh + 1) * HD)
                x1 = xb_sc[rows, cols].astype(f32) + cc
                x1_sc[rows, cols] = x1
                s1, s2, st = acc[th]
                for n in range(HD // 128):
                    d = x1[:, 128 * n:128 * (n + 1)]
                    s1 = d if s1 is None else s1 + d
                    s2 = d * d if s2 is None else s2 + d * d
                    t = d * wr[:, nh * HD + 128 * n:nh * HD + 128 * (n + 1)]
                    st = t if st is None else st + t
                acc[th] = [s1, s2, st]
            for th in range(2):
                s1, s2, st = acc[th]
                rows = pl.ds(pl.multiple_of(r0 + th * h, h), h)
                mean = jnp.sum(s1, axis=-1, keepdims=True) * (1.0 / D)
                v = jnp.maximum(jnp.sum(s2, axis=-1, keepdims=True) * (1.0 / D) - mean * mean, 0.0)
                rs = lax.rsqrt(v + EPS)
                r = rs * (jnp.sum(st, axis=-1, keepdims=True) - mean * wr_sum)
                r = r.astype(bf16).astype(f32)
                mean_sc[rows, :] = jnp.broadcast_to(mean, (h, 128))
                rs_sc[rows, :] = jnp.broadcast_to(rs, (h, 128))
                a = 1.0 + rs
                kn_sc[rows, :] = jnp.broadcast_to(a * lax.rsqrt(v * (a * a) + EPS), (h, 128))
                sub = lax.broadcasted_iota(jnp.int32, (8, 1), 0) + (r0 + th * h)
                for j in range(h // 8):
                    rj = r[8 * j:8 * j + 8]
                    idx = sub + 8 * j
                    g1 = rj > m1
                    g2 = rj > m2
                    m2 = jnp.where(g1, m1, jnp.where(g2, rj, m2))
                    i2 = jnp.where(g1, i1, jnp.where(g2, idx, i2))
                    m1 = jnp.where(g1, rj, m1)
                    i1 = jnp.where(g1, idx, i1)
        return m1, i1, m2, i2

    def out_phase():
        top = (jnp.full((8, 1), -jnp.inf, f32), jnp.zeros((8, 1), jnp.int32),
               jnp.full((8, 1), -jnp.inf, f32), jnp.ones((8, 1), jnp.int32))
        return lax.fori_loop(0, NOB, out_body, top)

    def ffn(layer, top):
        m1, i1, m2, i2 = top
        cv = jnp.concatenate([m1, m2], axis=0)
        ci = jnp.concatenate([i1, i2], axis=0)
        v1 = jnp.max(cv, axis=0, keepdims=True)
        j1 = jnp.min(jnp.where(cv == v1, ci, S), axis=0, keepdims=True)
        cv2 = jnp.where(ci == j1, -jnp.inf, cv)
        v2 = jnp.max(cv2, axis=0, keepdims=True)
        j2 = jnp.min(jnp.where(cv2 == v2, ci, S), axis=0, keepdims=True)
        t1 = jnp.clip(j1[0, 0], 0, S - 1)
        t2 = jnp.clip(j2[0, 0], 0, S - 1)
        b1 = pl.ds(pl.multiple_of((t1 // 8) * 8, 8), 8)
        b2 = pl.ds(pl.multiple_of((t2 // 8) * 8, 8), 8)

        def two(ref):
            return jnp.concatenate([ref[b1, :], ref[b2, :]], axis=0)
        xm = (two(x1_sc) - two(mean_sc)[:, 0:1]) * two(rs_sc)[:, 0:1]
        xs = xm.astype(bf16)
        base = two(x1_sc) + xm

        NCH = 16
        CH = S // NCH
        never = jnp.full((CH, 1), zero, jnp.int32) != 0

        def mod_rows(n, tok):
            rows = slice(n * CH, (n + 1) * CH)
            x1 = x1_sc[rows, :]
            mn = mean_sc[rows, 0:1]
            if tok is not None:
                mn = jnp.where(never, tok, mn)
            c = x1 - mn
            xb_sc[rows, :] = (x1 + c * rs_sc[rows, 0:1]).astype(bf16)
            xn_sc[rows, :] = (c * kn_sc[rows, 0:1]).astype(bf16)
            if (n + 1) % (NCH // NOUT) == 0:
                @pl.when(layer == 1)
                def _():
                    out_copy(n // (NCH // NOUT)).start()

        y = None
        mod_rows(0, None)
        mod_rows(1, None)
        for j in range(F // FC):
            gg = jnp.dot(xs, wg_sc[:, FC * j:FC * (j + 1)], preferred_element_type=f32)
            uu = jnp.dot(xs, wu_sc[:, FC * j:FC * (j + 1)], preferred_element_type=f32)
            hh = (gg * _sigmoid(gg) * uu).astype(bf16)
            t = jnp.dot(hh, wd_sc[FC * j:FC * (j + 1), :], preferred_element_type=f32)
            y = t if y is None else y + t
            if j < 7:
                mod_rows(2 + 2 * j, jnp.broadcast_to(gg[0:1, 0:1], (CH, 1)))
                mod_rows(3 + 2 * j, jnp.broadcast_to(t[0:1, 0:1], (CH, 1)))
        r8 = lax.broadcasted_iota(jnp.int32, (8, D), 0)
        y1 = jnp.where(r8 == t1 % 8, y[0:8] * _sigmoid(v1), 0.0)
        y2 = jnp.where(r8 == t2 % 8, y[8:16] * _sigmoid(v2), 0.0)
        same = t1 // 8 == t2 // 8
        n1 = base[0:8] + (y1 + jnp.where(same, y2, 0.0))
        n2 = base[8:16] + (y2 + jnp.where(same, y1, 0.0))

        @pl.when(layer == 1)
        def _():
            for i in range(NOUT):
                out_copy(i).wait()

        for b, xx in ((b1, n1), (b2, n2)):
            xb_sc[b, :] = xx.astype(bf16)
            cc = xx - jnp.mean(xx, axis=-1, keepdims=True)
            xn_sc[b, :] = (cc * lax.rsqrt(jnp.mean(cc * cc, axis=-1, keepdims=True) + EPS)).astype(bf16)

        @pl.when(layer == 1)
        def _():
            c1 = pltpu.make_async_copy(xb_sc.at[b1, :], out_hbm.at[b1, :], sems.at[7])
            c1.start()

            @pl.when(jnp.logical_not(same))
            def _():
                c2 = pltpu.make_async_copy(xb_sc.at[b2, :], out_hbm.at[b2, :], sems.at[8])
                c2.start()
                c2.wait()
            c1.wait()

    def prep_k_piece(n, c):
        for part in range(1 << LEV):
            wk_copy(n, part).wait()
        for m in range(8 // NWK):
            _prep(tk_sc, wk_sc, n * (8 // NWK) + m, 8, False)
        return c

    lax.fori_loop(0, NRB, ln_input, 0)
    lax.fori_loop(0, NWK, prep_k_piece, 0)

    def layer_body(layer, carry):
        first = layer == 0
        lax.fori_loop(0, NRB, functools.partial(proj_k_body, layer), 0)

        @pl.when(first)
        def _():
            cp["wq"].wait()
            prep_tr(tq_sc, wq_sc)
        lax.fori_loop(0, NRB, functools.partial(proj_q_body, layer), 0)

        @pl.when(first)
        def _():
            cp["wv"].wait()
            prep_tr(tv_sc, wv_sc)
        lax.fori_loop(0, NRB, proj_v_body, 0)
        attn_phase()

        @pl.when(first)
        def _():
            cp["wo"].wait()
            cp["wr"].wait()
            prep_nat(to_sc, wo_sc)
        top = out_phase()

        @pl.when(first)
        def _():
            cp["wg"].wait()
            cp["wu"].wait()
            cp["wd"].wait()
        ffn(layer, top)
        return carry

    lax.fori_loop(0, 2, layer_body, 0)


@jax.jit
def pallas_interleave_layers__memory_aug_infini_attn__moe_arch_mod__prompt_kernel(
    A_x: jax.Array,
    A_wq: jax.Array,
    A_wk: jax.Array,
    A_wv: jax.Array,
    A_wo: jax.Array,
    A_beta: jax.Array,
    B_x: jax.Array,
    B_w_r: jax.Array,
    B_w_gate: jax.Array,
    B_w_up: jax.Array,
    B_w_down: jax.Array,
):
    del B_x
    x = A_x.reshape(S, D)
    zero = jnp.zeros((1,), jnp.int32)
    any_spec = pl.BlockSpec(memory_space=pl.ANY)
    smem_spec = pl.BlockSpec(memory_space=pltpu.SMEM)
    V = pltpu.VMEM
    scratch = [
        V((S, D), f32),
        V((S, D), bf16),
        V((S, D), bf16),
        V((S, 128), f32), V((S, 128), f32), V((S, 128), f32),
    ] + [V((NP, BD // 2, BD), u32)] * 4 + [
        V((D, D), bf16), V((D, D), bf16), V((D, D), bf16), V((D, D), bf16),
        V((D, D), bf16),
        V((D,), bf16),
        V((D, F), bf16), V((D, F), bf16), V((F, D), bf16),
        V((G, S, 128), bf16), V((G, S, 128), bf16),
        V((NRB, G, 128, RB), bf16), V((NRB, G, 128, RB), bf16), V((NRB, G, 128, RB), bf16),
        V((G, S, 128), bf16),
        V((NRB, G, 8, 128), f32),
        V((H, 8, 128), f32),
        V((T, 4 * T), f32),
        pltpu.SemaphoreType.DMA((9,)),
        pltpu.SemaphoreType.DMA((NOUT,)),
        pltpu.SemaphoreType.DMA((NRB,)),
        pltpu.SemaphoreType.DMA((NWK, 1 << LEV)),
    ] + [V((T, 4 * T), f32)] * NSLOT
    out = pl.pallas_call(
        _kernel,
        in_specs=[smem_spec, pl.BlockSpec(memory_space=pltpu.VMEM)] + [any_spec] * 9,
        out_specs=any_spec,
        out_shape=jax.ShapeDtypeStruct((S, D), bf16),
        scratch_shapes=scratch,
        compiler_params=pltpu.CompilerParams(vmem_limit_bytes=120 * 1024 * 1024),
    )(zero, A_beta, x, A_wq, A_wk, A_wv, A_wo, B_w_r, B_w_gate, B_w_up, B_w_down)
    return out.reshape(1, S, D)
```

```python
import functools
import itertools

import jax
import jax.numpy as jnp
from jax import lax
import jax.experimental.pallas as pl
import jax.experimental.pallas.tpu as pltpu

S, D, H, DH, NSEG, L, F = 2048, 1024, 32, 32, 4, 512, 3584
G = 8
LEV = 2
NP = 7 ** LEV
BD = D >> LEV
HD = D // 2
RB = 128 << LEV
NRB = S // RB
OB = 1024
NOB = S // OB
NOUT = 16
FC = 256
NWK = 4
T = 128
LAG = 5
NSLOT = 5
EPS = 1e-05
LOG2E = 1.4426950408889634
QSCALE = (DH ** -0.5) * LOG2E
NEG = -1e30
NT = (((1,), (1,)), ((), ()))
ORDER = (2, 4, 3, 1, 0, 6, 5)

f32 = jnp.float32
bf16 = jnp.bfloat16
u32 = jnp.uint32


def _phi(t):
    return jnp.where(t > 0, t + 1.0, jnp.exp(t))


def _sigmoid(t):
    return 1.0 / (1.0 + jnp.exp(-t))


def _pk(x):
    return pltpu.bitcast(x, u32)


def _upk(x):
    return pltpu.bitcast(x, bf16)


def _row_fold(x, op):
    parts = [x[8 * r:8 * r + 8] for r in range(x.shape[0] // 8)]
    while len(parts) > 1:
        parts = [op(parts[i], parts[i + 1]) if i + 1 < len(parts) else parts[i] for i in range(0, len(parts), 2)]
    return parts[0]


def _quads(x):
    h, w = x.shape[0] // 2, x.shape[1] // 2
    return x[:h, :w], x[:h, w:], x[h:, :w], x[h:, w:]


def _lhs_ops(x, lev):
    if lev == 0:
        return [x.astype(bf16)]
    x00, x01, x10, x11 = _quads(x)
    a00, a01, a10, a11 = (t.astype(f32) for t in (x00, x01, x10, x11))
    ops = (a00 + a11, a10 + a11, x00, x11, a00 + a01, a10 - a00, a01 - a11)
    return [o for t in ops for o in _lhs_ops(t, lev - 1)]


def _rhs_ops(w, lev):
    if lev == 0:
        return [w[()].astype(bf16)]

    def sub(r, c):
        return {p[1:]: v for p, v in w.items() if p[0] == (r, c)}

    def add(x, y, sign=1):
        return {p: (x[p].astype(f32) + y[p].astype(f32) if sign > 0 else x[p].astype(f32) - y[p].astype(f32))
                for p in x}
    b11, b12, b21, b22 = sub(0, 0), sub(0, 1), sub(1, 0), sub(1, 1)
    ops = (add(b11, b22), b11, add(b12, b22, -1), add(b21, b11, -1), b22, add(b11, b12), add(b21, b22))
    return [o for t in ops for o in _rhs_ops(t, lev - 1)]


def _offsets(path):
    r = sum(rc[0] * (D >> (i + 1)) for i, rc in enumerate(path))
    c = sum(rc[1] * (D >> (i + 1)) for i, rc in enumerate(path))
    return r, c


def _prep(t_ref, w_ref, n, nch, transposed):
    ch = BD // nch
    w = {}
    for path in itertools.product(((0, 0), (0, 1), (1, 0), (1, 1)), repeat=LEV):
        r, c = _offsets(path)
        if transposed:
            r, c = c, r
        w[path] = w_ref[pl.ds(pl.multiple_of(r + n * ch, ch), ch), c:c + BD]
    rows = pl.ds(pl.multiple_of(n * (ch // 2), ch // 2), ch // 2)
    for i, t in enumerate(_rhs_ops(w, LEV)):
        t_ref[i, rows, :] = _pk(t)


def _combine(M):
    m1, m2, m3, m4, m5, m6, m7 = M
    return m1 + m4 - m5 + m7, m3 + m5, m2 + m4, m1 - m2 + m3 + m6


def _strassen(mm, transposed):
    def assemble(c11, c12, c21, c22):
        if transposed:
            c12, c21 = c21, c12
        return jnp.concatenate([jnp.concatenate([c11, c12], axis=1), jnp.concatenate([c21, c22], axis=1)], axis=0)

    def rec(base, lev):
        M = [None] * 7
        for i in ORDER:
            M[i] = mm(base * 7 + i) if lev == 1 else assemble(*rec(base * 7 + i, lev - 1)[0])
        return _combine(M), M
    return rec(0, LEV)


def _kernel(zero_smem, beta_ref, x_hbm, wq_hbm, wk_hbm, wv_hbm, wo_hbm, wr_hbm,
            wg_hbm, wu_hbm, wd_hbm, out_hbm,
            x1_sc, xb_sc, xn_sc, mean_sc, rs_sc, kn_sc, tk_sc, tq_sc, tv_sc, to_sc,
            wq_sc, wk_sc, wv_sc, wo_sc, wT_sc, wr_sc,
            wg_sc, wu_sc, wd_sc, k_sc, pk_sc, qT_sc, pqT_sc, vT_sc, o_sc, z_sc,
            gt_sc, am_sc, sems, osems, xsems, ksems, *s_sc):
    cp = {
        "wq": pltpu.make_async_copy(wq_hbm, wq_sc, sems.at[0]),
        "wv": pltpu.make_async_copy(wv_hbm, wv_sc, sems.at[1]),
        "wo": pltpu.make_async_copy(wo_hbm, wo_sc, sems.at[2]),
        "wr": pltpu.make_async_copy(wr_hbm, wr_sc, sems.at[3]),
        "wg": pltpu.make_async_copy(wg_hbm, wg_sc, sems.at[4]),
        "wu": pltpu.make_async_copy(wu_hbm, wu_sc, sems.at[5]),
        "wd": pltpu.make_async_copy(wd_hbm, wd_sc, sems.at[6]),
    }

    def x_copy(rb):
        rows = pl.ds(pl.multiple_of(rb * RB, RB), RB)
        return pltpu.make_async_copy(x_hbm.at[rows, :], xb_sc.at[rows, :], xsems.at[rb])

    def wk_copy(n, part):
        rows = pl.ds(part * BD + n * (BD // NWK), BD // NWK)
        return pltpu.make_async_copy(wk_hbm.at[rows, :], wk_sc.at[rows, :], ksems.at[n, part])

    def out_copy(i):
        rows = pl.ds(i * (S // NOUT), S // NOUT)
        return pltpu.make_async_copy(xb_sc.at[rows, :], out_hbm.at[rows, :], osems.at[i])

    x_copy(0).start()
    zero = zero_smem[0]

    am_sc[...] = jnp.zeros((T, 4 * T), f32)

    gates = _sigmoid(beta_ref[...].reshape(1, H).astype(f32))
    for h in range(H):
        gt_sc[h] = jnp.broadcast_to(gates[:, h:h + 1], (8, 128))

    row = lax.broadcasted_iota(jnp.int32, (T, T), 0)
    col = lax.broadcasted_iota(jnp.int32, (T, T), 1)
    cmask = row <= col
    hmask = (row // 32) == (col // 32)
    zrow = lax.broadcasted_iota(jnp.int32, (32, T), 0)
    zcol = lax.broadcasted_iota(jnp.int32, (32, T), 1)
    zmask = (zrow // 8) == (zcol // 32)

    def rows_of(rb):
        return pl.ds(pl.multiple_of(rb * RB, RB), RB)

    def prep_nat(t_ref, w_ref):
        lax.fori_loop(0, 8, lambda n, c: (_prep(t_ref, w_ref, n, 8, False), c)[1], 0)

    def prep_tr(t_ref, w_ref):
        for j in range(4):
            for i in range(4):
                wT_sc[256 * j:256 * (j + 1), 256 * i:256 * (i + 1)] = w_ref[256 * i:256 * (i + 1), 256 * j:256 * (j + 1)].T
        lax.fori_loop(0, 8, lambda n, c: (_prep(t_ref, wT_sc, n, 8, True), c)[1], 0)

    QUADS = lambda c: ((c[1], 0, 1), (c[2], 1, 0), (c[0], 0, 0), (c[3], 1, 1))

    def ln_input(rb):
        x_copy(rb).wait()
        if isinstance(rb, int):
            for n in range(NWK):
                for part in range(1 << LEV):
                    wk_copy(n, part).start()
        for n in range(RB // 128):
            rows = pl.ds(pl.multiple_of(rb * RB + n * 128, 128), 128)
            x = xb_sc[rows, :].astype(f32)
            c = x - jnp.mean(x, axis=-1, keepdims=True)
            v = jnp.mean(c * c, axis=-1, keepdims=True)
            xn_sc[rows, :] = (c * lax.rsqrt(v + EPS)).astype(bf16)

    def proj_k_body(layer, rb, carry):
        @pl.when(layer == 0)
        def _():
            @pl.when(rb == 0)
            def _():
                for i in range(1, NRB):
                    x_copy(i).start()
            for j, name in ((1, "wq"), (1, "wv"), (2, "wo"), (3, "wr")):
                @pl.when(rb == j)
                def _():
                    cp[name].start()

            @pl.when(rb > 0)
            def _():
                ln_input(rb)
        h = RB // 2
        r0 = pl.multiple_of(rb * RB, RB)
        A = _lhs_ops(xn_sc[rows_of(rb), :], LEV)
        c, _ = _strassen(lambda i: jnp.dot(A[i], _upk(tk_sc[i]), preferred_element_type=f32), False)
        zp = [None, None]
        for kk, th, nh in QUADS(c):
            pk = _phi(kk)
            zz = _row_fold(pk, jnp.add)
            zp[nh] = zz if zp[nh] is None else zp[nh] + zz
            rows = pl.ds(pl.multiple_of(r0 + th * h, h), h)
            for g in range(G // 2):
                k_sc[4 * nh + g, rows, :] = kk[:, 128 * g:128 * (g + 1)].astype(bf16)
                pk_sc[4 * nh + g, rows, :] = pk[:, 128 * g:128 * (g + 1)].astype(bf16)
        for nh in range(2):
            for g in range(G // 2):
                z_sc[rb, 4 * nh + g] = zp[nh][:, 128 * g:128 * (g + 1)]
        return carry

    def proj_qv_body(layer, rb, carry):
        @pl.when(jnp.logical_and(layer == 0, rb == 0))
        def _():
            for name in ("wg", "wu", "wd"):
                cp[name].start()
        h = RB // 2
        A = _lhs_ops(xn_sc[rows_of(rb), :], LEV)
        c, _ = _strassen(lambda i: lax.dot_general(_upk(tq_sc[i]), A[i], NT, preferred_element_type=f32), True)
        for qq, th, nh in QUADS(c):
            pq = _phi(qq)
            for g in range(G // 2):
                qT_sc[rb, 4 * nh + g, :, th * h:(th + 1) * h] = (qq[128 * g:128 * (g + 1)] * QSCALE).astype(bf16)
                pqT_sc[rb, 4 * nh + g, :, th * h:(th + 1) * h] = pq[128 * g:128 * (g + 1)].astype(bf16)
        c, _ = _strassen(lambda i: lax.dot_general(_upk(tv_sc[i]), A[i], NT, preferred_element_type=f32), True)
        for vv, th, nh in QUADS(c):
            for g in range(G // 2):
                vT_sc[rb, 4 * nh + g, :, th * h:(th + 1) * h] = vv[128 * g:128 * (g + 1)].astype(bf16)
        return carry

    TILES = [(s, i) for s in range(NSEG) for i in (3, 2, 1, 0)]
    STREAM = [(t, c) for t, (s, i) in enumerate(TILES) for c in range(i + 1)]
    NPOS = len(STREAM)

    def sref(k, h):
        return s_sc[k % NSLOT].at[pl.ds(pl.multiple_of(zero, 8), T), T * h:T * (h + 1)]

    def tcols(ref, g, t0, n, rows=slice(None)):
        parts = []
        for t in range(t0, t0 + n, min(n, RB)):
            parts.append(ref[t // RB, g, rows, t % RB:t % RB + min(n, RB)])
        return parts[0] if len(parts) == 1 else jnp.concatenate(parts, axis=1)

    def q_weights(g, s, i):
        QT = tcols(qT_sc, g, s * L + i * T, T)
        z = jnp.zeros((32, T), bf16)
        return jnp.concatenate(
            [jnp.concatenate([QT[32 * h:32 * h + 32] if hh == h else z for hh in range(4)], axis=0)
             for h in range(4)], axis=1)

    def qk(g, k, m):
        t, c = STREAM[k]
        s, i = TILES[t]
        k0 = s * L + c * T
        K = k_sc[g, k0:k0 + T, :]
        S4 = jnp.dot(K, q_weights(g, s, i), preferred_element_type=f32)
        out = []
        for h in range(4):
            Sx = S4[:, T * h:T * (h + 1)]
            if c == i:
                Sx = jnp.where(cmask, Sx, NEG)
            sref(k, h)[...] = Sx
            mm = Sx[0:8]
            for r in range(1, 16):
                mm = jnp.maximum(mm, Sx[8 * r:8 * r + 8])
            mm = mm if c == 0 else jnp.maximum(m[h], mm)
            if c == i:
                mm = jnp.broadcast_to(jnp.max(mm, axis=0, keepdims=True), (8, T))
            out.append(mm)
        return out

    def attn_prologue():
        m = {}
        for k in range(LAG):
            t = STREAM[k][0]
            m[t] = qk(0, k, m.get(t))
        return tuple(m[STREAM[0][0]]) + tuple(m[STREAM[LAG - 1][0]])

    def finish(g, s, i, O, l):
        outs = []
        for h in range(4):
            lt = jnp.sum(l[h], axis=0, keepdims=True)
            gt = jnp.concatenate([gt_sc[4 * g + h]] * 4, axis=0)
            o = O[h] * ((1.0 - gt) * (1.0 / lt))
            if s > 0:
                o = o + am_sc[32 * h:32 * h + 32, i * T:(i + 1) * T]
            outs.append(o)
        ot = jnp.concatenate(outs, axis=0).astype(bf16)
        r0 = s * L + i * T
        o_sc[g, r0:r0 + T, :] = ot.T

    def attn_body(g, carry):
        gn = jnp.minimum(g + 1, G - 1)
        m = {STREAM[0][0]: list(carry[0:4]), STREAM[LAG - 1][0]: list(carry[4:8])}
        l, O, P, M, mn = {}, {}, {}, {}, {}

        def mem_read(s):
            zs = z_sc[0, g]
            for rb in range(1, s * L // RB):
                zs = zs + z_sc[rb, g]
            zs = jnp.sum(zs, axis=0, keepdims=True)
            zrows = jnp.where(zmask, zs, 0.0).astype(bf16)
            mbd = jnp.where(hmask, M[0], 0.0).astype(bf16)
            lhs = jnp.concatenate([mbd, zrows], axis=0)
            pq = tcols(pqT_sc, g, s * L, L)
            nd = jnp.dot(lhs, pq, preferred_element_type=f32)
            for h in range(4):
                den = nd[128 + 8 * h:128 + 8 * h + 8] + 1e-06
                gd = jnp.concatenate([gt_sc[4 * g + h]] * 4, axis=1) / den
                am_sc[32 * h:32 * h + 32, :] = nd[32 * h:32 * h + 32] * jnp.concatenate([gd] * 4, axis=0)

        def mem_write(s):
            vt = tcols(vT_sc, g, s * L, L)
            pk = pk_sc[g, s * L:(s + 1) * L, :]
            inc = jnp.dot(vt, pk, preferred_element_type=f32)
            M[0] = inc if s == 0 else M[0] + inc

        def ex(k):
            t, c = STREAM[k]
            out = []
            for h in range(4):
                Pp = jnp.exp2(sref(k, h)[...] - jnp.concatenate([m[t][h]] * (T // 8), axis=0))
                a = Pp[0:8] + Pp[8:16]
                b = Pp[16:24] + Pp[24:32]
                for r in range(2, 8, 2):
                    a = a + (Pp[16 * r:16 * r + 8] + Pp[16 * r + 8:16 * r + 16])
                    b = b + (Pp[16 * r + 16:16 * r + 24] + Pp[16 * r + 24:16 * r + 32])
                ll = a + b
                if c == 0:
                    l.setdefault(t, [None] * 4)[h] = ll
                else:
                    l[t][h] = l[t][h] + ll
                out.append(Pp.astype(bf16))
            P[k] = out

        def pv(k):
            t, c = STREAM[k]
            s, i = TILES[t]
            if c == 0:
                O[t] = [None] * 4
            for h in range(4):
                vt = tcols(vT_sc, g, s * L + c * T, T, slice(32 * h, 32 * h + 32))
                o = jnp.dot(vt, P[k][h], preferred_element_type=f32)
                O[t][h] = o if O[t][h] is None else O[t][h] + o
            del P[k]

        finish(jnp.maximum(g - 1, 0), NSEG - 1, 0, carry[8:12], carry[12:16])
        done = None
        for j in range(NPOS):
            ex(j)
            k = j + LAG
            if k < NPOS:
                t = STREAM[k][0]
                m[t] = qk(g, k, m.get(t))
            else:
                t = STREAM[k - NPOS][0]
                mn[t] = qk(gn, k - NPOS, mn.get(t))
            pv(j)
            if done is not None:
                s, i = TILES[done]
                finish(g, s, i, O[done], l[done])
                if i == 0:
                    mem_read(s + 1)
                done = None
            t, c = STREAM[j]
            if c == TILES[t][1]:
                done = t
                if TILES[t][1] == 3 and TILES[t][0] < NSEG - 1:
                    mem_write(TILES[t][0])
        return (tuple(mn[STREAM[0][0]]) + tuple(mn[STREAM[LAG - 1][0]]) + tuple(O[done]) + tuple(l[done]))

    def attn_phase():
        init = attn_prologue() + (jnp.zeros((32, T), f32),) * 4 + (jnp.ones((8, T), f32),) * 4
        carry = lax.fori_loop(0, G, attn_body, init)
        finish(G - 1, NSEG - 1, 0, carry[8:12], carry[12:16])

    def out_body(ob_i, top):
        wr = wr_sc[...].reshape(1, D).astype(f32)
        wr_sum = jnp.sum(wr, axis=-1, keepdims=True)
        h = RB // 2
        m1, i1, m2, i2 = top
        for k in range(OB // RB):
            r0 = pl.multiple_of(ob_i * OB + k * RB, RB)
            ob = jnp.concatenate([o_sc[g, pl.ds(r0, RB), :] for g in range(G)], axis=1)
            A = _lhs_ops(ob, LEV)
            c, _ = _strassen(lambda i: jnp.dot(A[i], _upk(to_sc[i]), preferred_element_type=f32), False)
            acc = [[None] * 3, [None] * 3]
            for cc, th, nh in QUADS(c):
                rows = pl.ds(pl.multiple_of(r0 + th * h, h), h)
                cols = slice(nh * HD, (nh + 1) * HD)
                x1 = xb_sc[rows, cols].astype(f32) + cc
                x1_sc[rows, cols] = x1
                s1, s2, st = acc[th]
                for n in range(HD // 128):
                    d = x1[:, 128 * n:128 * (n + 1)]
                    s1 = d if s1 is None else s1 + d
                    s2 = d * d if s2 is None else s2 + d * d
                    t = d * wr[:, nh * HD + 128 * n:nh * HD + 128 * (n + 1)]
                    st = t if st is None else st + t
                acc[th] = [s1, s2, st]
            for th in range(2):
                s1, s2, st = acc[th]
                rows = pl.ds(pl.multiple_of(r0 + th * h, h), h)
                mean = jnp.sum(s1, axis=-1, keepdims=True) * (1.0 / D)
                v = jnp.maximum(jnp.sum(s2, axis=-1, keepdims=True) * (1.0 / D) - mean * mean, 0.0)
                rs = lax.rsqrt(v + EPS)
                r = rs * (jnp.sum(st, axis=-1, keepdims=True) - mean * wr_sum)
                r = r.astype(bf16).astype(f32)
                mean_sc[rows, :] = jnp.broadcast_to(mean, (h, 128))
                rs_sc[rows, :] = jnp.broadcast_to(rs, (h, 128))
                a = 1.0 + rs
                kn_sc[rows, :] = jnp.broadcast_to(a * lax.rsqrt(v * (a * a) + EPS), (h, 128))
                sub = lax.broadcasted_iota(jnp.int32, (8, 1), 0) + (r0 + th * h)
                for j in range(h // 8):
                    rj = r[8 * j:8 * j + 8]
                    idx = sub + 8 * j
                    g1 = rj > m1
                    g2 = rj > m2
                    m2 = jnp.where(g1, m1, jnp.where(g2, rj, m2))
                    i2 = jnp.where(g1, i1, jnp.where(g2, idx, i2))
                    m1 = jnp.where(g1, rj, m1)
                    i1 = jnp.where(g1, idx, i1)
        return m1, i1, m2, i2

    def out_phase():
        top = (jnp.full((8, 1), -jnp.inf, f32), jnp.zeros((8, 1), jnp.int32),
               jnp.full((8, 1), -jnp.inf, f32), jnp.ones((8, 1), jnp.int32))
        return lax.fori_loop(0, NOB, out_body, top)

    def ffn(layer, top):
        m1, i1, m2, i2 = top
        cv = jnp.concatenate([m1, m2], axis=0)
        ci = jnp.concatenate([i1, i2], axis=0)
        v1 = jnp.max(cv, axis=0, keepdims=True)
        j1 = jnp.min(jnp.where(cv == v1, ci, S), axis=0, keepdims=True)
        cv2 = jnp.where(ci == j1, -jnp.inf, cv)
        v2 = jnp.max(cv2, axis=0, keepdims=True)
        j2 = jnp.min(jnp.where(cv2 == v2, ci, S), axis=0, keepdims=True)
        t1 = jnp.clip(j1[0, 0], 0, S - 1)
        t2 = jnp.clip(j2[0, 0], 0, S - 1)
        b1 = pl.ds(pl.multiple_of((t1 // 8) * 8, 8), 8)
        b2 = pl.ds(pl.multiple_of((t2 // 8) * 8, 8), 8)

        def two(ref):
            return jnp.concatenate([ref[b1, :], ref[b2, :]], axis=0)
        xm = (two(x1_sc) - two(mean_sc)[:, 0:1]) * two(rs_sc)[:, 0:1]
        xs = xm.astype(bf16)
        base = two(x1_sc) + xm

        NCH = 16
        CH = S // NCH
        never = jnp.full((CH, 1), zero, jnp.int32) != 0

        def mod_rows(n, tok):
            rows = slice(n * CH, (n + 1) * CH)
            x1 = x1_sc[rows, :]
            mn = mean_sc[rows, 0:1]
            if tok is not None:
                mn = jnp.where(never, tok, mn)
            c = x1 - mn
            xb_sc[rows, :] = (x1 + c * rs_sc[rows, 0:1]).astype(bf16)
            xn_sc[rows, :] = (c * kn_sc[rows, 0:1]).astype(bf16)
            if (n + 1) % (NCH // NOUT) == 0:
                @pl.when(layer == 1)
                def _():
                    out_copy(n // (NCH // NOUT)).start()

        y = None
        mod_rows(0, None)
        mod_rows(1, None)
        for j in range(F // FC):
            gg = jnp.dot(xs, wg_sc[:, FC * j:FC * (j + 1)], preferred_element_type=f32)
            uu = jnp.dot(xs, wu_sc[:, FC * j:FC * (j + 1)], preferred_element_type=f32)
            hh = (gg * _sigmoid(gg) * uu).astype(bf16)
            t = jnp.dot(hh, wd_sc[FC * j:FC * (j + 1), :], preferred_element_type=f32)
            y = t if y is None else y + t
            if j < 7:
                mod_rows(2 + 2 * j, jnp.broadcast_to(gg[0:1, 0:1], (CH, 1)))
                mod_rows(3 + 2 * j, jnp.broadcast_to(t[0:1, 0:1], (CH, 1)))
        r8 = lax.broadcasted_iota(jnp.int32, (8, D), 0)
        y1 = jnp.where(r8 == t1 % 8, y[0:8] * _sigmoid(v1), 0.0)
        y2 = jnp.where(r8 == t2 % 8, y[8:16] * _sigmoid(v2), 0.0)
        same = t1 // 8 == t2 // 8
        n1 = base[0:8] + (y1 + jnp.where(same, y2, 0.0))
        n2 = base[8:16] + (y2 + jnp.where(same, y1, 0.0))

        @pl.when(layer == 1)
        def _():
            for i in range(NOUT):
                out_copy(i).wait()

        for b, xx in ((b1, n1), (b2, n2)):
            xb_sc[b, :] = xx.astype(bf16)
            cc = xx - jnp.mean(xx, axis=-1, keepdims=True)
            xn_sc[b, :] = (cc * lax.rsqrt(jnp.mean(cc * cc, axis=-1, keepdims=True) + EPS)).astype(bf16)

        @pl.when(layer == 1)
        def _():
            c1 = pltpu.make_async_copy(xb_sc.at[b1, :], out_hbm.at[b1, :], sems.at[7])
            c1.start()

            @pl.when(jnp.logical_not(same))
            def _():
                c2 = pltpu.make_async_copy(xb_sc.at[b2, :], out_hbm.at[b2, :], sems.at[8])
                c2.start()
                c2.wait()
            c1.wait()

    def prep_k_piece(n, c):
        for part in range(1 << LEV):
            wk_copy(n, part).wait()
        for m in range(8 // NWK):
            _prep(tk_sc, wk_sc, n * (8 // NWK) + m, 8, False)
        return c

    ln_input(0)
    lax.fori_loop(0, NWK, prep_k_piece, 0)

    def layer_body(layer, carry):
        first = layer == 0
        lax.fori_loop(0, NRB, functools.partial(proj_k_body, layer), 0)

        @pl.when(first)
        def _():
            cp["wq"].wait()
            prep_tr(tq_sc, wq_sc)
            cp["wv"].wait()
            prep_tr(tv_sc, wv_sc)
        lax.fori_loop(0, NRB, functools.partial(proj_qv_body, layer), 0)
        attn_phase()

        @pl.when(first)
        def _():
            cp["wo"].wait()
            cp["wr"].wait()
            prep_nat(to_sc, wo_sc)
        top = out_phase()

        @pl.when(first)
        def _():
            cp["wg"].wait()
            cp["wu"].wait()
            cp["wd"].wait()
        ffn(layer, top)
        return carry

    lax.fori_loop(0, 2, layer_body, 0)


@jax.jit
def pallas_interleave_layers__memory_aug_infini_attn__moe_arch_mod__prompt_kernel(
    A_x: jax.Array,
    A_wq: jax.Array,
    A_wk: jax.Array,
    A_wv: jax.Array,
    A_wo: jax.Array,
    A_beta: jax.Array,
    B_x: jax.Array,
    B_w_r: jax.Array,
    B_w_gate: jax.Array,
    B_w_up: jax.Array,
    B_w_down: jax.Array,
):
    del B_x
    x = A_x.reshape(S, D)
    zero = jnp.zeros((1,), jnp.int32)
    any_spec = pl.BlockSpec(memory_space=pl.ANY)
    smem_spec = pl.BlockSpec(memory_space=pltpu.SMEM)
    V = pltpu.VMEM
    scratch = [
        V((S, D), f32),
        V((S, D), bf16),
        V((S, D), bf16),
        V((S, 128), f32), V((S, 128), f32), V((S, 128), f32),
    ] + [V((NP, BD // 2, BD), u32)] * 4 + [
        V((D, D), bf16), V((D, D), bf16), V((D, D), bf16), V((D, D), bf16),
        V((D, D), bf16),
        V((D,), bf16),
        V((D, F), bf16), V((D, F), bf16), V((F, D), bf16),
        V((G, S, 128), bf16), V((G, S, 128), bf16),
        V((NRB, G, 128, RB), bf16), V((NRB, G, 128, RB), bf16), V((NRB, G, 128, RB), bf16),
        V((G, S, 128), bf16),
        V((NRB, G, 8, 128), f32),
        V((H, 8, 128), f32),
        V((T, 4 * T), f32),
        pltpu.SemaphoreType.DMA((9,)),
        pltpu.SemaphoreType.DMA((NOUT,)),
        pltpu.SemaphoreType.DMA((NRB,)),
        pltpu.SemaphoreType.DMA((NWK, 1 << LEV)),
    ] + [V((T, 4 * T), f32)] * NSLOT
    out = pl.pallas_call(
        _kernel,
        in_specs=[smem_spec, pl.BlockSpec(memory_space=pltpu.VMEM)] + [any_spec] * 9,
        out_specs=any_spec,
        out_shape=jax.ShapeDtypeStruct((S, D), bf16),
        scratch_shapes=scratch,
        compiler_params=pltpu.CompilerParams(vmem_limit_bytes=120 * 1024 * 1024),
    )(zero, A_beta, x, A_wq, A_wk, A_wv, A_wo, B_w_r, B_w_gate, B_w_up, B_w_down)
    return out.reshape(1, S, D)
```

```python
import functools
import itertools

import jax
import jax.numpy as jnp
from jax import lax
import jax.experimental.pallas as pl
import jax.experimental.pallas.tpu as pltpu

S, D, H, DH, NSEG, L, F = 2048, 1024, 32, 32, 4, 512, 3584
G = 8
LEV = 2
NP = 7 ** LEV
BD = D >> LEV
HD = D // 2
RB = 128 << LEV
NRB = S // RB
OB = 1024
NOB = S // OB
NOUT = 16
FC = 256
NWK = 4
NPC = 16
T = 128
LAG = 5
NSLOT = 5
EPS = 1e-05
LOG2E = 1.4426950408889634
QSCALE = (DH ** -0.5) * LOG2E
NEG = -1e30
NT = (((1,), (1,)), ((), ()))
ORDER = (2, 4, 3, 1, 0, 6, 5)

f32 = jnp.float32
bf16 = jnp.bfloat16
u32 = jnp.uint32


def _phi(t):
    return jnp.where(t > 0, t + 1.0, jnp.exp(t))


def _sigmoid(t):
    return 1.0 / (1.0 + jnp.exp(-t))


def _pk(x):
    return pltpu.bitcast(x, u32)


def _upk(x):
    return pltpu.bitcast(x, bf16)


def _row_fold(x, op):
    parts = [x[8 * r:8 * r + 8] for r in range(x.shape[0] // 8)]
    while len(parts) > 1:
        parts = [op(parts[i], parts[i + 1]) if i + 1 < len(parts) else parts[i] for i in range(0, len(parts), 2)]
    return parts[0]


def _quads(x):
    h, w = x.shape[0] // 2, x.shape[1] // 2
    return x[:h, :w], x[:h, w:], x[h:, :w], x[h:, w:]


def _lhs_ops(x, lev):
    if lev == 0:
        return [x.astype(bf16)]
    x00, x01, x10, x11 = _quads(x)
    a00, a01, a10, a11 = (t.astype(f32) for t in (x00, x01, x10, x11))
    ops = (a00 + a11, a10 + a11, x00, x11, a00 + a01, a10 - a00, a01 - a11)
    return [o for t in ops for o in _lhs_ops(t, lev - 1)]


def _rhs_ops(w, lev):
    if lev == 0:
        return [w[()].astype(bf16)]

    def sub(r, c):
        return {p[1:]: v for p, v in w.items() if p[0] == (r, c)}

    def add(x, y, sign=1):
        return {p: (x[p].astype(f32) + y[p].astype(f32) if sign > 0 else x[p].astype(f32) - y[p].astype(f32))
                for p in x}
    b11, b12, b21, b22 = sub(0, 0), sub(0, 1), sub(1, 0), sub(1, 1)
    ops = (add(b11, b22), b11, add(b12, b22, -1), add(b21, b11, -1), b22, add(b11, b12), add(b21, b22))
    return [o for t in ops for o in _rhs_ops(t, lev - 1)]


def _offsets(path):
    r = sum(rc[0] * (D >> (i + 1)) for i, rc in enumerate(path))
    c = sum(rc[1] * (D >> (i + 1)) for i, rc in enumerate(path))
    return r, c


def _prep(t_ref, w_ref, n, nch, transposed):
    ch = BD // nch
    w = {}
    for path in itertools.product(((0, 0), (0, 1), (1, 0), (1, 1)), repeat=LEV):
        r, c = _offsets(path)
        if transposed:
            r, c = c, r
        w[path] = w_ref[pl.ds(pl.multiple_of(r + n * ch, ch), ch), c:c + BD]
    packed = t_ref.dtype == u32
    rows = pl.ds(pl.multiple_of(n * (ch // 2), ch // 2), ch // 2) if packed else pl.ds(pl.multiple_of(n * ch, ch), ch)
    for i, t in enumerate(_rhs_ops(w, LEV)):
        t_ref[i, rows, :] = _pk(t) if packed else t


def _combine(M):
    m1, m2, m3, m4, m5, m6, m7 = M
    return m1 + m4 - m5 + m7, m3 + m5, m2 + m4, m1 - m2 + m3 + m6


def _strassen(mm, transposed):
    def assemble(c11, c12, c21, c22):
        if transposed:
            c12, c21 = c21, c12
        return jnp.concatenate([jnp.concatenate([c11, c12], axis=1), jnp.concatenate([c21, c22], axis=1)], axis=0)

    def rec(base, lev):
        M = [None] * 7
        for i in ORDER:
            M[i] = mm(base * 7 + i) if lev == 1 else assemble(*rec(base * 7 + i, lev - 1)[0])
        return _combine(M), M
    return rec(0, LEV)


def _kernel(zero_smem, beta_ref, x_hbm, wq_hbm, wk_hbm, wv_hbm, wo_hbm, wr_hbm,
            wg_hbm, wu_hbm, wd_hbm, out_hbm,
            x1_sc, xb_sc, xn_sc, mean_sc, rs_sc, kn_sc, tk_sc, tq_sc, tv_sc, to_sc,
            wq_sc, wk_sc, wv_sc, wo_sc, wT_sc, wr_sc,
            wg_sc, wu_sc, wd_sc, k_sc, pk_sc, qT_sc, pqT_sc, vT_sc, o_sc, z_sc,
            gt_sc, am_sc, sems, osems, xsems, ksems, *s_sc):
    cp = {
        "wq": pltpu.make_async_copy(wq_hbm, wq_sc, sems.at[0]),
        "wv": pltpu.make_async_copy(wv_hbm, wv_sc, sems.at[1]),
        "wo": pltpu.make_async_copy(wo_hbm, wo_sc, sems.at[2]),
        "wr": pltpu.make_async_copy(wr_hbm, wr_sc, sems.at[3]),
        "wg": pltpu.make_async_copy(wg_hbm, wg_sc, sems.at[4]),
        "wu": pltpu.make_async_copy(wu_hbm, wu_sc, sems.at[5]),
        "wd": pltpu.make_async_copy(wd_hbm, wd_sc, sems.at[6]),
    }

    def x_copy(rb):
        rows = pl.ds(pl.multiple_of(rb * RB, RB), RB)
        return pltpu.make_async_copy(x_hbm.at[rows, :], xb_sc.at[rows, :], xsems.at[rb])

    def wk_copy(n, part):
        rows = pl.ds(part * BD + n * (BD // NWK), BD // NWK)
        return pltpu.make_async_copy(wk_hbm.at[rows, :], wk_sc.at[rows, :], ksems.at[n, part])

    def out_copy(i):
        rows = pl.ds(i * (S // NOUT), S // NOUT)
        return pltpu.make_async_copy(xb_sc.at[rows, :], out_hbm.at[rows, :], osems.at[i])

    x_copy(0).start()
    zero = zero_smem[0]

    am_sc[...] = jnp.zeros((T, 4 * T), f32)

    gates = _sigmoid(beta_ref[...].reshape(1, H).astype(f32))
    for h in range(H):
        gt_sc[h] = jnp.broadcast_to(gates[:, h:h + 1], (8, 128))

    row = lax.broadcasted_iota(jnp.int32, (T, T), 0)
    col = lax.broadcasted_iota(jnp.int32, (T, T), 1)
    cmask = row <= col
    hmask = (row // 32) == (col // 32)
    zrow = lax.broadcasted_iota(jnp.int32, (32, T), 0)
    zcol = lax.broadcasted_iota(jnp.int32, (32, T), 1)
    zmask = (zrow // 8) == (zcol // 32)

    def rows_of(rb):
        return pl.ds(pl.multiple_of(rb * RB, RB), RB)

    def prep_nat(t_ref, w_ref):
        lax.fori_loop(0, NPC, lambda n, c: (_prep(t_ref, w_ref, n, NPC, False), c)[1], 0)

    def prep_tr(t_ref, w_ref):
        for j in range(4):
            for i in range(4):
                wT_sc[256 * j:256 * (j + 1), 256 * i:256 * (i + 1)] = w_ref[256 * i:256 * (i + 1), 256 * j:256 * (j + 1)].T
        lax.fori_loop(0, NPC, lambda n, c: (_prep(t_ref, wT_sc, n, NPC, True), c)[1], 0)

    QUADS = lambda c: ((c[1], 0, 1), (c[2], 1, 0), (c[0], 0, 0), (c[3], 1, 1))

    def ln_input(rb):
        x_copy(rb).wait()
        if isinstance(rb, int):
            for n in range(NWK):
                for part in range(1 << LEV):
                    wk_copy(n, part).start()
        for n in range(RB // 128):
            rows = pl.ds(pl.multiple_of(rb * RB + n * 128, 128), 128)
            x = xb_sc[rows, :].astype(f32)
            c = x - jnp.mean(x, axis=-1, keepdims=True)
            v = jnp.mean(c * c, axis=-1, keepdims=True)
            xn_sc[rows, :] = (c * lax.rsqrt(v + EPS)).astype(bf16)

    def proj_k_body(layer, rb, carry):
        @pl.when(layer == 0)
        def _():
            @pl.when(rb == 0)
            def _():
                for i in range(1, NRB):
                    x_copy(i).start()
            for j, name in ((1, "wq"), (1, "wv"), (2, "wo"), (3, "wr")):
                @pl.when(rb == j)
                def _():
                    cp[name].start()

            @pl.when(rb > 0)
            def _():
                ln_input(rb)
        h = RB // 2
        r0 = pl.multiple_of(rb * RB, RB)
        A = _lhs_ops(xn_sc[rows_of(rb), :], LEV)
        c, _ = _strassen(lambda i: jnp.dot(A[i], tk_sc[i], preferred_element_type=f32), False)
        zp = [None, None]
        for kk, th, nh in QUADS(c):
            pk = _phi(kk)
            zz = _row_fold(pk, jnp.add)
            zp[nh] = zz if zp[nh] is None else zp[nh] + zz
            rows = pl.ds(pl.multiple_of(r0 + th * h, h), h)
            for g in range(G // 2):
                k_sc[4 * nh + g, rows, :] = kk[:, 128 * g:128 * (g + 1)].astype(bf16)
                pk_sc[4 * nh + g, rows, :] = pk[:, 128 * g:128 * (g + 1)].astype(bf16)
        for nh in range(2):
            for g in range(G // 2):
                z_sc[rb, 4 * nh + g] = zp[nh][:, 128 * g:128 * (g + 1)]
        return carry

    def proj_qv_body(layer, rb, carry):
        @pl.when(jnp.logical_and(layer == 0, rb == 0))
        def _():
            for name in ("wg", "wu", "wd"):
                cp[name].start()
        h = RB // 2
        A = _lhs_ops(xn_sc[rows_of(rb), :], LEV)
        c, _ = _strassen(lambda i: lax.dot_general(tq_sc[i], A[i], NT, preferred_element_type=f32), True)
        for qq, th, nh in QUADS(c):
            pq = _phi(qq)
            for g in range(G // 2):
                qT_sc[rb, 4 * nh + g, :, th * h:(th + 1) * h] = (qq[128 * g:128 * (g + 1)] * QSCALE).astype(bf16)
                pqT_sc[rb, 4 * nh + g, :, th * h:(th + 1) * h] = pq[128 * g:128 * (g + 1)].astype(bf16)
        c, _ = _strassen(lambda i: lax.dot_general(tv_sc[i], A[i], NT, preferred_element_type=f32), True)
        for vv, th, nh in QUADS(c):
            for g in range(G // 2):
                vT_sc[rb, 4 * nh + g, :, th * h:(th + 1) * h] = vv[128 * g:128 * (g + 1)].astype(bf16)
        return carry

    TILES = [(s, i) for s in range(NSEG) for i in (3, 2, 1, 0)]
    STREAM = [(t, c) for t, (s, i) in enumerate(TILES) for c in range(i + 1)]
    NPOS = len(STREAM)

    def sref(k, h):
        return s_sc[k % NSLOT].at[pl.ds(pl.multiple_of(zero, 8), T), T * h:T * (h + 1)]

    def tcols(ref, g, t0, n, rows=slice(None)):
        parts = []
        for t in range(t0, t0 + n, min(n, RB)):
            parts.append(ref[t // RB, g, rows, t % RB:t % RB + min(n, RB)])
        return parts[0] if len(parts) == 1 else jnp.concatenate(parts, axis=1)

    def q_weights(g, s, i):
        QT = tcols(qT_sc, g, s * L + i * T, T)
        z = jnp.zeros((32, T), bf16)
        return jnp.concatenate(
            [jnp.concatenate([QT[32 * h:32 * h + 32] if hh == h else z for hh in range(4)], axis=0)
             for h in range(4)], axis=1)

    def qk(g, k, m):
        t, c = STREAM[k]
        s, i = TILES[t]
        k0 = s * L + c * T
        K = k_sc[g, k0:k0 + T, :]
        S4 = jnp.dot(K, q_weights(g, s, i), preferred_element_type=f32)
        out = []
        for h in range(4):
            Sx = S4[:, T * h:T * (h + 1)]
            if c == i:
                Sx = jnp.where(cmask, Sx, NEG)
            sref(k, h)[...] = Sx
            mm = Sx[0:8]
            for r in range(1, 16):
                mm = jnp.maximum(mm, Sx[8 * r:8 * r + 8])
            mm = mm if c == 0 else jnp.maximum(m[h], mm)
            if c == i:
                mm = jnp.broadcast_to(jnp.max(mm, axis=0, keepdims=True), (8, T))
            out.append(mm)
        return out

    def attn_prologue():
        m = {}
        for k in range(LAG):
            t = STREAM[k][0]
            m[t] = qk(0, k, m.get(t))
        return tuple(m[STREAM[0][0]]) + tuple(m[STREAM[LAG - 1][0]])

    def finish(g, s, i, O, l):
        outs = []
        for h in range(4):
            lt = jnp.sum(l[h], axis=0, keepdims=True)
            gt = jnp.concatenate([gt_sc[4 * g + h]] * 4, axis=0)
            o = O[h] * ((1.0 - gt) * (1.0 / lt))
            if s > 0:
                o = o + am_sc[32 * h:32 * h + 32, i * T:(i + 1) * T]
            outs.append(o)
        ot = jnp.concatenate(outs, axis=0).astype(bf16)
        r0 = s * L + i * T
        o_sc[g, r0:r0 + T, :] = ot.T

    def attn_body(g, carry):
        gn = jnp.minimum(g + 1, G - 1)
        m = {STREAM[0][0]: list(carry[0:4]), STREAM[LAG - 1][0]: list(carry[4:8])}
        l, O, P, M, mn = {}, {}, {}, {}, {}

        def mem_read(s):
            zs = z_sc[0, g]
            for rb in range(1, s * L // RB):
                zs = zs + z_sc[rb, g]
            zs = jnp.sum(zs, axis=0, keepdims=True)
            zrows = jnp.where(zmask, zs, 0.0).astype(bf16)
            mbd = jnp.where(hmask, M[0], 0.0).astype(bf16)
            lhs = jnp.concatenate([mbd, zrows], axis=0)
            pq = tcols(pqT_sc, g, s * L, L)
            nd = jnp.dot(lhs, pq, preferred_element_type=f32)
            for h in range(4):
                den = nd[128 + 8 * h:128 + 8 * h + 8] + 1e-06
                gd = jnp.concatenate([gt_sc[4 * g + h]] * 4, axis=1) / den
                am_sc[32 * h:32 * h + 32, :] = nd[32 * h:32 * h + 32] * jnp.concatenate([gd] * 4, axis=0)

        def mem_write(s):
            vt = tcols(vT_sc, g, s * L, L)
            pk = pk_sc[g, s * L:(s + 1) * L, :]
            inc = jnp.dot(vt, pk, preferred_element_type=f32)
            M[0] = inc if s == 0 else M[0] + inc

        def ex(k):
            t, c = STREAM[k]
            out = []
            for h in range(4):
                Pp = jnp.exp2(sref(k, h)[...] - jnp.concatenate([m[t][h]] * (T // 8), axis=0))
                a = Pp[0:8] + Pp[8:16]
                b = Pp[16:24] + Pp[24:32]
                for r in range(2, 8, 2):
                    a = a + (Pp[16 * r:16 * r + 8] + Pp[16 * r + 8:16 * r + 16])
                    b = b + (Pp[16 * r + 16:16 * r + 24] + Pp[16 * r + 24:16 * r + 32])
                ll = a + b
                if c == 0:
                    l.setdefault(t, [None] * 4)[h] = ll
                else:
                    l[t][h] = l[t][h] + ll
                out.append(Pp.astype(bf16))
            P[k] = out

        def pv(k):
            t, c = STREAM[k]
            s, i = TILES[t]
            if c == 0:
                O[t] = [None] * 4
            for h in range(4):
                vt = tcols(vT_sc, g, s * L + c * T, T, slice(32 * h, 32 * h + 32))
                o = jnp.dot(vt, P[k][h], preferred_element_type=f32)
                O[t][h] = o if O[t][h] is None else O[t][h] + o
            del P[k]

        finish(jnp.maximum(g - 1, 0), NSEG - 1, 0, carry[8:12], carry[12:16])
        done = None
        for j in range(NPOS):
            ex(j)
            k = j + LAG
            if k < NPOS:
                t = STREAM[k][0]
                m[t] = qk(g, k, m.get(t))
            else:
                t = STREAM[k - NPOS][0]
                mn[t] = qk(gn, k - NPOS, mn.get(t))
            pv(j)
            if done is not None:
                s, i = TILES[done]
                finish(g, s, i, O[done], l[done])
                if i == 0:
                    mem_read(s + 1)
                done = None
            t, c = STREAM[j]
            if c == TILES[t][1]:
                done = t
                if TILES[t][1] == 3 and TILES[t][0] < NSEG - 1:
                    mem_write(TILES[t][0])
        return (tuple(mn[STREAM[0][0]]) + tuple(mn[STREAM[LAG - 1][0]]) + tuple(O[done]) + tuple(l[done]))

    def attn_phase():
        init = attn_prologue() + (jnp.zeros((32, T), f32),) * 4 + (jnp.ones((8, T), f32),) * 4
        carry = lax.fori_loop(0, G, attn_body, init)
        finish(G - 1, NSEG - 1, 0, carry[8:12], carry[12:16])

    def out_body(ob_i, top):
        wr = wr_sc[...].reshape(1, D).astype(f32)
        wr_sum = jnp.sum(wr, axis=-1, keepdims=True)
        h = RB // 2
        m1, i1, m2, i2 = top
        for k in range(OB // RB):
            r0 = pl.multiple_of(ob_i * OB + k * RB, RB)
            ob = jnp.concatenate([o_sc[g, pl.ds(r0, RB), :] for g in range(G)], axis=1)
            A = _lhs_ops(ob, LEV)
            c, _ = _strassen(lambda i: jnp.dot(A[i], _upk(to_sc[i]), preferred_element_type=f32), False)
            acc = [[None] * 3, [None] * 3]
            for cc, th, nh in QUADS(c):
                rows = pl.ds(pl.multiple_of(r0 + th * h, h), h)
                cols = slice(nh * HD, (nh + 1) * HD)
                x1 = xb_sc[rows, cols].astype(f32) + cc
                x1_sc[rows, cols] = x1
                s1, s2, st = acc[th]
                for n in range(HD // 128):
                    d = x1[:, 128 * n:128 * (n + 1)]
                    s1 = d if s1 is None else s1 + d
                    s2 = d * d if s2 is None else s2 + d * d
                    t = d * wr[:, nh * HD + 128 * n:nh * HD + 128 * (n + 1)]
                    st = t if st is None else st + t
                acc[th] = [s1, s2, st]
            for th in range(2):
                s1, s2, st = acc[th]
                rows = pl.ds(pl.multiple_of(r0 + th * h, h), h)
                mean = jnp.sum(s1, axis=-1, keepdims=True) * (1.0 / D)
                v = jnp.maximum(jnp.sum(s2, axis=-1, keepdims=True) * (1.0 / D) - mean * mean, 0.0)
                rs = lax.rsqrt(v + EPS)
                r = rs * (jnp.sum(st, axis=-1, keepdims=True) - mean * wr_sum)
                r = r.astype(bf16).astype(f32)
                mean_sc[rows, :] = jnp.broadcast_to(mean, (h, 128))
                rs_sc[rows, :] = jnp.broadcast_to(rs, (h, 128))
                a = 1.0 + rs
                kn_sc[rows, :] = jnp.broadcast_to(a * lax.rsqrt(v * (a * a) + EPS), (h, 128))
                sub = lax.broadcasted_iota(jnp.int32, (8, 1), 0) + (r0 + th * h)
                for j in range(h // 8):
                    rj = r[8 * j:8 * j + 8]
                    idx = sub + 8 * j
                    g1 = rj > m1
                    g2 = rj > m2
                    m2 = jnp.where(g1, m1, jnp.where(g2, rj, m2))
                    i2 = jnp.where(g1, i1, jnp.where(g2, idx, i2))
                    m1 = jnp.where(g1, rj, m1)
                    i1 = jnp.where(g1, idx, i1)
        return m1, i1, m2, i2

    def out_phase():
        top = (jnp.full((8, 1), -jnp.inf, f32), jnp.zeros((8, 1), jnp.int32),
               jnp.full((8, 1), -jnp.inf, f32), jnp.ones((8, 1), jnp.int32))
        return lax.fori_loop(0, NOB, out_body, top)

    def ffn(layer, top):
        m1, i1, m2, i2 = top
        cv = jnp.concatenate([m1, m2], axis=0)
        ci = jnp.concatenate([i1, i2], axis=0)
        v1 = jnp.max(cv, axis=0, keepdims=True)
        j1 = jnp.min(jnp.where(cv == v1, ci, S), axis=0, keepdims=True)
        cv2 = jnp.where(ci == j1, -jnp.inf, cv)
        v2 = jnp.max(cv2, axis=0, keepdims=True)
        j2 = jnp.min(jnp.where(cv2 == v2, ci, S), axis=0, keepdims=True)
        t1 = jnp.clip(j1[0, 0], 0, S - 1)
        t2 = jnp.clip(j2[0, 0], 0, S - 1)
        b1 = pl.ds(pl.multiple_of((t1 // 8) * 8, 8), 8)
        b2 = pl.ds(pl.multiple_of((t2 // 8) * 8, 8), 8)

        def two(ref):
            return jnp.concatenate([ref[b1, :], ref[b2, :]], axis=0)
        xm = (two(x1_sc) - two(mean_sc)[:, 0:1]) * two(rs_sc)[:, 0:1]
        xs = xm.astype(bf16)
        base = two(x1_sc) + xm

        NCH = 16
        CH = S // NCH
        never = jnp.full((CH, 1), zero, jnp.int32) != 0

        def mod_rows(n, tok):
            rows = slice(n * CH, (n + 1) * CH)
            x1 = x1_sc[rows, :]
            mn = mean_sc[rows, 0:1]
            if tok is not None:
                mn = jnp.where(never, tok, mn)
            c = x1 - mn
            xb_sc[rows, :] = (x1 + c * rs_sc[rows, 0:1]).astype(bf16)
            xn_sc[rows, :] = (c * kn_sc[rows, 0:1]).astype(bf16)
            if (n + 1) % (NCH // NOUT) == 0:
                @pl.when(layer == 1)
                def _():
                    out_copy(n // (NCH // NOUT)).start()

        y = None
        mod_rows(0, None)
        mod_rows(1, None)
        for j in range(F // FC):
            gg = jnp.dot(xs, wg_sc[:, FC * j:FC * (j + 1)], preferred_element_type=f32)
            uu = jnp.dot(xs, wu_sc[:, FC * j:FC * (j + 1)], preferred_element_type=f32)
            hh = (gg * _sigmoid(gg) * uu).astype(bf16)
            t = jnp.dot(hh, wd_sc[FC * j:FC * (j + 1), :], preferred_element_type=f32)
            y = t if y is None else y + t
            if j < 7:
                mod_rows(2 + 2 * j, jnp.broadcast_to(gg[0:1, 0:1], (CH, 1)))
                mod_rows(3 + 2 * j, jnp.broadcast_to(t[0:1, 0:1], (CH, 1)))
        r8 = lax.broadcasted_iota(jnp.int32, (8, D), 0)
        y1 = jnp.where(r8 == t1 % 8, y[0:8] * _sigmoid(v1), 0.0)
        y2 = jnp.where(r8 == t2 % 8, y[8:16] * _sigmoid(v2), 0.0)
        same = t1 // 8 == t2 // 8
        n1 = base[0:8] + (y1 + jnp.where(same, y2, 0.0))
        n2 = base[8:16] + (y2 + jnp.where(same, y1, 0.0))

        @pl.when(layer == 1)
        def _():
            for i in range(NOUT):
                out_copy(i).wait()

        for b, xx in ((b1, n1), (b2, n2)):
            xb_sc[b, :] = xx.astype(bf16)
            cc = xx - jnp.mean(xx, axis=-1, keepdims=True)
            xn_sc[b, :] = (cc * lax.rsqrt(jnp.mean(cc * cc, axis=-1, keepdims=True) + EPS)).astype(bf16)

        @pl.when(layer == 1)
        def _():
            c1 = pltpu.make_async_copy(xb_sc.at[b1, :], out_hbm.at[b1, :], sems.at[7])
            c1.start()

            @pl.when(jnp.logical_not(same))
            def _():
                c2 = pltpu.make_async_copy(xb_sc.at[b2, :], out_hbm.at[b2, :], sems.at[8])
                c2.start()
                c2.wait()
            c1.wait()

    def prep_k_piece(n, c):
        for part in range(1 << LEV):
            wk_copy(n, part).wait()
        return lax.fori_loop(n * (NPC // NWK), (n + 1) * (NPC // NWK),
                             lambda m, c_: (_prep(tk_sc, wk_sc, m, NPC, False), c_)[1], c)

    ln_input(0)
    lax.fori_loop(0, NWK, prep_k_piece, 0)

    def layer_body(layer, carry):
        first = layer == 0
        lax.fori_loop(0, NRB, functools.partial(proj_k_body, layer), 0)

        @pl.when(first)
        def _():
            cp["wq"].wait()
            prep_tr(tq_sc, wq_sc)
            cp["wv"].wait()
            prep_tr(tv_sc, wv_sc)
        lax.fori_loop(0, NRB, functools.partial(proj_qv_body, layer), 0)
        attn_phase()

        @pl.when(first)
        def _():
            cp["wo"].wait()
            cp["wr"].wait()
            prep_nat(to_sc, wo_sc)
        top = out_phase()

        @pl.when(first)
        def _():
            cp["wg"].wait()
            cp["wu"].wait()
            cp["wd"].wait()
        ffn(layer, top)
        return carry

    lax.fori_loop(0, 2, layer_body, 0)


@jax.jit
def pallas_interleave_layers__memory_aug_infini_attn__moe_arch_mod__prompt_kernel(
    A_x: jax.Array,
    A_wq: jax.Array,
    A_wk: jax.Array,
    A_wv: jax.Array,
    A_wo: jax.Array,
    A_beta: jax.Array,
    B_x: jax.Array,
    B_w_r: jax.Array,
    B_w_gate: jax.Array,
    B_w_up: jax.Array,
    B_w_down: jax.Array,
):
    del B_x
    x = A_x.reshape(S, D)
    zero = jnp.zeros((1,), jnp.int32)
    any_spec = pl.BlockSpec(memory_space=pl.ANY)
    smem_spec = pl.BlockSpec(memory_space=pltpu.SMEM)
    V = pltpu.VMEM
    scratch = [
        V((S, D), f32),
        V((S, D), bf16),
        V((S, D), bf16),
        V((S, 128), f32), V((S, 128), f32), V((S, 128), f32),
            V((NP, BD, BD), bf16), V((NP, BD, BD), bf16), V((NP, BD, BD), bf16),
        V((NP, BD // 2, BD), u32),
    ] + [
        V((D, D), bf16), V((D, D), bf16), V((D, D), bf16), V((D, D), bf16),
        V((D, D), bf16),
        V((D,), bf16),
        V((D, F), bf16), V((D, F), bf16), V((F, D), bf16),
        V((G, S, 128), bf16), V((G, S, 128), bf16),
        V((NRB, G, 128, RB), bf16), V((NRB, G, 128, RB), bf16), V((NRB, G, 128, RB), bf16),
        V((G, S, 128), bf16),
        V((NRB, G, 8, 128), f32),
        V((H, 8, 128), f32),
        V((T, 4 * T), f32),
        pltpu.SemaphoreType.DMA((9,)),
        pltpu.SemaphoreType.DMA((NOUT,)),
        pltpu.SemaphoreType.DMA((NRB,)),
        pltpu.SemaphoreType.DMA((NWK, 1 << LEV)),
    ] + [V((T, 4 * T), f32)] * NSLOT
    out = pl.pallas_call(
        _kernel,
        in_specs=[smem_spec, pl.BlockSpec(memory_space=pltpu.VMEM)] + [any_spec] * 9,
        out_specs=any_spec,
        out_shape=jax.ShapeDtypeStruct((S, D), bf16),
        scratch_shapes=scratch,
        compiler_params=pltpu.CompilerParams(vmem_limit_bytes=120 * 1024 * 1024),
    )(zero, A_beta, x, A_wq, A_wk, A_wv, A_wo, B_w_r, B_w_gate, B_w_up, B_w_down)
    return out.reshape(1, S, D)
```

```python
import functools
import itertools

import jax
import jax.numpy as jnp
from jax import lax
import jax.experimental.pallas as pl
import jax.experimental.pallas.tpu as pltpu

S, D, H, DH, NSEG, L, F = 2048, 1024, 32, 32, 4, 512, 3584
G = 8
LEV = 2
NP = 7 ** LEV
BD = D >> LEV
HD = D // 2
RB = 128 << LEV
NRB = S // RB
OB = 1024
NOB = S // OB
CH = 128
CPS = 3
PRO = 4
NOUT = 1 + (S // CH - PRO) // CPS
FC = 256
NWK = 4
NPC = 16
T = 128
LAG = 5
NSLOT = 5
EPS = 1e-05
LOG2E = 1.4426950408889634
QSCALE = (DH ** -0.5) * LOG2E
NEG = -1e30
NT = (((1,), (1,)), ((), ()))
ORDER = (2, 4, 3, 1, 0, 6, 5)

f32 = jnp.float32
bf16 = jnp.bfloat16
u32 = jnp.uint32


def _phi(t):
    return jnp.where(t > 0, t + 1.0, jnp.exp(t))


def _sigmoid(t):
    return 1.0 / (1.0 + jnp.exp(-t))


def _pk(x):
    return pltpu.bitcast(x, u32)


def _upk(x):
    return pltpu.bitcast(x, bf16)


def _row_fold(x, op):
    parts = [x[8 * r:8 * r + 8] for r in range(x.shape[0] // 8)]
    while len(parts) > 1:
        parts = [op(parts[i], parts[i + 1]) if i + 1 < len(parts) else parts[i] for i in range(0, len(parts), 2)]
    return parts[0]


def _quads(x):
    h, w = x.shape[0] // 2, x.shape[1] // 2
    return x[:h, :w], x[:h, w:], x[h:, :w], x[h:, w:]


def _lhs_ops(x, lev):
    if lev == 0:
        return [x.astype(bf16)]
    x00, x01, x10, x11 = _quads(x)
    a00, a01, a10, a11 = (t.astype(f32) for t in (x00, x01, x10, x11))
    ops = (a00 + a11, a10 + a11, x00, x11, a00 + a01, a10 - a00, a01 - a11)
    return [o for t in ops for o in _lhs_ops(t, lev - 1)]


def _rhs_ops(w, lev):
    if lev == 0:
        return [w[()].astype(bf16)]

    def sub(r, c):
        return {p[1:]: v for p, v in w.items() if p[0] == (r, c)}

    def add(x, y, sign=1):
        return {p: (x[p].astype(f32) + y[p].astype(f32) if sign > 0 else x[p].astype(f32) - y[p].astype(f32))
                for p in x}
    b11, b12, b21, b22 = sub(0, 0), sub(0, 1), sub(1, 0), sub(1, 1)
    ops = (add(b11, b22), b11, add(b12, b22, -1), add(b21, b11, -1), b22, add(b11, b12), add(b21, b22))
    return [o for t in ops for o in _rhs_ops(t, lev - 1)]


def _offsets(path):
    r = sum(rc[0] * (D >> (i + 1)) for i, rc in enumerate(path))
    c = sum(rc[1] * (D >> (i + 1)) for i, rc in enumerate(path))
    return r, c


def _prep(t_ref, w_ref, n, nch, transposed):
    ch = BD // nch
    w = {}
    for path in itertools.product(((0, 0), (0, 1), (1, 0), (1, 1)), repeat=LEV):
        r, c = _offsets(path)
        if transposed:
            r, c = c, r
        w[path] = w_ref[pl.ds(pl.multiple_of(r + n * ch, ch), ch), c:c + BD]
    packed = t_ref.dtype == u32
    rows = pl.ds(pl.multiple_of(n * (ch // 2), ch // 2), ch // 2) if packed else pl.ds(pl.multiple_of(n * ch, ch), ch)
    for i, t in enumerate(_rhs_ops(w, LEV)):
        t_ref[i, rows, :] = _pk(t) if packed else t


def _combine(M):
    m1, m2, m3, m4, m5, m6, m7 = M
    return m1 + m4 - m5 + m7, m3 + m5, m2 + m4, m1 - m2 + m3 + m6


def _strassen(mm, transposed):
    def assemble(c11, c12, c21, c22):
        if transposed:
            c12, c21 = c21, c12
        return jnp.concatenate([jnp.concatenate([c11, c12], axis=1), jnp.concatenate([c21, c22], axis=1)], axis=0)

    def rec(base, lev):
        M = [None] * 7
        for i in ORDER:
            M[i] = mm(base * 7 + i) if lev == 1 else assemble(*rec(base * 7 + i, lev - 1)[0])
        return _combine(M), M
    return rec(0, LEV)


def _kernel(zero_smem, beta_ref, x_hbm, wq_hbm, wk_hbm, wv_hbm, wo_hbm, wr_hbm,
            wg_hbm, wu_hbm, wd_hbm, out_hbm,
            x1_sc, xb_sc, xn_sc, mean_sc, rs_sc, kn_sc, r_sc, tk_sc, tq_sc, tv_sc, to_sc,
            wq_sc, wk_sc, wv_sc, wo_sc, wT_sc, wr_sc,
            wg_sc, wu_sc, wd_sc, k_sc, pk_sc, qT_sc, pqT_sc, vT_sc, o_sc, z_sc,
            gt_sc, am_sc, sems, osems, xsems, ksems, *s_sc):
    cp = {
        "wq": pltpu.make_async_copy(wq_hbm, wq_sc, sems.at[0]),
        "wv": pltpu.make_async_copy(wv_hbm, wv_sc, sems.at[1]),
        "wo": pltpu.make_async_copy(wo_hbm, wo_sc, sems.at[2]),
        "wr": pltpu.make_async_copy(wr_hbm, wr_sc, sems.at[3]),
        "wg": pltpu.make_async_copy(wg_hbm, wg_sc, sems.at[4]),
        "wu": pltpu.make_async_copy(wu_hbm, wu_sc, sems.at[5]),
        "wd": pltpu.make_async_copy(wd_hbm, wd_sc, sems.at[6]),
    }

    def x_copy(rb):
        rows = pl.ds(pl.multiple_of(rb * RB, RB), RB)
        return pltpu.make_async_copy(x_hbm.at[rows, :], xb_sc.at[rows, :], xsems.at[rb])

    def wk_copy(n, part):
        rows = pl.ds(part * BD + n * (BD // NWK), BD // NWK)
        return pltpu.make_async_copy(wk_hbm.at[rows, :], wk_sc.at[rows, :], ksems.at[n, part])

    def out_copy(i):
        rows = pl.ds(0, PRO * CH) if isinstance(i, int) and i == 0 else pl.ds(pl.multiple_of((PRO + (i - 1) * CPS) * CH, CH), CPS * CH)
        return pltpu.make_async_copy(xb_sc.at[rows, :], out_hbm.at[rows, :], osems.at[i])

    x_copy(0).start()
    zero = zero_smem[0]

    am_sc[...] = jnp.zeros((T, 4 * T), f32)

    gates = _sigmoid(beta_ref[...].reshape(1, H).astype(f32))
    for h in range(H):
        gt_sc[h] = jnp.broadcast_to(gates[:, h:h + 1], (8, 128))

    row = lax.broadcasted_iota(jnp.int32, (T, T), 0)
    col = lax.broadcasted_iota(jnp.int32, (T, T), 1)
    cmask = row <= col
    hmask = (row // 32) == (col // 32)
    zrow = lax.broadcasted_iota(jnp.int32, (32, T), 0)
    zcol = lax.broadcasted_iota(jnp.int32, (32, T), 1)
    zmask = (zrow // 8) == (zcol // 32)

    def rows_of(rb):
        return pl.ds(pl.multiple_of(rb * RB, RB), RB)

    def prep_nat(t_ref, w_ref):
        lax.fori_loop(0, NPC, lambda n, c: (_prep(t_ref, w_ref, n, NPC, False), c)[1], 0)

    def prep_tr(t_ref, w_ref):
        for j in range(4):
            for i in range(4):
                wT_sc[256 * j:256 * (j + 1), 256 * i:256 * (i + 1)] = w_ref[256 * i:256 * (i + 1), 256 * j:256 * (j + 1)].T
        lax.fori_loop(0, NPC, lambda n, c: (_prep(t_ref, wT_sc, n, NPC, True), c)[1], 0)

    QUADS = lambda c: ((c[1], 0, 1), (c[2], 1, 0), (c[0], 0, 0), (c[3], 1, 1))

    def ln_input(rb):
        x_copy(rb).wait()
        if isinstance(rb, int):
            for n in range(NWK):
                for part in range(1 << LEV):
                    wk_copy(n, part).start()
        for n in range(RB // 128):
            rows = pl.ds(pl.multiple_of(rb * RB + n * 128, 128), 128)
            x = xb_sc[rows, :].astype(f32)
            c = x - jnp.mean(x, axis=-1, keepdims=True)
            v = jnp.mean(c * c, axis=-1, keepdims=True)
            xn_sc[rows, :] = (c * lax.rsqrt(v + EPS)).astype(bf16)

    def proj_k_body(layer, rb, carry):
        @pl.when(layer == 0)
        def _():
            @pl.when(rb == 0)
            def _():
                for i in range(1, NRB):
                    x_copy(i).start()
            for j, name in ((1, "wq"), (1, "wv"), (2, "wo"), (3, "wr")):
                @pl.when(rb == j)
                def _():
                    cp[name].start()

            @pl.when(rb > 0)
            def _():
                ln_input(rb)
        h = RB // 2
        r0 = pl.multiple_of(rb * RB, RB)
        A = _lhs_ops(xn_sc[rows_of(rb), :], LEV)
        c, _ = _strassen(lambda i: jnp.dot(A[i], tk_sc[i], preferred_element_type=f32), False)
        zp = [None, None]
        for kk, th, nh in QUADS(c):
            pk = _phi(kk)
            zz = _row_fold(pk, jnp.add)
            zp[nh] = zz if zp[nh] is None else zp[nh] + zz
            rows = pl.ds(pl.multiple_of(r0 + th * h, h), h)
            for g in range(G // 2):
                k_sc[4 * nh + g, rows, :] = kk[:, 128 * g:128 * (g + 1)].astype(bf16)
                pk_sc[4 * nh + g, rows, :] = pk[:, 128 * g:128 * (g + 1)].astype(bf16)
        for nh in range(2):
            for g in range(G // 2):
                z_sc[rb, 4 * nh + g] = zp[nh][:, 128 * g:128 * (g + 1)]
        return carry

    def proj_qv_body(layer, rb, carry):
        @pl.when(jnp.logical_and(layer == 0, rb == 0))
        def _():
            for name in ("wg", "wu", "wd"):
                cp[name].start()
        h = RB // 2
        A = _lhs_ops(xn_sc[rows_of(rb), :], LEV)
        c, _ = _strassen(lambda i: lax.dot_general(tq_sc[i], A[i], NT, preferred_element_type=f32), True)
        for qq, th, nh in QUADS(c):
            pq = _phi(qq)
            for g in range(G // 2):
                qT_sc[rb, 4 * nh + g, :, th * h:(th + 1) * h] = (qq[128 * g:128 * (g + 1)] * QSCALE).astype(bf16)
                pqT_sc[rb, 4 * nh + g, :, th * h:(th + 1) * h] = pq[128 * g:128 * (g + 1)].astype(bf16)
        c, _ = _strassen(lambda i: lax.dot_general(tv_sc[i], A[i], NT, preferred_element_type=f32), True)
        for vv, th, nh in QUADS(c):
            for g in range(G // 2):
                vT_sc[rb, 4 * nh + g, :, th * h:(th + 1) * h] = vv[128 * g:128 * (g + 1)].astype(bf16)
        return carry

    TILES = [(s, i) for s in range(NSEG) for i in (3, 2, 1, 0)]
    STREAM = [(t, c) for t, (s, i) in enumerate(TILES) for c in range(i + 1)]
    NPOS = len(STREAM)

    def sref(k, h):
        return s_sc[k % NSLOT].at[pl.ds(pl.multiple_of(zero, 8), T), T * h:T * (h + 1)]

    def tcols(ref, g, t0, n, rows=slice(None)):
        parts = []
        for t in range(t0, t0 + n, min(n, RB)):
            parts.append(ref[t // RB, g, rows, t % RB:t % RB + min(n, RB)])
        return parts[0] if len(parts) == 1 else jnp.concatenate(parts, axis=1)

    def q_weights(g, s, i):
        QT = tcols(qT_sc, g, s * L + i * T, T)
        z = jnp.zeros((32, T), bf16)
        return jnp.concatenate(
            [jnp.concatenate([QT[32 * h:32 * h + 32] if hh == h else z for hh in range(4)], axis=0)
             for h in range(4)], axis=1)

    def qk(g, k, m):
        t, c = STREAM[k]
        s, i = TILES[t]
        k0 = s * L + c * T
        K = k_sc[g, k0:k0 + T, :]
        S4 = jnp.dot(K, q_weights(g, s, i), preferred_element_type=f32)
        out = []
        for h in range(4):
            Sx = S4[:, T * h:T * (h + 1)]
            if c == i:
                Sx = jnp.where(cmask, Sx, NEG)
            sref(k, h)[...] = Sx
            mm = Sx[0:8]
            for r in range(1, 16):
                mm = jnp.maximum(mm, Sx[8 * r:8 * r + 8])
            mm = mm if c == 0 else jnp.maximum(m[h], mm)
            if c == i:
                mm = jnp.broadcast_to(jnp.max(mm, axis=0, keepdims=True), (8, T))
            out.append(mm)
        return out

    def attn_prologue():
        m = {}
        for k in range(LAG):
            t = STREAM[k][0]
            m[t] = qk(0, k, m.get(t))
        return tuple(m[STREAM[0][0]]) + tuple(m[STREAM[LAG - 1][0]])

    def finish(g, s, i, O, l):
        outs = []
        for h in range(4):
            lt = jnp.sum(l[h], axis=0, keepdims=True)
            gt = jnp.concatenate([gt_sc[4 * g + h]] * 4, axis=0)
            o = O[h] * ((1.0 - gt) * (1.0 / lt))
            if s > 0:
                o = o + am_sc[32 * h:32 * h + 32, i * T:(i + 1) * T]
            outs.append(o)
        ot = jnp.concatenate(outs, axis=0).astype(bf16)
        r0 = s * L + i * T
        o_sc[g, r0:r0 + T, :] = ot.T

    def attn_body(g, carry):
        gn = jnp.minimum(g + 1, G - 1)
        m = {STREAM[0][0]: list(carry[0:4]), STREAM[LAG - 1][0]: list(carry[4:8])}
        l, O, P, M, mn = {}, {}, {}, {}, {}

        def mem_read(s):
            zs = z_sc[0, g]
            for rb in range(1, s * L // RB):
                zs = zs + z_sc[rb, g]
            zs = jnp.sum(zs, axis=0, keepdims=True)
            zrows = jnp.where(zmask, zs, 0.0).astype(bf16)
            mbd = jnp.where(hmask, M[0], 0.0).astype(bf16)
            lhs = jnp.concatenate([mbd, zrows], axis=0)
            pq = tcols(pqT_sc, g, s * L, L)
            nd = jnp.dot(lhs, pq, preferred_element_type=f32)
            for h in range(4):
                den = nd[128 + 8 * h:128 + 8 * h + 8] + 1e-06
                gd = jnp.concatenate([gt_sc[4 * g + h]] * 4, axis=1) / den
                am_sc[32 * h:32 * h + 32, :] = nd[32 * h:32 * h + 32] * jnp.concatenate([gd] * 4, axis=0)

        def mem_write(s):
            vt = tcols(vT_sc, g, s * L, L)
            pk = pk_sc[g, s * L:(s + 1) * L, :]
            inc = jnp.dot(vt, pk, preferred_element_type=f32)
            M[0] = inc if s == 0 else M[0] + inc

        def ex(k):
            t, c = STREAM[k]
            out = []
            for h in range(4):
                Pp = jnp.exp2(sref(k, h)[...] - jnp.concatenate([m[t][h]] * (T // 8), axis=0))
                a = Pp[0:8] + Pp[8:16]
                b = Pp[16:24] + Pp[24:32]
                for r in range(2, 8, 2):
                    a = a + (Pp[16 * r:16 * r + 8] + Pp[16 * r + 8:16 * r + 16])
                    b = b + (Pp[16 * r + 16:16 * r + 24] + Pp[16 * r + 24:16 * r + 32])
                ll = a + b
                if c == 0:
                    l.setdefault(t, [None] * 4)[h] = ll
                else:
                    l[t][h] = l[t][h] + ll
                out.append(Pp.astype(bf16))
            P[k] = out

        def pv(k):
            t, c = STREAM[k]
            s, i = TILES[t]
            if c == 0:
                O[t] = [None] * 4
            for h in range(4):
                vt = tcols(vT_sc, g, s * L + c * T, T, slice(32 * h, 32 * h + 32))
                o = jnp.dot(vt, P[k][h], preferred_element_type=f32)
                O[t][h] = o if O[t][h] is None else O[t][h] + o
            del P[k]

        finish(jnp.maximum(g - 1, 0), NSEG - 1, 0, carry[8:12], carry[12:16])
        done = None
        for j in range(NPOS):
            ex(j)
            k = j + LAG
            if k < NPOS:
                t = STREAM[k][0]
                m[t] = qk(g, k, m.get(t))
            else:
                t = STREAM[k - NPOS][0]
                mn[t] = qk(gn, k - NPOS, mn.get(t))
            pv(j)
            if done is not None:
                s, i = TILES[done]
                finish(g, s, i, O[done], l[done])
                if i == 0:
                    mem_read(s + 1)
                done = None
            t, c = STREAM[j]
            if c == TILES[t][1]:
                done = t
                if TILES[t][1] == 3 and TILES[t][0] < NSEG - 1:
                    mem_write(TILES[t][0])
        return (tuple(mn[STREAM[0][0]]) + tuple(mn[STREAM[LAG - 1][0]]) + tuple(O[done]) + tuple(l[done]))

    def attn_phase():
        init = attn_prologue() + (jnp.zeros((32, T), f32),) * 4 + (jnp.ones((8, T), f32),) * 4
        carry = lax.fori_loop(0, G, attn_body, init, unroll=2)
        finish(G - 1, NSEG - 1, 0, carry[8:12], carry[12:16])

    def out_body(ob_i, carry):
        wr = wr_sc[...].reshape(1, D).astype(f32)
        wr_sum = jnp.sum(wr, axis=-1, keepdims=True)
        h = RB // 2
        for k in range(OB // RB):
            r0 = pl.multiple_of(ob_i * OB + k * RB, RB)
            ob = jnp.concatenate([o_sc[g, pl.ds(r0, RB), :] for g in range(G)], axis=1)
            A = _lhs_ops(ob, LEV)
            c, _ = _strassen(lambda i: jnp.dot(A[i], _upk(to_sc[i]), preferred_element_type=f32), False)
            acc = [[None] * 3, [None] * 3]
            for cc, th, nh in QUADS(c):
                rows = pl.ds(pl.multiple_of(r0 + th * h, h), h)
                cols = slice(nh * HD, (nh + 1) * HD)
                x1 = xb_sc[rows, cols].astype(f32) + cc
                x1_sc[rows, cols] = x1
                s1, s2, st = acc[th]
                for n in range(HD // 128):
                    d = x1[:, 128 * n:128 * (n + 1)]
                    s1 = d if s1 is None else s1 + d
                    s2 = d * d if s2 is None else s2 + d * d
                    t = d * wr[:, nh * HD + 128 * n:nh * HD + 128 * (n + 1)]
                    st = t if st is None else st + t
                acc[th] = [s1, s2, st]
            for th in range(2):
                for b in range(h // 128):
                    s1, s2, st = (jnp.sum(t[128 * b:128 * (b + 1)].T, axis=0, keepdims=True) for t in acc[th])
                    mean = s1 * (1.0 / D)
                    v = jnp.maximum(s2 * (1.0 / D) - mean * mean, 0.0)
                    rs = lax.rsqrt(v + EPS)
                    r = rs * (st - mean * wr_sum)
                    a = 1.0 + rs
                    blk = pl.ds(ob_i * (OB // 128) + k * (RB // 128) + th * (h // 128) + b, 1)
                    mean_sc[blk, :] = mean
                    rs_sc[blk, :] = rs
                    kn_sc[blk, :] = a * lax.rsqrt(v * (a * a) + EPS)
                    r_sc[blk, :] = r.astype(bf16).astype(f32)
        return carry

    def out_phase():
        lax.fori_loop(0, NOB, out_body, 0)

    def ffn(layer):
        R = r_sc[...]
        bits = pltpu.bitcast(jnp.where(R == 0.0, 0.0, R), jnp.int32)
        idx = (lax.broadcasted_iota(jnp.int32, bits.shape, 0) * 128 + lax.broadcasted_iota(jnp.int32, bits.shape, 1))
        key = (jnp.where(bits < 0, bits ^ 0x7FFFFFFF, bits) & -65536) | (S - 1 - idx)

        def top(k):
            k1 = jnp.max(jnp.max(k, axis=0, keepdims=True), axis=1, keepdims=True)
            v = pltpu.bitcast(jnp.where(k1 < 0, k1 ^ 0x7FFFFFFF, k1) & -65536, f32)
            return k1, v, S - 1 - (k1[0, 0] & (S - 1))
        k1, v1, t1 = top(key)
        _, v2, t2 = top(jnp.where(key == k1, -2 ** 31, key))
        b1 = pl.ds(pl.multiple_of((t1 // 8) * 8, 8), 8)
        b2 = pl.ds(pl.multiple_of((t2 // 8) * 8, 8), 8)

        x1r = jnp.concatenate([x1_sc[b1, :], x1_sc[b2, :]], axis=0)
        mr = jnp.mean(x1r, axis=-1, keepdims=True)
        vr = jnp.maximum(jnp.mean(x1r * x1r, axis=-1, keepdims=True) - mr * mr, 0.0)
        xm = (x1r - mr) * lax.rsqrt(vr + EPS)
        xs = xm.astype(bf16)
        base = x1r + xm

        def mod_rows(n):
            rows = pl.ds(pl.multiple_of(n * CH, CH), CH)

            def per_row(ref):
                t = jnp.broadcast_to(ref[pl.ds(n, 1), :], (CH, 128)).T
                return jnp.concatenate([t] * (D // 128), axis=1)
            x1 = x1_sc[rows, :]
            c = x1 - per_row(mean_sc)
            xb_sc[rows, :] = (x1 + c * per_row(rs_sc)).astype(bf16)
            xn_sc[rows, :] = (c * per_row(kn_sc)).astype(bf16)

        def gate_up(j):
            cols = pl.ds(pl.multiple_of(j * FC, FC), FC)
            gg = jnp.dot(xs, wg_sc[:, cols], preferred_element_type=f32)
            uu = jnp.dot(xs, wu_sc[:, cols], preferred_element_type=f32)
            return (gg * _sigmoid(gg) * uu).astype(bf16)

        def down(j, hh):
            return jnp.dot(hh, wd_sc[pl.ds(pl.multiple_of(j * FC, FC), FC), :], preferred_element_type=f32)

        def step(j, carry):
            y, hh = carry

            @pl.when(jnp.logical_and(layer == 1, j > 1))
            def _():
                out_copy(j - 1).start()
            hn = gate_up(j)
            y = y + down(j - 1, hh)
            for i in range(CPS):
                mod_rows(PRO + (j - 1) * CPS + i)
            return y, hn

        for n in range(PRO):
            mod_rows(n)
        hh = gate_up(0)

        @pl.when(layer == 1)
        def _():
            out_copy(0).start()
        y, hh = lax.fori_loop(1, NOUT, step, (jnp.zeros((16, D), f32), hh))

        @pl.when(layer == 1)
        def _():
            out_copy(NOUT - 1).start()
        for j in range(NOUT, F // FC):
            hn = gate_up(j)
            y = y + down(j - 1, hh)
            hh = hn
        y = y + down(F // FC - 1, hh)
        r8 = lax.broadcasted_iota(jnp.int32, (8, D), 0)
        y1 = jnp.where(r8 == t1 % 8, y[0:8] * _sigmoid(v1), 0.0)
        y2 = jnp.where(r8 == t2 % 8, y[8:16] * _sigmoid(v2), 0.0)
        same = t1 // 8 == t2 // 8
        n1 = base[0:8] + (y1 + jnp.where(same, y2, 0.0))
        n2 = base[8:16] + (y2 + jnp.where(same, y1, 0.0))

        @pl.when(layer == 1)
        def _():
            for i in range(NOUT):
                out_copy(i).wait()

        for b, xx in ((b1, n1), (b2, n2)):
            xb_sc[b, :] = xx.astype(bf16)
            cc = xx - jnp.mean(xx, axis=-1, keepdims=True)
            xn_sc[b, :] = (cc * lax.rsqrt(jnp.mean(cc * cc, axis=-1, keepdims=True) + EPS)).astype(bf16)

        @pl.when(layer == 1)
        def _():
            c1 = pltpu.make_async_copy(xb_sc.at[b1, :], out_hbm.at[b1, :], sems.at[7])
            c1.start()

            @pl.when(jnp.logical_not(same))
            def _():
                c2 = pltpu.make_async_copy(xb_sc.at[b2, :], out_hbm.at[b2, :], sems.at[8])
                c2.start()
                c2.wait()
            c1.wait()

    def prep_k_piece(n, c):
        for part in range(1 << LEV):
            wk_copy(n, part).wait()
        return lax.fori_loop(n * (NPC // NWK), (n + 1) * (NPC // NWK),
                             lambda m, c_: (_prep(tk_sc, wk_sc, m, NPC, False), c_)[1], c)

    ln_input(0)
    lax.fori_loop(0, NWK, prep_k_piece, 0)

    def layer_body(layer, carry):
        first = layer == 0
        lax.fori_loop(0, NRB, functools.partial(proj_k_body, layer), 0)

        @pl.when(first)
        def _():
            cp["wq"].wait()
            prep_tr(tq_sc, wq_sc)
            cp["wv"].wait()
            prep_tr(tv_sc, wv_sc)
        lax.fori_loop(0, NRB, functools.partial(proj_qv_body, layer), 0)
        attn_phase()

        @pl.when(first)
        def _():
            cp["wo"].wait()
            cp["wr"].wait()
            prep_nat(to_sc, wo_sc)
        out_phase()

        @pl.when(first)
        def _():
            cp["wg"].wait()
            cp["wu"].wait()
            cp["wd"].wait()
        ffn(layer)
        return carry

    lax.fori_loop(0, 2, layer_body, 0)


@jax.jit
def pallas_interleave_layers__memory_aug_infini_attn__moe_arch_mod__prompt_kernel(
    A_x: jax.Array,
    A_wq: jax.Array,
    A_wk: jax.Array,
    A_wv: jax.Array,
    A_wo: jax.Array,
    A_beta: jax.Array,
    B_x: jax.Array,
    B_w_r: jax.Array,
    B_w_gate: jax.Array,
    B_w_up: jax.Array,
    B_w_down: jax.Array,
):
    del B_x
    x = A_x.reshape(S, D)
    zero = jnp.zeros((1,), jnp.int32)
    any_spec = pl.BlockSpec(memory_space=pl.ANY)
    smem_spec = pl.BlockSpec(memory_space=pltpu.SMEM)
    V = pltpu.VMEM
    scratch = [
        V((S, D), f32),
        V((S, D), bf16),
        V((S, D), bf16),
        V((S // 128, 128), f32), V((S // 128, 128), f32), V((S // 128, 128), f32), V((S // 128, 128), f32),
            V((NP, BD, BD), bf16), V((NP, BD, BD), bf16), V((NP, BD, BD), bf16),
        V((NP, BD // 2, BD), u32),
    ] + [
        V((D, D), bf16), V((D, D), bf16), V((D, D), bf16), V((D, D), bf16),
        V((D, D), bf16),
        V((D,), bf16),
        V((D, F), bf16), V((D, F), bf16), V((F, D), bf16),
        V((G, S, 128), bf16), V((G, S, 128), bf16),
        V((NRB, G, 128, RB), bf16), V((NRB, G, 128, RB), bf16), V((NRB, G, 128, RB), bf16),
        V((G, S, 128), bf16),
        V((NRB, G, 8, 128), f32),
        V((H, 8, 128), f32),
        V((T, 4 * T), f32),
        pltpu.SemaphoreType.DMA((9,)),
        pltpu.SemaphoreType.DMA((NOUT,)),
        pltpu.SemaphoreType.DMA((NRB,)),
        pltpu.SemaphoreType.DMA((NWK, 1 << LEV)),
    ] + [V((T, 4 * T), f32)] * NSLOT
    out = pl.pallas_call(
        _kernel,
        in_specs=[smem_spec, pl.BlockSpec(memory_space=pltpu.VMEM)] + [any_spec] * 9,
        out_specs=any_spec,
        out_shape=jax.ShapeDtypeStruct((S, D), bf16),
        scratch_shapes=scratch,
        compiler_params=pltpu.CompilerParams(vmem_limit_bytes=120 * 1024 * 1024),
    )(zero, A_beta, x, A_wq, A_wk, A_wv, A_wo, B_w_r, B_w_gate, B_w_up, B_w_down)
    return out.reshape(1, S, D)
```

```python
import functools
import itertools

import jax
import jax.numpy as jnp
from jax import lax
import jax.experimental.pallas as pl
import jax.experimental.pallas.tpu as pltpu

S, D, H, DH, NSEG, L, F = 2048, 1024, 32, 32, 4, 512, 3584
G = 8
LEV = 2
NP = 7 ** LEV
BD = D >> LEV
HD = D // 2
RB = 128 << LEV
NRB = S // RB
OB = 1024
NOB = S // OB
CH = 128
CPS = 3
PRO = 4
NOUT = 1 + (S // CH - PRO) // CPS
FC = 256
NWK = 4
NPC = 16
T = 128
LAG = 5
NSLOT = 5
EPS = 1e-05
LOG2E = 1.4426950408889634
QSCALE = (DH ** -0.5) * LOG2E
NEG = -1e30
NT = (((1,), (1,)), ((), ()))
ORDER = (2, 4, 3, 1, 0, 6, 5)

f32 = jnp.float32
bf16 = jnp.bfloat16
u32 = jnp.uint32


def _phi(t):
    return jnp.where(t > 0, t + 1.0, jnp.exp(t))


def _sigmoid(t):
    return 1.0 / (1.0 + jnp.exp(-t))


def _pk(x):
    return pltpu.bitcast(x, u32)


def _upk(x):
    return pltpu.bitcast(x, bf16)


def _row_fold(x, op):
    parts = [x[8 * r:8 * r + 8] for r in range(x.shape[0] // 8)]
    while len(parts) > 1:
        parts = [op(parts[i], parts[i + 1]) if i + 1 < len(parts) else parts[i] for i in range(0, len(parts), 2)]
    return parts[0]


def _quads(x):
    h, w = x.shape[0] // 2, x.shape[1] // 2
    return x[:h, :w], x[:h, w:], x[h:, :w], x[h:, w:]


def _lhs_ops(x, lev):
    if lev == 0:
        return [x.astype(bf16)]
    x00, x01, x10, x11 = _quads(x)
    a00, a01, a10, a11 = (t.astype(f32) for t in (x00, x01, x10, x11))
    ops = (a00 + a11, a10 + a11, x00, x11, a00 + a01, a10 - a00, a01 - a11)
    return [o for t in ops for o in _lhs_ops(t, lev - 1)]


def _rhs_ops(w, lev):
    if lev == 0:
        return [w[()].astype(bf16)]

    def sub(r, c):
        return {p[1:]: v for p, v in w.items() if p[0] == (r, c)}

    def add(x, y, sign=1):
        return {p: (x[p].astype(f32) + y[p].astype(f32) if sign > 0 else x[p].astype(f32) - y[p].astype(f32))
                for p in x}
    b11, b12, b21, b22 = sub(0, 0), sub(0, 1), sub(1, 0), sub(1, 1)
    ops = (add(b11, b22), b11, add(b12, b22, -1), add(b21, b11, -1), b22, add(b11, b12), add(b21, b22))
    return [o for t in ops for o in _rhs_ops(t, lev - 1)]


def _offsets(path):
    r = sum(rc[0] * (D >> (i + 1)) for i, rc in enumerate(path))
    c = sum(rc[1] * (D >> (i + 1)) for i, rc in enumerate(path))
    return r, c


def _prep(t_ref, w_ref, n, nch, transposed):
    ch = BD // nch
    w = {}
    for path in itertools.product(((0, 0), (0, 1), (1, 0), (1, 1)), repeat=LEV):
        r, c = _offsets(path)
        if transposed:
            r, c = c, r
        w[path] = w_ref[pl.ds(pl.multiple_of(r + n * ch, ch), ch), c:c + BD]
    packed = t_ref.dtype == u32
    rows = pl.ds(pl.multiple_of(n * (ch // 2), ch // 2), ch // 2) if packed else pl.ds(pl.multiple_of(n * ch, ch), ch)
    for i, t in enumerate(_rhs_ops(w, LEV)):
        t_ref[i, rows, :] = _pk(t) if packed else t


def _combine(M):
    m1, m2, m3, m4, m5, m6, m7 = M
    return m1 + m4 - m5 + m7, m3 + m5, m2 + m4, m1 - m2 + m3 + m6


def _strassen(mm, transposed):
    def assemble(c11, c12, c21, c22):
        if transposed:
            c12, c21 = c21, c12
        return jnp.concatenate([jnp.concatenate([c11, c12], axis=1), jnp.concatenate([c21, c22], axis=1)], axis=0)

    def rec(base, lev):
        M = [None] * 7
        for i in ORDER:
            M[i] = mm(base * 7 + i) if lev == 1 else assemble(*rec(base * 7 + i, lev - 1)[0])
        return _combine(M), M
    return rec(0, LEV)


def _kernel(zero_smem, beta_ref, x_hbm, wq_hbm, wk_hbm, wv_hbm, wo_hbm, wr_hbm,
            wg_hbm, wu_hbm, wd_hbm, out_hbm,
            x1_sc, xb_sc, xn_sc, mean_sc, rs_sc, kn_sc, r_sc, tk_sc, tq_sc, tv_sc, to_sc,
            wq_sc, wk_sc, wv_sc, wo_sc, wT_sc, wr_sc,
            wg_sc, wu_sc, wd_sc, k_sc, pk_sc, qT_sc, pqT_sc, vT_sc, o_sc, z_sc,
            gt_sc, am_sc, sems, osems, xsems, ksems, *s_sc):
    cp = {
        "wq": pltpu.make_async_copy(wq_hbm, wq_sc, sems.at[0]),
        "wv": pltpu.make_async_copy(wv_hbm, wv_sc, sems.at[1]),
        "wo": pltpu.make_async_copy(wo_hbm, wo_sc, sems.at[2]),
        "wr": pltpu.make_async_copy(wr_hbm, wr_sc, sems.at[3]),
        "wg": pltpu.make_async_copy(wg_hbm, wg_sc, sems.at[4]),
        "wu": pltpu.make_async_copy(wu_hbm, wu_sc, sems.at[5]),
        "wd": pltpu.make_async_copy(wd_hbm, wd_sc, sems.at[6]),
    }

    def x_copy(rb):
        rows = pl.ds(pl.multiple_of(rb * RB, RB), RB)
        return pltpu.make_async_copy(x_hbm.at[rows, :], xb_sc.at[rows, :], xsems.at[rb])

    def wk_copy(n, part):
        rows = pl.ds(part * BD + n * (BD // NWK), BD // NWK)
        return pltpu.make_async_copy(wk_hbm.at[rows, :], wk_sc.at[rows, :], ksems.at[n, part])

    def out_copy(i):
        if isinstance(i, int) and i in (0, NOUT):
            rows = pl.ds(0, CH) if i == NOUT else pl.ds(CH, (PRO - 1) * CH)
        else:
            rows = pl.ds(pl.multiple_of((PRO + (i - 1) * CPS) * CH, CH), CPS * CH)
        return pltpu.make_async_copy(xb_sc.at[rows, :], out_hbm.at[rows, :], osems.at[i])

    x_copy(0).start()
    zero = zero_smem[0]

    am_sc[...] = jnp.zeros((T, 4 * T), f32)

    gates = _sigmoid(beta_ref[...].reshape(1, H).astype(f32))
    for h in range(H):
        gt_sc[h] = jnp.broadcast_to(gates[:, h:h + 1], (8, 128))

    row = lax.broadcasted_iota(jnp.int32, (T, T), 0)
    col = lax.broadcasted_iota(jnp.int32, (T, T), 1)
    cmask = row <= col
    hmask = (row // 32) == (col // 32)
    zrow = lax.broadcasted_iota(jnp.int32, (32, T), 0)
    zcol = lax.broadcasted_iota(jnp.int32, (32, T), 1)
    zmask = (zrow // 8) == (zcol // 32)

    def rows_of(rb):
        return pl.ds(pl.multiple_of(rb * RB, RB), RB)

    def prep_nat(t_ref, w_ref):
        lax.fori_loop(0, NPC, lambda n, c: (_prep(t_ref, w_ref, n, NPC, False), c)[1], 0)

    def prep_tr(t_ref, w_ref):
        for j in range(4):
            for i in range(4):
                wT_sc[256 * j:256 * (j + 1), 256 * i:256 * (i + 1)] = w_ref[256 * i:256 * (i + 1), 256 * j:256 * (j + 1)].T
        lax.fori_loop(0, NPC, lambda n, c: (_prep(t_ref, wT_sc, n, NPC, True), c)[1], 0)

    QUADS = lambda c: ((c[1], 0, 1), (c[2], 1, 0), (c[0], 0, 0), (c[3], 1, 1))

    def ln_input(rb):
        x_copy(rb).wait()
        if isinstance(rb, int):
            for n in range(NWK):
                for part in range(1 << LEV):
                    wk_copy(n, part).start()
        for n in range(RB // 128):
            rows = pl.ds(pl.multiple_of(rb * RB + n * 128, 128), 128)
            x = xb_sc[rows, :].astype(f32)
            c = x - jnp.mean(x, axis=-1, keepdims=True)
            v = jnp.mean(c * c, axis=-1, keepdims=True)
            xn_sc[rows, :] = (c * lax.rsqrt(v + EPS)).astype(bf16)

    def proj_k_body(layer, rb, carry):
        @pl.when(layer == 0)
        def _():
            @pl.when(rb == 0)
            def _():
                for i in range(1, NRB):
                    x_copy(i).start()
            for j, name in ((1, "wq"), (1, "wv"), (2, "wo"), (3, "wr")):
                @pl.when(rb == j)
                def _():
                    cp[name].start()

            @pl.when(rb > 0)
            def _():
                ln_input(rb)
        h = RB // 2
        r0 = pl.multiple_of(rb * RB, RB)
        A = _lhs_ops(xn_sc[rows_of(rb), :], LEV)
        c, _ = _strassen(lambda i: jnp.dot(A[i], tk_sc[i], preferred_element_type=f32), False)
        zp = [None, None]
        for kk, th, nh in QUADS(c):
            pk = _phi(kk)
            zz = _row_fold(pk, jnp.add)
            zp[nh] = zz if zp[nh] is None else zp[nh] + zz
            rows = pl.ds(pl.multiple_of(r0 + th * h, h), h)
            for g in range(G // 2):
                k_sc[4 * nh + g, rows, :] = kk[:, 128 * g:128 * (g + 1)].astype(bf16)
                pk_sc[4 * nh + g, rows, :] = pk[:, 128 * g:128 * (g + 1)].astype(bf16)
        for nh in range(2):
            for g in range(G // 2):
                z_sc[rb, 4 * nh + g] = zp[nh][:, 128 * g:128 * (g + 1)]
        return carry

    def proj_qv_body(layer, rb, carry):
        @pl.when(jnp.logical_and(layer == 0, rb == 0))
        def _():
            for name in ("wg", "wu", "wd"):
                cp[name].start()
        h = RB // 2
        A = _lhs_ops(xn_sc[rows_of(rb), :], LEV)
        c, _ = _strassen(lambda i: lax.dot_general(tq_sc[i], A[i], NT, preferred_element_type=f32), True)
        for qq, th, nh in QUADS(c):
            pq = _phi(qq)
            for g in range(G // 2):
                qT_sc[rb, 4 * nh + g, :, th * h:(th + 1) * h] = (qq[128 * g:128 * (g + 1)] * QSCALE).astype(bf16)
                pqT_sc[rb, 4 * nh + g, :, th * h:(th + 1) * h] = pq[128 * g:128 * (g + 1)].astype(bf16)
        c, _ = _strassen(lambda i: lax.dot_general(tv_sc[i], A[i], NT, preferred_element_type=f32), True)
        for vv, th, nh in QUADS(c):
            for g in range(G // 2):
                vT_sc[rb, 4 * nh + g, :, th * h:(th + 1) * h] = vv[128 * g:128 * (g + 1)].astype(bf16)
        return carry

    TILES = [(s, i) for s in range(NSEG) for i in (3, 2, 1, 0)]
    STREAM = [(t, c) for t, (s, i) in enumerate(TILES) for c in range(i + 1)]
    NPOS = len(STREAM)

    def sref(k, h):
        return s_sc[k % NSLOT].at[pl.ds(pl.multiple_of(zero, 8), T), T * h:T * (h + 1)]

    def tcols(ref, g, t0, n, rows=slice(None)):
        parts = []
        for t in range(t0, t0 + n, min(n, RB)):
            parts.append(ref[t // RB, g, rows, t % RB:t % RB + min(n, RB)])
        return parts[0] if len(parts) == 1 else jnp.concatenate(parts, axis=1)

    def q_weights(g, s, i):
        QT = tcols(qT_sc, g, s * L + i * T, T)
        z = jnp.zeros((32, T), bf16)
        return jnp.concatenate(
            [jnp.concatenate([QT[32 * h:32 * h + 32] if hh == h else z for hh in range(4)], axis=0)
             for h in range(4)], axis=1)

    def qk(g, k, m):
        t, c = STREAM[k]
        s, i = TILES[t]
        k0 = s * L + c * T
        K = k_sc[g, k0:k0 + T, :]
        S4 = jnp.dot(K, q_weights(g, s, i), preferred_element_type=f32)
        out = []
        for h in range(4):
            Sx = S4[:, T * h:T * (h + 1)]
            if c == i:
                Sx = jnp.where(cmask, Sx, NEG)
            sref(k, h)[...] = Sx
            mm = Sx[0:8]
            for r in range(1, 16):
                mm = jnp.maximum(mm, Sx[8 * r:8 * r + 8])
            mm = mm if c == 0 else jnp.maximum(m[h], mm)
            if c == i:
                mm = jnp.broadcast_to(jnp.max(mm, axis=0, keepdims=True), (8, T))
            out.append(mm)
        return out

    def attn_prologue():
        m = {}
        for k in range(LAG):
            t = STREAM[k][0]
            m[t] = qk(0, k, m.get(t))
        return tuple(m[STREAM[0][0]]) + tuple(m[STREAM[LAG - 1][0]])

    def finish(g, s, i, O, l):
        outs = []
        for h in range(4):
            lt = jnp.sum(l[h], axis=0, keepdims=True)
            gt = jnp.concatenate([gt_sc[4 * g + h]] * 4, axis=0)
            o = O[h] * ((1.0 - gt) * (1.0 / lt))
            if s > 0:
                o = o + am_sc[32 * h:32 * h + 32, i * T:(i + 1) * T]
            outs.append(o)
        ot = jnp.concatenate(outs, axis=0).astype(bf16)
        r0 = s * L + i * T
        o_sc[g, r0:r0 + T, :] = ot.T

    def attn_body(g, carry):
        gn = jnp.minimum(g + 1, G - 1)
        m = {STREAM[0][0]: list(carry[0:4]), STREAM[LAG - 1][0]: list(carry[4:8])}
        l, O, P, M, mn = {}, {}, {}, {}, {}

        def mem_read(s):
            zs = z_sc[0, g]
            for rb in range(1, s * L // RB):
                zs = zs + z_sc[rb, g]
            zs = jnp.sum(zs, axis=0, keepdims=True)
            zrows = jnp.where(zmask, zs, 0.0).astype(bf16)
            mbd = jnp.where(hmask, M[0], 0.0).astype(bf16)
            lhs = jnp.concatenate([mbd, zrows], axis=0)
            pq = tcols(pqT_sc, g, s * L, L)
            nd = jnp.dot(lhs, pq, preferred_element_type=f32)
            for h in range(4):
                den = nd[128 + 8 * h:128 + 8 * h + 8] + 1e-06
                gd = jnp.concatenate([gt_sc[4 * g + h]] * 4, axis=1) / den
                am_sc[32 * h:32 * h + 32, :] = nd[32 * h:32 * h + 32] * jnp.concatenate([gd] * 4, axis=0)

        def mem_write(s):
            vt = tcols(vT_sc, g, s * L, L)
            pk = pk_sc[g, s * L:(s + 1) * L, :]
            inc = jnp.dot(vt, pk, preferred_element_type=f32)
            M[0] = inc if s == 0 else M[0] + inc

        def ex(k):
            t, c = STREAM[k]
            out = []
            for h in range(4):
                Pp = jnp.exp2(sref(k, h)[...] - jnp.concatenate([m[t][h]] * (T // 8), axis=0))
                a = Pp[0:8] + Pp[8:16]
                b = Pp[16:24] + Pp[24:32]
                for r in range(2, 8, 2):
                    a = a + (Pp[16 * r:16 * r + 8] + Pp[16 * r + 8:16 * r + 16])
                    b = b + (Pp[16 * r + 16:16 * r + 24] + Pp[16 * r + 24:16 * r + 32])
                ll = a + b
                if c == 0:
                    l.setdefault(t, [None] * 4)[h] = ll
                else:
                    l[t][h] = l[t][h] + ll
                out.append(Pp.astype(bf16))
            P[k] = out

        def pv(k):
            t, c = STREAM[k]
            s, i = TILES[t]
            if c == 0:
                O[t] = [None] * 4
            for h in range(4):
                vt = tcols(vT_sc, g, s * L + c * T, T, slice(32 * h, 32 * h + 32))
                o = jnp.dot(vt, P[k][h], preferred_element_type=f32)
                O[t][h] = o if O[t][h] is None else O[t][h] + o
            del P[k]

        finish(jnp.maximum(g - 1, 0), NSEG - 1, 0, carry[8:12], carry[12:16])
        done = None
        for j in range(NPOS):
            ex(j)
            k = j + LAG
            if k < NPOS:
                t = STREAM[k][0]
                m[t] = qk(g, k, m.get(t))
            else:
                t = STREAM[k - NPOS][0]
                mn[t] = qk(gn, k - NPOS, mn.get(t))
            pv(j)
            if done is not None:
                s, i = TILES[done]
                finish(g, s, i, O[done], l[done])
                if i == 0:
                    mem_read(s + 1)
                done = None
            t, c = STREAM[j]
            if c == TILES[t][1]:
                done = t
                if TILES[t][1] == 3 and TILES[t][0] < NSEG - 1:
                    mem_write(TILES[t][0])
        return (tuple(mn[STREAM[0][0]]) + tuple(mn[STREAM[LAG - 1][0]]) + tuple(O[done]) + tuple(l[done]))

    def attn_phase():
        init = attn_prologue() + (jnp.zeros((32, T), f32),) * 4 + (jnp.ones((8, T), f32),) * 4
        carry = lax.fori_loop(0, G, attn_body, init, unroll=2)
        finish(G - 1, NSEG - 1, 0, carry[8:12], carry[12:16])

    def out_body(ob_i, carry):
        wr = wr_sc[...].reshape(1, D).astype(f32)
        wr_sum = jnp.sum(wr, axis=-1, keepdims=True)
        h = RB // 2
        for k in range(OB // RB):
            r0 = pl.multiple_of(ob_i * OB + k * RB, RB)
            ob = jnp.concatenate([o_sc[g, pl.ds(r0, RB), :] for g in range(G)], axis=1)
            A = _lhs_ops(ob, LEV)
            c, _ = _strassen(lambda i: jnp.dot(A[i], _upk(to_sc[i]), preferred_element_type=f32), False)
            acc = [[None] * 3, [None] * 3]
            for cc, th, nh in QUADS(c):
                rows = pl.ds(pl.multiple_of(r0 + th * h, h), h)
                cols = slice(nh * HD, (nh + 1) * HD)
                x1 = xb_sc[rows, cols].astype(f32) + cc
                x1_sc[rows, cols] = x1
                s1, s2, st = acc[th]
                for n in range(HD // 128):
                    d = x1[:, 128 * n:128 * (n + 1)]
                    s1 = d if s1 is None else s1 + d
                    s2 = d * d if s2 is None else s2 + d * d
                    t = d * wr[:, nh * HD + 128 * n:nh * HD + 128 * (n + 1)]
                    st = t if st is None else st + t
                acc[th] = [s1, s2, st]
            for th in range(2):
                for b in range(h // 128):
                    s1, s2, st = (jnp.sum(t[128 * b:128 * (b + 1)].T, axis=0, keepdims=True) for t in acc[th])
                    mean = s1 * (1.0 / D)
                    v = jnp.maximum(s2 * (1.0 / D) - mean * mean, 0.0)
                    rs = lax.rsqrt(v + EPS)
                    r = rs * (st - mean * wr_sum)
                    a = 1.0 + rs
                    blk = pl.ds(ob_i * (OB // 128) + k * (RB // 128) + th * (h // 128) + b, 1)
                    mean_sc[blk, :] = mean
                    rs_sc[blk, :] = rs
                    kn_sc[blk, :] = a * lax.rsqrt(v * (a * a) + EPS)
                    r_sc[blk, :] = r.astype(bf16).astype(f32)
        return carry

    def out_phase():
        lax.fori_loop(0, NOB, out_body, 0)

    def ffn(layer):
        R = r_sc[...]
        bits = pltpu.bitcast(jnp.where(R == 0.0, 0.0, R), jnp.int32)
        idx = (lax.broadcasted_iota(jnp.int32, bits.shape, 0) * 128 + lax.broadcasted_iota(jnp.int32, bits.shape, 1))
        key = (jnp.where(bits < 0, bits ^ 0x7FFFFFFF, bits) & -65536) | (S - 1 - idx)

        def top(k):
            k1 = jnp.max(jnp.max(k, axis=0, keepdims=True), axis=1, keepdims=True)
            v = pltpu.bitcast(jnp.where(k1 < 0, k1 ^ 0x7FFFFFFF, k1) & -65536, f32)
            return k1, v, S - 1 - (k1[0, 0] & (S - 1))
        k1, v1, t1 = top(key)
        _, v2, t2 = top(jnp.where(key == k1, -2 ** 31, key))
        b1 = pl.ds(pl.multiple_of((t1 // 8) * 8, 8), 8)
        b2 = pl.ds(pl.multiple_of((t2 // 8) * 8, 8), 8)

        x1r = jnp.concatenate([x1_sc[b1, :], x1_sc[b2, :]], axis=0)
        mr = jnp.mean(x1r, axis=-1, keepdims=True)
        vr = jnp.maximum(jnp.mean(x1r * x1r, axis=-1, keepdims=True) - mr * mr, 0.0)
        xm = (x1r - mr) * lax.rsqrt(vr + EPS)
        xs = xm.astype(bf16)
        base = x1r + xm

        def mod_rows(n):
            rows = pl.ds(pl.multiple_of(n * CH, CH), CH)

            def per_row(ref):
                t = jnp.broadcast_to(ref[pl.ds(n, 1), :], (CH, 128)).T
                return jnp.concatenate([t] * (D // 128), axis=1)
            x1 = x1_sc[rows, :]
            c = x1 - per_row(mean_sc)
            xb_sc[rows, :] = (x1 + c * per_row(rs_sc)).astype(bf16)
            xn_sc[rows, :] = (c * per_row(kn_sc)).astype(bf16)

        def gate_up(j):
            cols = pl.ds(pl.multiple_of(j * FC, FC), FC)
            gg = jnp.dot(xs, wg_sc[:, cols], preferred_element_type=f32)
            uu = jnp.dot(xs, wu_sc[:, cols], preferred_element_type=f32)
            return (gg * _sigmoid(gg) * uu).astype(bf16)

        def down(j, hh):
            return jnp.dot(hh, wd_sc[pl.ds(pl.multiple_of(j * FC, FC), FC), :], preferred_element_type=f32)

        def step(j, carry):
            y, hh = carry

            @pl.when(jnp.logical_and(layer == 1, j > 1))
            def _():
                out_copy(j - 1).start()
            hn = gate_up(j)
            y = y + down(j - 1, hh)
            for i in range(CPS):
                mod_rows(PRO + (j - 1) * CPS + i)
            return y, hn

        for n in range(PRO):
            mod_rows(n)
            if n == 0:
                @pl.when(layer == 1)
                def _():
                    out_copy(NOUT).start()
        hh = gate_up(0)

        @pl.when(layer == 1)
        def _():
            out_copy(0).start()
        y, hh = lax.fori_loop(1, NOUT, step, (jnp.zeros((16, D), f32), hh))

        @pl.when(layer == 1)
        def _():
            out_copy(NOUT - 1).start()
        for j in range(NOUT, F // FC):
            hn = gate_up(j)
            y = y + down(j - 1, hh)
            hh = hn
        y = y + down(F // FC - 1, hh)
        r8 = lax.broadcasted_iota(jnp.int32, (8, D), 0)
        y1 = jnp.where(r8 == t1 % 8, y[0:8] * _sigmoid(v1), 0.0)
        y2 = jnp.where(r8 == t2 % 8, y[8:16] * _sigmoid(v2), 0.0)
        same = t1 // 8 == t2 // 8
        n1 = base[0:8] + (y1 + jnp.where(same, y2, 0.0))
        n2 = base[8:16] + (y2 + jnp.where(same, y1, 0.0))

        @pl.when(layer == 1)
        def _():
            for i in range(NOUT + 1):
                out_copy(i).wait()

        for b, xx in ((b1, n1), (b2, n2)):
            xb_sc[b, :] = xx.astype(bf16)
            cc = xx - jnp.mean(xx, axis=-1, keepdims=True)
            xn_sc[b, :] = (cc * lax.rsqrt(jnp.mean(cc * cc, axis=-1, keepdims=True) + EPS)).astype(bf16)

        @pl.when(layer == 1)
        def _():
            c1 = pltpu.make_async_copy(xb_sc.at[b1, :], out_hbm.at[b1, :], sems.at[7])
            c1.start()

            @pl.when(jnp.logical_not(same))
            def _():
                c2 = pltpu.make_async_copy(xb_sc.at[b2, :], out_hbm.at[b2, :], sems.at[8])
                c2.start()
                c2.wait()
            c1.wait()

    def prep_k_piece(n, c):
        for part in range(1 << LEV):
            wk_copy(n, part).wait()
        return lax.fori_loop(n * (NPC // NWK), (n + 1) * (NPC // NWK),
                             lambda m, c_: (_prep(tk_sc, wk_sc, m, NPC, False), c_)[1], c)

    ln_input(0)
    lax.fori_loop(0, NWK, prep_k_piece, 0)

    def layer_body(layer, carry):
        first = layer == 0
        lax.fori_loop(0, NRB, functools.partial(proj_k_body, layer), 0)

        @pl.when(first)
        def _():
            cp["wq"].wait()
            prep_tr(tq_sc, wq_sc)
            cp["wv"].wait()
            prep_tr(tv_sc, wv_sc)
        lax.fori_loop(0, NRB, functools.partial(proj_qv_body, layer), 0)
        attn_phase()

        @pl.when(first)
        def _():
            cp["wo"].wait()
            cp["wr"].wait()
            prep_nat(to_sc, wo_sc)
        out_phase()

        @pl.when(first)
        def _():
            cp["wg"].wait()
            cp["wu"].wait()
            cp["wd"].wait()
        ffn(layer)
        return carry

    lax.fori_loop(0, 2, layer_body, 0)


@jax.jit
def pallas_interleave_layers__memory_aug_infini_attn__moe_arch_mod__prompt_kernel(
    A_x: jax.Array,
    A_wq: jax.Array,
    A_wk: jax.Array,
    A_wv: jax.Array,
    A_wo: jax.Array,
    A_beta: jax.Array,
    B_x: jax.Array,
    B_w_r: jax.Array,
    B_w_gate: jax.Array,
    B_w_up: jax.Array,
    B_w_down: jax.Array,
):
    del B_x
    x = A_x.reshape(S, D)
    zero = jnp.zeros((1,), jnp.int32)
    any_spec = pl.BlockSpec(memory_space=pl.ANY)
    smem_spec = pl.BlockSpec(memory_space=pltpu.SMEM)
    V = pltpu.VMEM
    scratch = [
        V((S, D), f32),
        V((S, D), bf16),
        V((S, D), bf16),
        V((S // 128, 128), f32), V((S // 128, 128), f32), V((S // 128, 128), f32), V((S // 128, 128), f32),
            V((NP, BD, BD), bf16), V((NP, BD, BD), bf16), V((NP, BD, BD), bf16),
        V((NP, BD // 2, BD), u32),
    ] + [
        V((D, D), bf16), V((D, D), bf16), V((D, D), bf16), V((D, D), bf16),
        V((D, D), bf16),
        V((D,), bf16),
        V((D, F), bf16), V((D, F), bf16), V((F, D), bf16),
        V((G, S, 128), bf16), V((G, S, 128), bf16),
        V((NRB, G, 128, RB), bf16), V((NRB, G, 128, RB), bf16), V((NRB, G, 128, RB), bf16),
        V((G, S, 128), bf16),
        V((NRB, G, 8, 128), f32),
        V((H, 8, 128), f32),
        V((T, 4 * T), f32),
        pltpu.SemaphoreType.DMA((9,)),
        pltpu.SemaphoreType.DMA((NOUT + 1,)),
        pltpu.SemaphoreType.DMA((NRB,)),
        pltpu.SemaphoreType.DMA((NWK, 1 << LEV)),
    ] + [V((T, 4 * T), f32)] * NSLOT
    out = pl.pallas_call(
        _kernel,
        in_specs=[smem_spec, pl.BlockSpec(memory_space=pltpu.VMEM)] + [any_spec] * 9,
        out_specs=any_spec,
        out_shape=jax.ShapeDtypeStruct((S, D), bf16),
        scratch_shapes=scratch,
        compiler_params=pltpu.CompilerParams(vmem_limit_bytes=120 * 1024 * 1024),
    )(zero, A_beta, x, A_wq, A_wk, A_wv, A_wo, B_w_r, B_w_gate, B_w_up, B_w_down)
    return out.reshape(1, S, D)
```

```python
import functools
import itertools

import jax
import jax.numpy as jnp
from jax import lax
import jax.experimental.pallas as pl
import jax.experimental.pallas.tpu as pltpu

S, D, H, DH, NSEG, L, F = 2048, 1024, 32, 32, 4, 512, 3584
G = 8
LEV = 2
NP = 7 ** LEV
BD = D >> LEV
HD = D // 2
RB = 128 << LEV
NRB = S // RB
OB = 1024
NOB = S // OB
CH = 128
CPS = 3
PRO = 4
NOUT = 1 + (S // CH - PRO) // CPS
FC = 256
NWK = 4
NPC = 16
T = 128
LAG = 6
NSLOT = 8
EPS = 1e-05
LOG2E = 1.4426950408889634
QSCALE = (DH ** -0.5) * LOG2E
NEG = -1e30
NT = (((1,), (1,)), ((), ()))
ORDER = (2, 4, 3, 1, 0, 6, 5)

f32 = jnp.float32
bf16 = jnp.bfloat16
u32 = jnp.uint32


def _phi(t):
    return jnp.where(t > 0, t + 1.0, jnp.exp(t))


def _sigmoid(t):
    return 1.0 / (1.0 + jnp.exp(-t))


def _pk(x):
    return pltpu.bitcast(x, u32)


def _upk(x):
    return pltpu.bitcast(x, bf16)


def _row_fold(x, op):
    parts = [x[8 * r:8 * r + 8] for r in range(x.shape[0] // 8)]
    while len(parts) > 1:
        parts = [op(parts[i], parts[i + 1]) if i + 1 < len(parts) else parts[i] for i in range(0, len(parts), 2)]
    return parts[0]


def _quads(x):
    h, w = x.shape[0] // 2, x.shape[1] // 2
    return x[:h, :w], x[:h, w:], x[h:, :w], x[h:, w:]


def _lhs_ops(x, lev):
    if lev == 0:
        return [x.astype(bf16)]
    x00, x01, x10, x11 = _quads(x)
    a00, a01, a10, a11 = (t.astype(f32) for t in (x00, x01, x10, x11))
    ops = (a00 + a11, a10 + a11, x00, x11, a00 + a01, a10 - a00, a01 - a11)
    return [o for t in ops for o in _lhs_ops(t, lev - 1)]


def _rhs_ops(w, lev):
    if lev == 0:
        return [w[()].astype(bf16)]

    def sub(r, c):
        return {p[1:]: v for p, v in w.items() if p[0] == (r, c)}

    def add(x, y, sign=1):
        return {p: (x[p].astype(f32) + y[p].astype(f32) if sign > 0 else x[p].astype(f32) - y[p].astype(f32))
                for p in x}
    b11, b12, b21, b22 = sub(0, 0), sub(0, 1), sub(1, 0), sub(1, 1)
    ops = (add(b11, b22), b11, add(b12, b22, -1), add(b21, b11, -1), b22, add(b11, b12), add(b21, b22))
    return [o for t in ops for o in _rhs_ops(t, lev - 1)]


def _offsets(path):
    r = sum(rc[0] * (D >> (i + 1)) for i, rc in enumerate(path))
    c = sum(rc[1] * (D >> (i + 1)) for i, rc in enumerate(path))
    return r, c


def _prep(t_ref, w_ref, n, nch, transposed):
    ch = BD // nch
    w = {}
    for path in itertools.product(((0, 0), (0, 1), (1, 0), (1, 1)), repeat=LEV):
        r, c = _offsets(path)
        if transposed:
            r, c = c, r
        w[path] = w_ref[pl.ds(pl.multiple_of(r + n * ch, ch), ch), c:c + BD]
    packed = t_ref.dtype == u32
    rows = pl.ds(pl.multiple_of(n * (ch // 2), ch // 2), ch // 2) if packed else pl.ds(pl.multiple_of(n * ch, ch), ch)
    for i, t in enumerate(_rhs_ops(w, LEV)):
        t_ref[i, rows, :] = _pk(t) if packed else t


def _combine(M):
    m1, m2, m3, m4, m5, m6, m7 = M
    return m1 + m4 - m5 + m7, m3 + m5, m2 + m4, m1 - m2 + m3 + m6


def _strassen(mm, transposed):
    def assemble(c11, c12, c21, c22):
        if transposed:
            c12, c21 = c21, c12
        return jnp.concatenate([jnp.concatenate([c11, c12], axis=1), jnp.concatenate([c21, c22], axis=1)], axis=0)

    def rec(base, lev):
        M = [None] * 7
        for i in ORDER:
            M[i] = mm(base * 7 + i) if lev == 1 else assemble(*rec(base * 7 + i, lev - 1)[0])
        return _combine(M), M
    return rec(0, LEV)


def _kernel(zero_smem, beta_ref, x_hbm, wq_hbm, wk_hbm, wv_hbm, wo_hbm, wr_hbm,
            wg_hbm, wu_hbm, wd_hbm, out_hbm,
            x1_sc, xb_sc, xn_sc, mean_sc, rs_sc, kn_sc, r_sc, tk_sc, tq_sc, tv_sc, to_sc,
            wq_sc, wk_sc, wv_sc, wo_sc, wT_sc, wr_sc,
            wg_sc, wu_sc, wd_sc, k_sc, pk_sc, qT_sc, pqT_sc, vT_sc, o_sc, z_sc,
            gt_sc, am_sc, sems, osems, xsems, ksems, *s_sc):
    cp = {
        "wq": pltpu.make_async_copy(wq_hbm, wq_sc, sems.at[0]),
        "wv": pltpu.make_async_copy(wv_hbm, wv_sc, sems.at[1]),
        "wo": pltpu.make_async_copy(wo_hbm, wo_sc, sems.at[2]),
        "wr": pltpu.make_async_copy(wr_hbm, wr_sc, sems.at[3]),
        "wg": pltpu.make_async_copy(wg_hbm, wg_sc, sems.at[4]),
        "wu": pltpu.make_async_copy(wu_hbm, wu_sc, sems.at[5]),
        "wd": pltpu.make_async_copy(wd_hbm, wd_sc, sems.at[6]),
    }

    def x_copy(rb):
        rows = pl.ds(pl.multiple_of(rb * RB, RB), RB)
        return pltpu.make_async_copy(x_hbm.at[rows, :], xb_sc.at[rows, :], xsems.at[rb])

    def wk_copy(n, part):
        rows = pl.ds(part * BD + n * (BD // NWK), BD // NWK)
        return pltpu.make_async_copy(wk_hbm.at[rows, :], wk_sc.at[rows, :], ksems.at[n, part])

    def out_copy(i):
        if isinstance(i, int) and i in (0, NOUT):
            rows = pl.ds(0, CH) if i == NOUT else pl.ds(CH, (PRO - 1) * CH)
        else:
            rows = pl.ds(pl.multiple_of((PRO + (i - 1) * CPS) * CH, CH), CPS * CH)
        return pltpu.make_async_copy(xb_sc.at[rows, :], out_hbm.at[rows, :], osems.at[i])

    x_copy(0).start()
    zero = zero_smem[0]

    am_sc[...] = jnp.zeros((T, 4 * T), f32)

    gates = _sigmoid(beta_ref[...].reshape(1, H).astype(f32))
    for h in range(H):
        gt_sc[h] = jnp.broadcast_to(gates[:, h:h + 1], (8, 128))

    row = lax.broadcasted_iota(jnp.int32, (T, T), 0)
    col = lax.broadcasted_iota(jnp.int32, (T, T), 1)
    cmask = row <= col
    hmask = (row // 32) == (col // 32)
    zrow = lax.broadcasted_iota(jnp.int32, (32, T), 0)
    zcol = lax.broadcasted_iota(jnp.int32, (32, T), 1)
    zmask = (zrow // 8) == (zcol // 32)

    def rows_of(rb):
        return pl.ds(pl.multiple_of(rb * RB, RB), RB)

    def prep_nat(t_ref, w_ref):
        lax.fori_loop(0, NPC, lambda n, c: (_prep(t_ref, w_ref, n, NPC, False), c)[1], 0)

    def prep_tr(t_ref, w_ref):
        for j in range(4):
            for i in range(4):
                wT_sc[256 * j:256 * (j + 1), 256 * i:256 * (i + 1)] = w_ref[256 * i:256 * (i + 1), 256 * j:256 * (j + 1)].T
        lax.fori_loop(0, NPC, lambda n, c: (_prep(t_ref, wT_sc, n, NPC, True), c)[1], 0)

    QUADS = lambda c: ((c[1], 0, 1), (c[2], 1, 0), (c[0], 0, 0), (c[3], 1, 1))

    def ln_input(rb):
        x_copy(rb).wait()
        if isinstance(rb, int):
            for n in range(NWK):
                for part in range(1 << LEV):
                    wk_copy(n, part).start()
        for n in range(RB // 128):
            rows = pl.ds(pl.multiple_of(rb * RB + n * 128, 128), 128)
            x = xb_sc[rows, :].astype(f32)
            c = x - jnp.mean(x, axis=-1, keepdims=True)
            v = jnp.mean(c * c, axis=-1, keepdims=True)
            xn_sc[rows, :] = (c * lax.rsqrt(v + EPS)).astype(bf16)

    def proj_k_body(layer, rb, carry):
        @pl.when(layer == 0)
        def _():
            @pl.when(rb == 0)
            def _():
                for i in range(1, NRB):
                    x_copy(i).start()
            for j, name in ((1, "wq"), (1, "wv"), (2, "wo"), (3, "wr")):
                @pl.when(rb == j)
                def _():
                    cp[name].start()

            @pl.when(rb > 0)
            def _():
                ln_input(rb)
        h = RB // 2
        r0 = pl.multiple_of(rb * RB, RB)
        A = _lhs_ops(xn_sc[rows_of(rb), :], LEV)
        c, _ = _strassen(lambda i: jnp.dot(A[i], tk_sc[i], preferred_element_type=f32), False)
        zp = [None, None]
        for kk, th, nh in QUADS(c):
            pk = _phi(kk)
            zz = _row_fold(pk, jnp.add)
            zp[nh] = zz if zp[nh] is None else zp[nh] + zz
            rows = pl.ds(pl.multiple_of(r0 + th * h, h), h)
            for g in range(G // 2):
                k_sc[4 * nh + g, rows, :] = kk[:, 128 * g:128 * (g + 1)].astype(bf16)
                pk_sc[4 * nh + g, rows, :] = pk[:, 128 * g:128 * (g + 1)].astype(bf16)
        for nh in range(2):
            for g in range(G // 2):
                z_sc[rb, 4 * nh + g] = zp[nh][:, 128 * g:128 * (g + 1)]
        return carry

    def proj_qv_body(layer, rb, carry):
        @pl.when(jnp.logical_and(layer == 0, rb == 0))
        def _():
            for name in ("wg", "wu", "wd"):
                cp[name].start()
        h = RB // 2
        A = _lhs_ops(xn_sc[rows_of(rb), :], LEV)
        c, _ = _strassen(lambda i: lax.dot_general(tq_sc[i], A[i], NT, preferred_element_type=f32), True)
        for qq, th, nh in QUADS(c):
            pq = _phi(qq)
            for g in range(G // 2):
                qT_sc[rb, 4 * nh + g, :, th * h:(th + 1) * h] = (qq[128 * g:128 * (g + 1)] * QSCALE).astype(bf16)
                pqT_sc[rb, 4 * nh + g, :, th * h:(th + 1) * h] = pq[128 * g:128 * (g + 1)].astype(bf16)
        c, _ = _strassen(lambda i: lax.dot_general(tv_sc[i], A[i], NT, preferred_element_type=f32), True)
        for vv, th, nh in QUADS(c):
            for g in range(G // 2):
                vT_sc[rb, 4 * nh + g, :, th * h:(th + 1) * h] = vv[128 * g:128 * (g + 1)].astype(bf16)
        return carry

    TILES = [(s, i) for s in range(NSEG) for i in (3, 2, 1, 0)]
    STREAM = [(t, c) for t, (s, i) in enumerate(TILES) for c in range(i + 1)]
    NPOS = len(STREAM)

    def sref(k, h):
        return s_sc[k % NSLOT].at[pl.ds(pl.multiple_of(zero, 8), T), T * h:T * (h + 1)]

    def tcols(ref, g, t0, n, rows=slice(None)):
        parts = []
        for t in range(t0, t0 + n, min(n, RB)):
            parts.append(ref[t // RB, g, rows, t % RB:t % RB + min(n, RB)])
        return parts[0] if len(parts) == 1 else jnp.concatenate(parts, axis=1)

    def q_weights(g, s, i):
        QT = tcols(qT_sc, g, s * L + i * T, T)
        z = jnp.zeros((32, T), bf16)
        return jnp.concatenate(
            [jnp.concatenate([QT[32 * h:32 * h + 32] if hh == h else z for hh in range(4)], axis=0)
             for h in range(4)], axis=1)

    def q_weights_hi(g, s, i):
        QT = _pk(tcols(qT_sc, g, s * L + i * T, T))
        left = lax.broadcasted_iota(jnp.int32, (16, T), 1) < T // 2
        z = jnp.zeros((16, T), u32)
        blk = [jnp.where(left, pltpu.roll(QT[16 * h:16 * h + 16], T // 2, 1), z) if h % 2 == 0
               else jnp.where(left, z, QT[16 * h:16 * h + 16]) for h in range(4)]
        return _upk(jnp.concatenate(
            [jnp.concatenate([blk[h] if h // 2 == p else z for h in range(4)], axis=0) for p in range(2)], axis=1))

    def qk(g, k, m):
        t, c = STREAM[k]
        s, i = TILES[t]
        k0 = s * L + c * T
        if c == i:
            S4 = jnp.dot(k_sc[g, k0:k0 + T // 2, :], q_weights(g, s, i), preferred_element_type=f32)
            S2 = jnp.dot(k_sc[g, k0 + T // 2:k0 + T, :], q_weights_hi(g, s, i), preferred_element_type=f32)
        else:
            S4 = jnp.dot(k_sc[g, k0:k0 + T, :], q_weights(g, s, i), preferred_element_type=f32)
        out = []
        for h in range(4):
            Sx = S4[:, T * h:T * (h + 1)]
            if c == i:
                lo = S2[:, T * (h // 2):T * (h // 2 + 1)]
                Sx = jnp.concatenate([Sx, lo if h % 2 else pltpu.roll(lo, T // 2, 1)], axis=0)
                Sx = jnp.where(cmask, Sx, NEG)
            sref(k, h)[...] = Sx
            mm = Sx[0:8]
            for r in range(1, 16):
                mm = jnp.maximum(mm, Sx[8 * r:8 * r + 8])
            mm = mm if c == 0 else jnp.maximum(m[h], mm)
            if c == i:
                mm = jnp.broadcast_to(jnp.max(mm, axis=0, keepdims=True), (8, T))
            out.append(mm)
        return out

    def attn_prologue():
        m = {}
        for k in range(LAG):
            t = STREAM[k][0]
            m[t] = qk(0, k, m.get(t))
        return tuple(m[STREAM[0][0]]) + tuple(m[STREAM[LAG - 1][0]])

    def finish(g, s, i, O, l):
        outs = []
        for h in range(4):
            lt = jnp.sum(l[h], axis=0, keepdims=True)
            gt = jnp.concatenate([gt_sc[4 * g + h]] * 4, axis=0)
            o = O[h] * ((1.0 - gt) * (1.0 / lt))
            if s > 0:
                o = o + am_sc[32 * h:32 * h + 32, i * T:(i + 1) * T]
            outs.append(o)
        ot = jnp.concatenate(outs, axis=0).astype(bf16)
        r0 = s * L + i * T
        o_sc[g, r0:r0 + T, :] = ot.T

    def attn_body(g, carry):
        gn = jnp.minimum(g + 1, G - 1)
        m = {STREAM[0][0]: list(carry[0:4]), STREAM[LAG - 1][0]: list(carry[4:8])}
        l, O, P, M, mn = {}, {}, {}, {}, {}

        def mem_read(s):
            zs = z_sc[0, g]
            for rb in range(1, s * L // RB):
                zs = zs + z_sc[rb, g]
            zs = jnp.sum(zs, axis=0, keepdims=True)
            zrows = jnp.where(zmask, zs, 0.0).astype(bf16)
            mbd = jnp.where(hmask, M[0], 0.0).astype(bf16)
            lhs = jnp.concatenate([mbd, zrows], axis=0)
            pq = tcols(pqT_sc, g, s * L, L)
            nd = jnp.dot(lhs, pq, preferred_element_type=f32)
            for h in range(4):
                den = nd[128 + 8 * h:128 + 8 * h + 8] + 1e-06
                gd = jnp.concatenate([gt_sc[4 * g + h]] * 4, axis=1) / den
                am_sc[32 * h:32 * h + 32, :] = nd[32 * h:32 * h + 32] * jnp.concatenate([gd] * 4, axis=0)

        def mem_write(s):
            vt = tcols(vT_sc, g, s * L, L)
            pk = pk_sc[g, s * L:(s + 1) * L, :]
            inc = jnp.dot(vt, pk, preferred_element_type=f32)
            M[0] = inc if s == 0 else M[0] + inc

        def ex(k):
            t, c = STREAM[k]
            out = []
            for h in range(4):
                Pp = jnp.exp2(sref(k, h)[...] - jnp.concatenate([m[t][h]] * (T // 8), axis=0))
                a = Pp[0:8] + Pp[8:16]
                b = Pp[16:24] + Pp[24:32]
                for r in range(2, 8, 2):
                    a = a + (Pp[16 * r:16 * r + 8] + Pp[16 * r + 8:16 * r + 16])
                    b = b + (Pp[16 * r + 16:16 * r + 24] + Pp[16 * r + 24:16 * r + 32])
                ll = a + b
                if c == 0:
                    l.setdefault(t, [None] * 4)[h] = ll
                else:
                    l[t][h] = l[t][h] + ll
                out.append(Pp.astype(bf16))
            P[k] = out

        def pv(k):
            t, c = STREAM[k]
            s, i = TILES[t]
            if c == 0:
                O[t] = [None] * 4
            for h in range(4):
                vt = tcols(vT_sc, g, s * L + c * T, T, slice(32 * h, 32 * h + 32))
                o = jnp.dot(vt, P[k][h], preferred_element_type=f32)
                O[t][h] = o if O[t][h] is None else O[t][h] + o
            del P[k]

        finish(jnp.maximum(g - 1, 0), NSEG - 1, 0, carry[8:12], carry[12:16])
        done = None
        for j in range(NPOS):
            ex(j)
            k = j + LAG
            if k < NPOS:
                t = STREAM[k][0]
                m[t] = qk(g, k, m.get(t))
            else:
                t = STREAM[k - NPOS][0]
                mn[t] = qk(gn, k - NPOS, mn.get(t))
            pv(j)
            if done is not None:
                s, i = TILES[done]
                finish(g, s, i, O[done], l[done])
                if i == 0:
                    mem_read(s + 1)
                done = None
            t, c = STREAM[j]
            if c == TILES[t][1]:
                done = t
                if TILES[t][1] == 3 and TILES[t][0] < NSEG - 1:
                    mem_write(TILES[t][0])
        return (tuple(mn[STREAM[0][0]]) + tuple(mn[STREAM[LAG - 1][0]]) + tuple(O[done]) + tuple(l[done]))

    def attn_phase():
        init = attn_prologue() + (jnp.zeros((32, T), f32),) * 4 + (jnp.ones((8, T), f32),) * 4
        carry = lax.fori_loop(0, G, attn_body, init, unroll=2)
        finish(G - 1, NSEG - 1, 0, carry[8:12], carry[12:16])

    def out_body(ob_i, carry):
        wr = wr_sc[...].reshape(1, D).astype(f32)
        wr_sum = jnp.sum(wr, axis=-1, keepdims=True)
        h = RB // 2
        for k in range(OB // RB):
            r0 = pl.multiple_of(ob_i * OB + k * RB, RB)
            ob = jnp.concatenate([o_sc[g, pl.ds(r0, RB), :] for g in range(G)], axis=1)
            A = _lhs_ops(ob, LEV)
            c, _ = _strassen(lambda i: jnp.dot(A[i], _upk(to_sc[i]), preferred_element_type=f32), False)
            acc = [[None] * 3, [None] * 3]
            for cc, th, nh in QUADS(c):
                rows = pl.ds(pl.multiple_of(r0 + th * h, h), h)
                cols = slice(nh * HD, (nh + 1) * HD)
                x1 = xb_sc[rows, cols].astype(f32) + cc
                x1_sc[rows, cols] = x1
                s1, s2, st = acc[th]
                for n in range(HD // 128):
                    d = x1[:, 128 * n:128 * (n + 1)]
                    s1 = d if s1 is None else s1 + d
                    s2 = d * d if s2 is None else s2 + d * d
                    t = d * wr[:, nh * HD + 128 * n:nh * HD + 128 * (n + 1)]
                    st = t if st is None else st + t
                acc[th] = [s1, s2, st]
            for th in range(2):
                for b in range(h // 128):
                    s1, s2, st = (jnp.sum(t[128 * b:128 * (b + 1)].T, axis=0, keepdims=True) for t in acc[th])
                    mean = s1 * (1.0 / D)
                    v = jnp.maximum(s2 * (1.0 / D) - mean * mean, 0.0)
                    rs = lax.rsqrt(v + EPS)
                    r = rs * (st - mean * wr_sum)
                    a = 1.0 + rs
                    blk = pl.ds(ob_i * (OB // 128) + k * (RB // 128) + th * (h // 128) + b, 1)
                    mean_sc[blk, :] = mean
                    rs_sc[blk, :] = rs
                    kn_sc[blk, :] = a * lax.rsqrt(v * (a * a) + EPS)
                    r_sc[blk, :] = r.astype(bf16).astype(f32)
        return carry

    def out_phase():
        lax.fori_loop(0, NOB, out_body, 0)

    def ffn(layer):
        R = r_sc[...]
        bits = pltpu.bitcast(jnp.where(R == 0.0, 0.0, R), jnp.int32)
        idx = (lax.broadcasted_iota(jnp.int32, bits.shape, 0) * 128 + lax.broadcasted_iota(jnp.int32, bits.shape, 1))
        key = (jnp.where(bits < 0, bits ^ 0x7FFFFFFF, bits) & -65536) | (S - 1 - idx)

        def top(k):
            k1 = jnp.max(jnp.max(k, axis=0, keepdims=True), axis=1, keepdims=True)
            v = pltpu.bitcast(jnp.where(k1 < 0, k1 ^ 0x7FFFFFFF, k1) & -65536, f32)
            return k1, v, S - 1 - (k1[0, 0] & (S - 1))
        k1, v1, t1 = top(key)
        _, v2, t2 = top(jnp.where(key == k1, -2 ** 31, key))
        b1 = pl.ds(pl.multiple_of((t1 // 8) * 8, 8), 8)
        b2 = pl.ds(pl.multiple_of((t2 // 8) * 8, 8), 8)

        x1r = jnp.concatenate([x1_sc[b1, :], x1_sc[b2, :]], axis=0)
        mr = jnp.mean(x1r, axis=-1, keepdims=True)
        vr = jnp.maximum(jnp.mean(x1r * x1r, axis=-1, keepdims=True) - mr * mr, 0.0)
        xm = (x1r - mr) * lax.rsqrt(vr + EPS)
        xs = xm.astype(bf16)
        base = x1r + xm

        def mod_rows(n):
            rows = pl.ds(pl.multiple_of(n * CH, CH), CH)

            def per_row(ref):
                t = jnp.broadcast_to(ref[pl.ds(n, 1), :], (CH, 128)).T
                return jnp.concatenate([t] * (D // 128), axis=1)
            x1 = x1_sc[rows, :]
            c = x1 - per_row(mean_sc)
            xb_sc[rows, :] = (x1 + c * per_row(rs_sc)).astype(bf16)
            xn_sc[rows, :] = (c * per_row(kn_sc)).astype(bf16)

        def gate_up(j):
            cols = pl.ds(pl.multiple_of(j * FC, FC), FC)
            gg = jnp.dot(xs, wg_sc[:, cols], preferred_element_type=f32)
            uu = jnp.dot(xs, wu_sc[:, cols], preferred_element_type=f32)
            return (gg * _sigmoid(gg) * uu).astype(bf16)

        def down(j, hh):
            return jnp.dot(hh, wd_sc[pl.ds(pl.multiple_of(j * FC, FC), FC), :], preferred_element_type=f32)

        def step(j, carry):
            y, hh = carry

            @pl.when(jnp.logical_and(layer == 1, j > 1))
            def _():
                out_copy(j - 1).start()
            hn = gate_up(j)
            y = y + down(j - 1, hh)
            for i in range(CPS):
                mod_rows(PRO + (j - 1) * CPS + i)
            return y, hn

        for n in range(PRO):
            mod_rows(n)
            if n == 0:
                @pl.when(layer == 1)
                def _():
                    out_copy(NOUT).start()
        hh = gate_up(0)

        @pl.when(layer == 1)
        def _():
            out_copy(0).start()
        y, hh = lax.fori_loop(1, NOUT, step, (jnp.zeros((16, D), f32), hh))

        @pl.when(layer == 1)
        def _():
            out_copy(NOUT - 1).start()
        for j in range(NOUT, F // FC):
            hn = gate_up(j)
            y = y + down(j - 1, hh)
            hh = hn
        y = y + down(F // FC - 1, hh)
        r8 = lax.broadcasted_iota(jnp.int32, (8, D), 0)
        y1 = jnp.where(r8 == t1 % 8, y[0:8] * _sigmoid(v1), 0.0)
        y2 = jnp.where(r8 == t2 % 8, y[8:16] * _sigmoid(v2), 0.0)
        same = t1 // 8 == t2 // 8
        n1 = base[0:8] + (y1 + jnp.where(same, y2, 0.0))
        n2 = base[8:16] + (y2 + jnp.where(same, y1, 0.0))

        @pl.when(layer == 1)
        def _():
            for i in range(NOUT + 1):
                out_copy(i).wait()

        for b, xx in ((b1, n1), (b2, n2)):
            xb_sc[b, :] = xx.astype(bf16)
            cc = xx - jnp.mean(xx, axis=-1, keepdims=True)
            xn_sc[b, :] = (cc * lax.rsqrt(jnp.mean(cc * cc, axis=-1, keepdims=True) + EPS)).astype(bf16)

        @pl.when(layer == 1)
        def _():
            c1 = pltpu.make_async_copy(xb_sc.at[b1, :], out_hbm.at[b1, :], sems.at[7])
            c1.start()

            @pl.when(jnp.logical_not(same))
            def _():
                c2 = pltpu.make_async_copy(xb_sc.at[b2, :], out_hbm.at[b2, :], sems.at[8])
                c2.start()
                c2.wait()
            c1.wait()

    def prep_k_piece(n, c):
        for part in range(1 << LEV):
            wk_copy(n, part).wait()
        return lax.fori_loop(n * (NPC // NWK), (n + 1) * (NPC // NWK),
                             lambda m, c_: (_prep(tk_sc, wk_sc, m, NPC, False), c_)[1], c)

    ln_input(0)
    lax.fori_loop(0, NWK, prep_k_piece, 0)

    def layer_body(layer, carry):
        first = layer == 0
        lax.fori_loop(0, NRB, functools.partial(proj_k_body, layer), 0)

        @pl.when(first)
        def _():
            cp["wq"].wait()
            prep_tr(tq_sc, wq_sc)
            cp["wv"].wait()
            prep_tr(tv_sc, wv_sc)
        lax.fori_loop(0, NRB, functools.partial(proj_qv_body, layer), 0)
        attn_phase()

        @pl.when(first)
        def _():
            cp["wo"].wait()
            cp["wr"].wait()
            prep_nat(to_sc, wo_sc)
        out_phase()

        @pl.when(first)
        def _():
            cp["wg"].wait()
            cp["wu"].wait()
            cp["wd"].wait()
        ffn(layer)
        return carry

    lax.fori_loop(0, 2, layer_body, 0)


@jax.jit
def pallas_interleave_layers__memory_aug_infini_attn__moe_arch_mod__prompt_kernel(
    A_x: jax.Array,
    A_wq: jax.Array,
    A_wk: jax.Array,
    A_wv: jax.Array,
    A_wo: jax.Array,
    A_beta: jax.Array,
    B_x: jax.Array,
    B_w_r: jax.Array,
    B_w_gate: jax.Array,
    B_w_up: jax.Array,
    B_w_down: jax.Array,
):
    del B_x
    x = A_x.reshape(S, D)
    zero = jnp.zeros((1,), jnp.int32)
    any_spec = pl.BlockSpec(memory_space=pl.ANY)
    smem_spec = pl.BlockSpec(memory_space=pltpu.SMEM)
    V = pltpu.VMEM
    scratch = [
        V((S, D), f32),
        V((S, D), bf16),
        V((S, D), bf16),
        V((S // 128, 128), f32), V((S // 128, 128), f32), V((S // 128, 128), f32), V((S // 128, 128), f32),
            V((NP, BD, BD), bf16), V((NP, BD, BD), bf16), V((NP, BD, BD), bf16),
        V((NP, BD // 2, BD), u32),
    ] + [
        V((D, D), bf16), V((D, D), bf16), V((D, D), bf16), V((D, D), bf16),
        V((D, D), bf16),
        V((D,), bf16),
        V((D, F), bf16), V((D, F), bf16), V((F, D), bf16),
        V((G, S, 128), bf16), V((G, S, 128), bf16),
        V((NRB, G, 128, RB), bf16), V((NRB, G, 128, RB), bf16), V((NRB, G, 128, RB), bf16),
        V((G, S, 128), bf16),
        V((NRB, G, 8, 128), f32),
        V((H, 8, 128), f32),
        V((T, 4 * T), f32),
        pltpu.SemaphoreType.DMA((9,)),
        pltpu.SemaphoreType.DMA((NOUT + 1,)),
        pltpu.SemaphoreType.DMA((NRB,)),
        pltpu.SemaphoreType.DMA((NWK, 1 << LEV)),
    ] + [V((T, 4 * T), f32)] * NSLOT
    out = pl.pallas_call(
        _kernel,
        in_specs=[smem_spec, pl.BlockSpec(memory_space=pltpu.VMEM)] + [any_spec] * 9,
        out_specs=any_spec,
        out_shape=jax.ShapeDtypeStruct((S, D), bf16),
        scratch_shapes=scratch,
        compiler_params=pltpu.CompilerParams(vmem_limit_bytes=120 * 1024 * 1024),
    )(zero, A_beta, x, A_wq, A_wk, A_wv, A_wo, B_w_r, B_w_gate, B_w_up, B_w_down)
    return out.reshape(1, S, D)
```
